```python
import jax
import jax.numpy as jnp

def _softmax(x, axis=-1):
    return jax.nn.softmax(x, axis=axis)
def _gelu(x):
    return jax.nn.gelu(x, approximate=True)
def _silu(x):
    return jax.nn.silu(x)
def _sigmoid(x):
    return jax.nn.sigmoid(x)
def _layernorm(x, axis=-1, eps=1e-5):
    m = jnp.mean(x, axis=axis, keepdims=True)
    v = jnp.var(x, axis=axis, keepdims=True)
    return (x - m) / jnp.sqrt(v + eps)
def _scatter_add(tgt, idx, src, axis=0):
    return tgt.at[idx].add(src)
def _segment_sum(src, seg, n):
    return jax.ops.segment_sum(src, seg, n)
class _Rng:
    def __init__(self, key):
        self._k = key
    def _next(self):
        self._k, sub = jax.random.split(self._k)
        return sub
    def normal(self, shape):
        return jax.random.normal(self._next(), shape, dtype=jnp.bfloat16)
    def randint(self, lo, hi, shape):
        return jax.random.randint(self._next(), shape, lo, hi, dtype=jnp.int32)
    def uniform(self, shape, lo=0.0, hi=1.0):
        return jax.random.uniform(self._next(), shape, jnp.bfloat16, lo, hi)
    def permutation(self, n):
        return jax.random.permutation(self._next(), n)


kernel_name = 'recurrent_scan__linear_kernel_hedgehog__moe_arch_mod__prompt'

def setup_inputs():
    _rng = _Rng(jax.random.key(int.from_bytes(__import__("os").urandom(4), "little")))
    _w = (lambda a: (lambda t: t.astype(jnp.bfloat16) if jnp.issubdtype(t.dtype, jnp.floating) else t)(jnp.asarray(a)))
    def _A_setup():
        B, S, D, H = 1, 2048, 1024, 32
        Dh = D // H
        return {
            "x": _w((lambda *s: _rng.normal(s) * 0.05)(B, S, D)),
            "wqkv": _w((lambda *s: _rng.normal(s) * 0.05)(D, 3 * D)),
            "w_phi": _w((lambda *s: _rng.normal(s) * 0.05)(H, Dh, Dh) * (Dh ** -0.5)),
            "wo": _w((lambda *s: _rng.normal(s) * 0.05)(D, D)),
        }
    _A_in = _A_setup()

    def _B_setup():
        B, S, D, F, C = 1, 2048, 1024, 3584, 1
        return {
            "x": _w((lambda *s: _rng.normal(s) * 0.05)(B, S, D)),
            "w_r": _w((lambda *s: _rng.normal(s) * 0.05)(D)),
            "w_gate": _w((lambda *s: _rng.normal(s) * 0.05)(D, F)),
            "w_up": _w((lambda *s: _rng.normal(s) * 0.05)(D, F)),
            "w_down": _w((lambda *s: _rng.normal(s) * 0.05)(F, D)),
        }
    _B_in = _B_setup()

    return {
        "A_x": _A_in["x"],
        "A_wqkv": _A_in["wqkv"],
        "A_w_phi": _A_in["w_phi"],
        "A_wo": _A_in["wo"],
        "B_x": _B_in["x"],
        "B_w_r": _B_in["w_r"],
        "B_w_gate": _B_in["w_gate"],
        "B_w_up": _B_in["w_up"],
        "B_w_down": _B_in["w_down"],
    }

def reference(A_x, A_wqkv, A_w_phi, A_wo, B_x, B_w_r, B_w_gate, B_w_up, B_w_down):
    def _A_ref(x, wqkv, w_phi, wo):
        B, S, D = x.shape
        H = 32; Dh = D // H
        qkv = (lambda x, *d: x.transpose(*d))((x @ wqkv).reshape(B, S, 3, H, Dh), 2, 0, 3, 1, 4)
        q, k, v = qkv[0], qkv[1], qkv[2]
        pq = jnp.einsum("bhsd,hdf->bhsf", q, w_phi)
        pk = jnp.einsum("bhsd,hdf->bhsf", k, w_phi)
        phi_q = jnp.concatenate([_softmax(pq, axis=-1), _softmax(-pq, axis=-1)], axis=-1)
        phi_k = jnp.concatenate([_softmax(pk, axis=-1), _softmax(-pk, axis=-1)], axis=-1)
        kv = jnp.einsum("bhsf,bhsd->bhfd", phi_k, v)
        z  = jnp.einsum("bhsf->bhf", phi_k)
        num = jnp.einsum("bhqf,bhfd->bhqd", phi_q, kv)
        den = jnp.einsum("bhqf,bhf->bhq", phi_q, z)[..., None] + 1e-6
        o = num / den
        return (lambda x, *d: x.transpose(*d))(o, 0, 2, 1, 3).reshape(B, S, D) @ wo

    def _B_ref(x, w_r, w_gate, w_up, w_down):
        B, S, D = x.shape
        C = 1
        r = x @ w_r
        idx = jnp.argsort(-r, axis=-1)[:, :C]
        idx_e = jnp.repeat(idx.reshape(B, C, 1), D, axis=2)
        x_sel = jnp.take_along_axis(x, idx_e, axis=1)
        g = _silu(x_sel @ w_gate)
        u = x_sel @ w_up
        y = (g * u) @ w_down
        r_sel = _sigmoid(jnp.take_along_axis(r, idx, axis=1))
        y = y * r_sel.reshape(B, C, 1)
        b_off = (jnp.arange(B) * S).reshape(B, 1)
        flat_idx = (idx + b_off).reshape(B * C)
        zero = (x * 0.0).reshape(B * S, D)
        upd = _scatter_add(zero, flat_idx, y.reshape(B * C, D), axis=0)
        return x + upd.reshape(B, S, D)

    x = A_x
    xn = _layernorm(x, axis=-1)
    s = _A_ref(xn, A_wqkv, A_w_phi, A_wo)
    g = _silu(_B_ref(xn, B_w_r, B_w_gate, B_w_up, B_w_down))
    return x + s * g
```

```python
import jax
import jax.numpy as jnp
from jax import lax
import jax.experimental.pallas as pl
import jax.experimental.pallas.tpu as pltpu

BF = jnp.bfloat16
F32 = jnp.float32
U32 = jnp.uint32
NN = (((1,), (0,)), ((), ()))
NT = (((1,), (1,)), ((), ()))
LOG2E = 1.4426950408889634

D, H, DH, FF = 1024, 32, 32, 3584
L = 128
HK = D // 2
KH = HK // L
NG = H // 4
NP = H // 2
TT = 2 * L
FC = 4 * L
NFC = FF // FC


def _dot(a, b, dims):
    return lax.dot_general(a, b, dims, preferred_element_type=F32)


def _unpack(w):
    return pltpu.bitcast(w, BF)


def _rnd(v):
    return v.astype(BF).astype(F32)


def _rcp(v):
    r = pltpu.reciprocal(v, approx=True)
    return r * (2.0 - v * r)


def _silu(v):
    h = 0.5 * v
    return h + h * jnp.tanh(h)


def _tree(v, op):
    while len(v) > 1:
        v = [op(v[i], v[i + 1]) for i in range(0, len(v), 2)]
    return v[0]


def _pair_reduce(v, op):
    r = _tree(v, op)
    r = op(r, pltpu.roll(r, 2, 0))
    return op(r, pltpu.roll(r, 4, 0))


def _dual_softmax(p):
    v = [p[8 * i:8 * i + 8] for i in range(8)]
    mx = _pair_reduce(v, jnp.maximum)
    mn = _pair_reduce(v, jnp.minimum)
    ep = [jnp.exp2(a - mx) for a in v]
    en = [jnp.exp2(mn - a) for a in v]
    rp = _rcp(_pair_reduce(ep, jnp.add))
    rn = _rcp(_pair_reduce(en, jnp.add))
    return jnp.concatenate([a * rp for a in ep] + [a * rn for a in en], axis=0).astype(BF)


def _lhs_operands(a11, a12, a21, a22):
    return (a11 + a22, a21 + a22, a11, a22, a11 + a12, a21 - a11, a12 - a22)


def _rhs_operands(b11, b12, b21, b22):
    return (b11 + b22, b11, b12 - b22, b21 - b11, b22, b11 + b12, b21 + b22)


_USES = ((0, 1.0, 3, 1.0), (2, 1.0, 3, -1.0), (1, 1.0, 3, 1.0), (0, 1.0, 2, 1.0),
         (0, -1.0, 1, 1.0), (3, 1.0), (0, 1.0))


def _strassen(lhs, rhs, dims, gap, order):
    pos, neg = [None] * 4, [None] * 4
    for j in order:
        m = gap(_dot(lhs(j), rhs(j), dims))
        for c, sign in zip(_USES[j][::2], _USES[j][1::2]):
            if sign > 0:
                pos[c] = m if pos[c] is None else pos[c] + m
            else:
                neg[c] = m
            if pos[c] is not None and neg[c] is not None:
                pos[c], neg[c] = pos[c] - neg[c], None
    return pos


class _Tasks:
    def __init__(self):
        self.q = []

    def add(self, gen):
        self.q.append(gen)

    def step(self, n=1):
        while n > 0 and self.q:
            try:
                next(self.q[0])
                n -= 1
            except StopIteration:
                self.q.pop(0)

    def drain(self):
        while self.q:
            self.step()


def make(S=2048, PR=1, FSTEP=1, FROWS=128, PROWS=64, PGAP=2, OGAP=1, LGAP=1, FLAGS=None, PROF=0, FSTART=2,
         MODE='', KVPOS=(1, 2, 4, 5), NDPOS=(3, 4, 5, 6, 7, 8, 9, 10), ORDER=(1, 3, 0, 4, 2, 6, 5), LNP=7, NOSIDE=0, ANCH=1, PROBE=1, FPAT=None):
    NTILE = S // TT
    SF = NTILE + 3 * NG + 3
    XS = 0
    AKV = XS + 9 * KH * (S // 2)
    AQ = AKV + 7 * KH * D
    BO = AQ + 7 * KH * HK
    PRB = BO + 7 * KH * HK
    END = PRB + 16
    NSUB = HK // FROWS
    NPART = (32 + 8 * NFC) * NSUB
    GU = S
    WD = GU + NFC * D
    WO = WD + FF
    ANCHOR = WO + D

    def kernel(x_hbm, wqkv_hbm, wphi_hbm, wo_hbm, wr_hbm, wg_hbm, wu_hbm, wd_hbm, out_hbm,
               wide, w_v, wphi_v, wr_v, fm_v, part, ar, oa0, oa1, kvl, kv_acc, out_v, xb, hb0, hb1, sems):

        def x_copy(n):
            return pltpu.make_async_copy(x_hbm.at[0, pl.ds(n * TT, TT)], wide.at[pl.ds(n * TT, TT)], sems.at[n])

        def w_copy(c):
            return pltpu.make_async_copy(wqkv_hbm.at[:, pl.ds(c * L, L)], w_v.at[c], sems.at[NTILE + c])

        wo_copy = pltpu.make_async_copy(wo_hbm, wide.at[pl.ds(WO, D)], sems.at[SF - 3])
        wphi_copy = pltpu.make_async_copy(wphi_hbm, wphi_v, sems.at[SF - 2])
        wr_copy = pltpu.make_async_copy(wr_hbm, wr_v, sems.at[SF - 1])

        def f_copies(c):
            cols = pl.ds(c * FC, FC)
            rows = pl.ds(GU + c * D, D)
            return [pltpu.make_async_copy(wg_hbm.at[:, cols], wide.at[rows, pl.ds(0, FC)], sems.at[SF + 3 * c]),
                    pltpu.make_async_copy(wu_hbm.at[:, cols], wide.at[rows, pl.ds(FC, FC)], sems.at[SF + 3 * c + 1]),
                    pltpu.make_async_copy(wd_hbm.at[cols], wide.at[pl.ds(WD + c * FC, FC)], sems.at[SF + 3 * c + 2])]

        def out_copy(row0, i):
            return pltpu.make_async_copy(out_v.at[pl.ds(row0, TT)], out_hbm.at[0, pl.ds(row0, TT)],
                                         sems.at[SF + 3 * NFC + i])

        def kv_copies(g):
            return [w_copy(NG + g), w_copy(2 * NG + g)]

        order = [wr_copy, wphi_copy, x_copy(0)]
        for g in range(NG):
            order += kv_copies(g)
            if g == 5:
                order.append(x_copy(1))
        order += [x_copy(n) for n in range(2, NTILE)]
        order += [w_copy(g) for g in range(NG)] + [wo_copy]
        for c in range(NFC):
            order += f_copies(c)
        if MODE:
            order = order[:2]
        for cp in order:
            cp.start(priority=PR)

        def wait(name, cps):
            if MODE and name != 'small':
                return
            if PROF:
                with jax.named_scope(name):
                    for cp in cps:
                        cp.wait()
            else:
                for cp in cps:
                    cp.wait()

        ar_w = ar.bitcast(U32)
        probes = set()

        wait('small', [wr_copy, wphi_copy])
        wr1 = wr_v[...].astype(F32).reshape(1, D)
        zero = pl.multiple_of(jnp.max(jnp.where(jnp.abs(wr1) < 0.0, pltpu.bitcast(wr1, jnp.int32), 0)), 16)

        rr = lax.broadcasted_iota(jnp.int32, (L, DH), 0)
        ff = lax.broadcasted_iota(jnp.int32, (L, DH), 1)
        sel = jnp.where(((rr & 63) >> 1) == ff, 1.0, 0.0).astype(BF)
        r2 = lax.broadcasted_iota(jnp.int32, (L, L), 0)
        c2 = lax.broadcasted_iota(jnp.int32, (L, L), 1)
        own = ((r2 >> 6) * 2 + (r2 & 1)) == (c2 >> 5)
        for g in range(0 if MODE else NG):
            a = wphi_v[4 * g:4 * g + 4].reshape(L, DH)
            fm_v[g] = jnp.where(own, _dot(sel, a, NT), 0.0).astype(BF)

        def put(row, v):
            probes.add('ar')
            ar[pl.ds(row, v.shape[0]), :] = v.astype(BF)

        def get(row, rows):
            return _unpack(ar_w[pl.ds(row // 2, rows // 2), :])

        def slabs(base, stride, j, row0, rows):
            return _unpack(jnp.concatenate(
                [ar_w[pl.ds((base + (j * KH + s) * stride) // 2 + row0, rows // 2), :] for s in range(KH)], axis=1))

        def folded(g, r0, rows, c, s):
            fm = _unpack(fm_v.bitcast(U32)[g, pl.ds(r0 // 2, rows // 2), :])
            return _dot(fm, _unpack(w_v.bitcast(U32)[c, pl.ds(s * L // 2, L // 2), :]), NT) * LOG2E

        def prep_kv(g):
            for s in range(KH):
                a11 = folded(g, 0, L, NG + g, s)
                a12 = folded(g, 0, L, NG + g, KH + s)
                a21 = w_v[2 * NG + g, pl.ds(s * L, L), :].astype(F32).T
                a22 = w_v[2 * NG + g, pl.ds(HK + s * L, L), :].astype(F32).T
                for j, v in enumerate(_lhs_operands(a11, a12, a21, a22)):
                    put(AKV + (j * KH + s) * D + g * L, v)
                if s % 2:
                    yield
                    yield

        def prep_q():
            for g in range(KH):
                for s in range(KH):
                    for r0 in range(0, L, PROWS):
                        ops = _lhs_operands(folded(g, r0, PROWS, g, s), folded(g, r0, PROWS, g, KH + s),
                                            folded(KH + g, r0, PROWS, KH + g, s),
                                            folded(KH + g, r0, PROWS, KH + g, KH + s))
                        for j, v in enumerate(ops):
                            put(AQ + (j * KH + s) * HK + g * L + r0, v)
                        for _ in range(PGAP):
                            yield

        def prep_o():
            for c in range(KH):
                for r0 in range(0, HK, 32):
                    def blk(kh, nh):
                        return wide[pl.ds(WO + kh * HK + r0, 32), pl.ds(nh * HK + c * L, L)].astype(F32)
                    for j, v in enumerate(_rhs_operands(blk(0, 0), blk(0, 1), blk(1, 0), blk(1, 1))):
                        put(BO + (j * KH + c) * HK + r0, v)
                    for _ in range(OGAP):
                        yield

        wr = jnp.broadcast_to(wr1, (16, D))
        best = [jnp.full((16, 1), -jnp.inf, F32), jnp.zeros((16, 1), jnp.int32)]

        def layernorm(n, pause):
            for c in range(L // 16):
                rows = (n * TT + c * 16, n * TT + L + c * 16)
                xf = [wide[pl.ds(r0, 16), :].astype(F32) for r0 in rows]
                mean = [jnp.sum(v, axis=1, keepdims=True) * (1.0 / D) for v in xf]
                d = [v - m for v, m in zip(xf, mean)]
                var = [jnp.sum(v * v, axis=1, keepdims=True) * (1.0 / D) for v in d]
                dr = [jnp.sum(v * wr, axis=1, keepdims=True) for v in d]
                rs = [_rcp(_rnd(jnp.sqrt(_rnd(_rnd(v) + 1e-5)))) for v in var]
                for r0, a, b in zip(rows, dr, rs):
                    r = a * b
                    up = r > best[0]
                    best[0] = jnp.where(up, r, best[0])
                    best[1] = jnp.where(up, r0, best[1])
                for s in range(KH):
                    b11, b21, b12, b22 = [d[t][:, k0 + s * L:k0 + (s + 1) * L] * rs[t]
                                          for t in range(2) for k0 in (0, HK)]
                    for j, t in enumerate(_rhs_operands(b11, b12, b21, b22) + (b12, b21)):
                        put(XS + (j * KH + s) * (S // 2) + n * L + c * 16, t)
                for _ in range(pause):
                    yield

        side = _Tasks()
        prep = _Tasks()
        tail = _Tasks()
        tail2 = _Tasks()

        count = [0]
        pattern = []

        never = zero > 0
        ar[pl.ds(PRB, 16), :] = jnp.zeros((16, L), BF)
        part[NPART] = jnp.zeros((8, L), F32)

        def gap(m):
            count[0] += 1
            if PROBE and count[0] % PROBE == 0:
                head = m[:8]
                if 'ar' in probes:
                    head = jnp.where(never, pltpu.bitcast(ar_w[pl.ds(PRB // 2 + zero, 8), :], F32), head)
                if 'part' in probes:
                    head = jnp.where(never, part[NPART + zero], head)
                if probes:
                    m = jnp.concatenate([head, m[8:]], axis=0)
                probes.clear()
            if (side.q or prep.q) and count[0] % ANCH == 0:
                wide[pl.ds(ANCHOR + zero, 8), pl.ds(0, 2 * L)] = jnp.concatenate([m[8:16], m[16:24]], axis=1).astype(BF)
            if prep.q:
                w_v[3 * NG, pl.ds(zero, 16), :] = m[8:24].astype(BF)
            tail.step()
            tail2.step()
            side.step(pattern.pop(0) if pattern else FSTEP)
            prep.step()
            return m

        def kv_tail(g, n, c11, c12, c21, c22):
            parts = []
            now = 0
            for b, (pp, ck, cv) in enumerate(((0, c12, c22), (1, c12, c22), (0, c11, c21), (1, c11, c21))):
                rows = slice(pp * 64, (pp + 1) * 64)
                vt = jnp.concatenate([cv[rows], jnp.ones((16, L), F32)], axis=0).astype(BF)
                phi = _dual_softmax(ck[rows])
                while now < KVPOS[b]:
                    now += 1
                    yield
                parts.append(_dot(vt, phi, NT))
                if b >= 2:
                    upd = parts[pp] + parts[b]
                    kv_acc[2 * g + pp] = upd if n == 0 else kv_acc[2 * g + pp] + upd

        route = {}

        def router():
            rmax = jnp.max(best[0])
            pos = best[1] + lax.broadcasted_iota(jnp.int32, (16, 1), 0)
            idx = jnp.min(jnp.where(best[0] == rmax, pos, S - 1))
            last = idx // TT
            half = (idx // L) % 2
            base = pl.multiple_of((last * L + ((idx % L) // 16) * 16) // 2, 8)
            hit = lax.broadcasted_iota(jnp.int32, (16, HK), 0) == idx % 16
            route.update(rmax=rmax, idx=idx, last=last)
            for k0, j1, j2 in ((0, 1, 7), (HK, 8, 4)):
                a = slabs(XS, S // 2, j1, base, 16).astype(F32)
                b = slabs(XS, S // 2, j2, base, 16).astype(F32)
                row = jnp.sum(jnp.where(hit, jnp.where(half == 0, a, b), 0.0), axis=0, keepdims=True)
                for s in range(KH):
                    xb[pl.ds(k0 + s * L, L), :] = jnp.broadcast_to(row[:, s * L:(s + 1) * L], (L, L)).T
                    yield

        wait('x0', [x_copy(0)])
        if not MODE:
            side.add(layernorm(0, 0))
            side.drain()
            wait('w0', kv_copies(0))
            prep.add(prep_kv(0))
        first_waits = {0: kv_copies(1), 1: kv_copies(2), 2: kv_copies(3), 3: kv_copies(4) + kv_copies(5),
                       5: [x_copy(1)] + kv_copies(6) + kv_copies(7)}
        NPREP = 3 if NTILE == 8 else 1
        for n in range({'': NTILE, 'A': NTILE - 1, 'B': 0}[MODE]):
            for g in range(NG):
                if MODE:
                    if g == 0 and not NOSIDE:
                        side.drain()
                        side.add(layernorm(n + 1, LNP))
                elif n == 0:
                    prep.drain()
                    if g in first_waits:
                        wait(f'w{g + 1}', first_waits[g])
                    if g + 1 < NG:
                        prep.add(prep_kv(g + 1))
                    if g == 5:
                        side.add(layernorm(1, 2))
                elif g == 0:
                    side.drain()
                    if n == 1:
                        wait('x2', [x_copy(i) for i in range(2, min(5, NTILE))])
                    if n == NPREP:
                        wait('wq', [x_copy(i) for i in range(5, NTILE)] + [w_copy(i) for i in range(NG)] + [wo_copy])
                        prep.add(prep_q())
                        prep.add(prep_o())
                    side.add(layernorm(n + 1, LNP) if n + 1 < NTILE else router())
                cs = _strassen(lambda j: slabs(AKV, D, j, g * L // 2, L),
                               lambda j: slabs(XS, S // 2, j, n * L // 2, L), NT, gap, ORDER)
                tail.drain()
                tail.add(kv_tail(g, n, *cs))
        side.drain()
        prep.drain()
        if MODE == 'A':
            tail.drain()
            out_v[pl.ds(0, 16), pl.ds(0, 1)] = (best[0] + best[1]).astype(BF)
            return
        if MODE == 'B':
            route.update(rmax=jnp.max(wr1), idx=zero, last=zero)
        rmax, idx, last = route['rmax'], route['idx'], route['last']

        def finish_kv():
            r3 = lax.broadcasted_iota(jnp.int32, (80, L), 0)
            c3 = lax.broadcasted_iota(jnp.int32, (80, L), 1)
            keep = jnp.where(r3 < 64, r3 >> 5, (r3 - 64) >> 3) == (c3 & 1)
            for p in range(NP):
                kvl[p] = jnp.where(keep, kv_acc[p], 0.0).astype(BF)
            yield

        if not MODE:
            tail.add(finish_kv())

        ffn_out = []

        def matvec(row0, col0, vec, k0, slot):
            acc = [[None, None], [None, None]]
            for k in range(k0, k0 + FROWS, 8):
                vk = vec[pl.ds(k, 8), :]
                wk = wide[pl.ds(row0 + k, 8), pl.ds(col0, 2 * L)].astype(F32)
                for t in range(2):
                    pr = wk[:, t * L:(t + 1) * L] * vk
                    a = acc[t][(k // 8) % 2]
                    acc[t][(k // 8) % 2] = pr if a is None else a + pr
            probes.add('part')
            for t in range(2):
                part[slot(t)] = acc[t][0] + acc[t][1]

        def total(slots):
            return _tree([part[s] for s in slots], jnp.add)

        def ffn():
            def gu_slot(c, t, p):
                return ((c % 2) * 8 + t) * 2 * NSUB + p

            def y_slot(c, t, p):
                return 32 * NSUB + (t * NFC + c) * NSUB + p

            def down(c):
                for t in range(0, 8, 2):
                    for p in range(NSUB):
                        matvec(WD + c * FC, t * L, (hb0, hb1)[c % 2], p * FROWS, lambda u: y_slot(c, t + u, p))
                        yield

            for c in range(NFC):
                for t in range(0, 8, 2):
                    for p in range(2 * NSUB):
                        matvec(GU + c * D, t * L, xb, p * FROWS, lambda u: gu_slot(c, t + u, p))
                        yield
                for t in range(4):
                    gt = jnp.sum(total([gu_slot(c, t, p) for p in range(2 * NSUB)]), axis=0, keepdims=True)
                    ut = jnp.sum(total([gu_slot(c, 4 + t, p) for p in range(2 * NSUB)]), axis=0, keepdims=True)
                    (hb0, hb1)[c % 2][pl.ds(t * L, L), :] = jnp.broadcast_to(_silu(gt) * ut, (L, L)).T
                yield
                if c > 0:
                    yield from down(c - 1)
            yield
            yield
            yield from down(NFC - 1)
            gate = 1.0 / (1.0 + jnp.exp(-jnp.full((8, L), rmax, F32)))
            for t in range(8):
                yt = sum(total([y_slot(c, t, p) for p in range(NSUB)]) for c in range(NFC))
                ffn_out.append(jnp.broadcast_to(jnp.sum(yt, axis=0, keepdims=True), (8, L)) * gate)

        def tile_of(i):
            return (last + 1 + i) % NTILE

        def q_tail(g, i, c11, c12, c21, c22):
            blocks = {}
            now = 0
            for b, (gg, ck) in enumerate(((KH + g, c21), (g, c12), (g, c11), (KH + g, c22))):
                rows_out = []
                for pp in range(2):
                    phi = _dual_softmax(ck[pp * 64:(pp + 1) * 64])
                    while now < NDPOS[2 * b + pp]:
                        now += 1
                        yield
                    nd = _dot(_unpack(kvl.bitcast(U32)[2 * gg + pp]), phi, NN)
                    for jj in range(2):
                        rd = _rcp(nd[64 + 8 * jj:72 + 8 * jj] + 1e-6)
                        rows_out += [nd[jj * DH + 8 * q:jj * DH + 8 * q + 8] * rd for q in range(4)]
                blocks[b] = jnp.concatenate(rows_out, axis=0).T
            a12, a21, a11, a22 = blocks[0], blocks[1], blocks[2], blocks[3]
            for r0 in (0, 64):
                sl = slice(r0, r0 + 64)
                for j, v in enumerate(_lhs_operands(a11[sl], a12[sl], a21[sl], a22[sl])):
                    (oa0, oa1)[i % 2][j, g, sl, :] = v.astype(BF)

        def o_tail(c, i, c11, c12, c21, c22):
            t = tile_of(i)
            xrow = pl.multiple_of(t * (L // 2), L // 2)
            for th, nh, sblk, j in ((0, 0, c11, 1), (0, 1, c12, 8), (1, 0, c21, 7), (1, 1, c22, 4)):
                rows = pl.ds(pl.multiple_of(t * TT + th * L, L), L)
                cols = pl.ds(nh * HK + c * L, L)
                xn = _unpack(ar_w[pl.ds((XS + (j * KH + c) * (S // 2)) // 2 + xrow, L // 2), :]).astype(F32)
                if i == NTILE - 1:
                    yv = ffn_out[nh * KH + c]
                    rid = lax.broadcasted_iota(jnp.int32, (L, L), 0) + th * L
                    xn = xn + jnp.where(rid == idx % TT, jnp.concatenate([yv] * (L // 8), axis=0), 0.0)
                out_v[rows, cols] = (wide[rows, cols].astype(F32) + sblk * _silu(xn)).astype(BF)
                yield
            if c == KH - 1:
                out_copy(pl.multiple_of(t * TT, TT), i).start()

        def q_unit(g, i):
            xrow = pl.multiple_of(tile_of(i) * (L // 2), L // 2)
            cs = _strassen(lambda j: slabs(AQ, HK, j, g * L // 2, L),
                           lambda j: slabs(XS, S // 2, j, xrow, L), NT, gap, ORDER)
            tail.drain()
            tail.add(q_tail(g, i, *cs))

        def o_unit(c, i):
            oa = (oa0, oa1)[i % 2].bitcast(U32)
            cs = _strassen(lambda j: _unpack(jnp.concatenate([oa[j, s] for s in range(KH)], axis=1)),
                           lambda j: get(BO + (j * KH + c) * HK, HK), NN, gap, ORDER)
            tail2.drain()
            if i == NTILE - 1:
                side.drain()
            tail2.add(o_tail(c, i, *cs))

        for g in range(KH):
            if g == FSTART:
                wait('f', [cp for c in range(NFC) for cp in f_copies(c)])
                if not NOSIDE:
                    side.add(ffn())
            if MODE != 'B':
                q_unit(g, 0)
        for i in range(1, NTILE):
            for g in range(KH):
                if FPAT:
                    pattern.extend(FPAT)
                q_unit(g, i)
                o_unit(g, i - 1)
        tail.drain()
        for c in range(KH):
            if MODE != 'B':
                o_unit(c, NTILE - 1)
        tail2.drain()
        wait('out', [out_copy(0, i) for i in range(NTILE)])

    @jax.jit
    def run(A_x, A_wqkv, A_w_phi, A_wo, B_x, B_w_r, B_w_gate, B_w_up, B_w_down):
        any_spec = pl.BlockSpec(memory_space=pl.ANY)
        return pl.pallas_call(
            kernel,
            out_shape=jax.ShapeDtypeStruct(A_x.shape, A_x.dtype),
            in_specs=[any_spec] * 8,
            out_specs=any_spec,
            scratch_shapes=[
                pltpu.VMEM((ANCHOR + 8, D), BF),
                pltpu.VMEM((3 * NG + 1, D, L), BF),
                pltpu.VMEM((H, DH, DH), BF),
                pltpu.VMEM((D,), BF),
                pltpu.VMEM((NG, L, L), BF),
                pltpu.VMEM((NPART + 1, 8, L), F32),
                pltpu.VMEM((END, L), BF),
                pltpu.VMEM((7, KH, L, L), BF),
                pltpu.VMEM((7, KH, L, L), BF),
                pltpu.VMEM((NP, 80, L), BF),
                pltpu.VMEM((NP, 80, L), F32),
                pltpu.VMEM((S, D), BF),
                pltpu.VMEM((D, L), F32),
                pltpu.VMEM((FC, L), F32),
                pltpu.VMEM((FC, L), F32),
                pltpu.SemaphoreType.DMA((SF + 3 * NFC + NTILE,)),
            ],
            compiler_params=pltpu.CompilerParams(vmem_limit_bytes=110 << 20, flags=FLAGS),
            name="hedgehog_mod",
        )(A_x, A_wqkv, A_w_phi, A_wo, B_w_r, B_w_gate, B_w_up, B_w_down)

    return run


_run = make(PROWS=128, PGAP=6, FPAT=(1,1,1,1,1,1,1,1,1,1,1,1,0,0))


@jax.jit
def pallas_recurrent_scan__linear_kernel_hedgehog__moe_arch_mod__prompt_kernel(
    A_x, A_wqkv, A_w_phi, A_wo, B_x, B_w_r, B_w_gate, B_w_up, B_w_down,
):
    return _run(A_x, A_wqkv, A_w_phi, A_wo, B_x, B_w_r, B_w_gate, B_w_up, B_w_down)
```

```python
import jax
import jax.numpy as jnp
from jax import lax
import jax.experimental.pallas as pl
import jax.experimental.pallas.tpu as pltpu

BF = jnp.bfloat16
F32 = jnp.float32
U32 = jnp.uint32
NN = (((1,), (0,)), ((), ()))
NT = (((1,), (1,)), ((), ()))
LOG2E = 1.4426950408889634

D, H, DH, FF = 1024, 32, 32, 3584
L = 128
HK = D // 2
KH = HK // L
NG = H // 4
NP = H // 2
TT = 4 * L
FC = 4 * L
NFC = FF // FC
NOP = 26
RAW = ((1, 26), (27, 2), (7, 8), (16, 28))
RAWL = ((26, 0), (3, 27), (7, 8), (28, 15))
STAGE = {k: i for i, k in enumerate(sum(RAWL, ()))}


NOTES = {}


def note(*k):
    NOTES[k] = NOTES.get(k, 0) + 1
    assert NOTES[k] < 999, k


def _dot(a, b, dims):
    return lax.dot_general(a, b, dims, preferred_element_type=F32)


def _unpack(w):
    return pltpu.bitcast(w, BF)


def _rnd(v):
    return v.astype(BF).astype(F32)


def _rcp(v):
    return pltpu.reciprocal(v, approx=True)


def _silu(v):
    h = 0.5 * v
    return h + h * jnp.tanh(h)


def _tree(v, op):
    while len(v) > 1:
        v = [op(v[i], v[i + 1]) for i in range(0, len(v), 2)]
    return v[0]


def _pair_reduce(v, op):
    r = _tree(v, op)
    r = op(r, pltpu.roll(r, 2, 0))
    return op(r, pltpu.roll(r, 4, 0))


def _dual_exp(p):
    v = [p[8 * i:8 * i + 8] for i in range(8)]
    mx = _pair_reduce(v, jnp.maximum)
    mn = _pair_reduce(v, jnp.minimum)
    ep = [jnp.exp2(a - mx) for a in v]
    en = [jnp.exp2(mn - a) for a in v]
    return ep, en, _pair_reduce(ep, jnp.add), _pair_reduce(en, jnp.add)


def _key_features(p):
    ep, en, sp, sn = _dual_exp(p)
    rp, rn = _rcp(sp), _rcp(sn)
    return jnp.concatenate([a * rp for a in ep] + [a * rn for a in en], axis=0).astype(BF)


def _query_features(p):
    ep, en, sp, sn = _dual_exp(p)
    ratio = sp * _rcp(sn)
    return jnp.concatenate(ep + [a * ratio for a in en], axis=0).astype(BF), sp


class _Signed:
    def __init__(self, sign, v):
        self.sign, self.v = sign, v

    def __neg__(self):
        return _Signed(-self.sign, self.v)

    def __add__(self, o):
        if self.sign == o.sign:
            return _Signed(self.sign, self.v + o.v)
        return _Signed(1, self.v - o.v if self.sign > 0 else o.v - self.v)

    def __sub__(self, o):
        return self + (-o)


def _nxt(k, d=1):
    return (k - 1 + d) % 3 + 1


def _operands(block, left):
    lo, hi = (1, 2) if left else (2, 1)

    def forms(i):
        x, y = block(i)
        if left:
            return {1: _Signed(1, x), 2: _Signed(-1, y), 3: _Signed(1, y - x)}
        return {1: _Signed(1, y), 2: _Signed(1, x), 3: _Signed(-1, x + y)}

    def diag(g, k):
        yield g[_nxt(k, lo)]
        yield g[_nxt(k, hi)]

    def pair(ga, gb, k, s):
        m = _nxt(k, 2)
        for n in (_nxt(m, lo), _nxt(m, hi)):
            s[n] = ga[n] + gb[n]
            yield s[n]
        yield gb[k] - ga[_nxt(k)] if left else ga[_nxt(k)] - gb[k]

    f0 = forms(0)
    yield from diag(f0, 1)
    f1 = forms(1)
    yield from diag(f1, 2)
    yield from pair(f0, f1, 1, {})
    f2 = forms(2)
    yield from diag(f2, 3)
    yield from pair(f1, f2, 2, {})
    s02 = {}
    yield from pair(f2, f0, 3, s02)
    s02[2] = f0[2] + f2[2]
    f3 = forms(3)
    yield from diag(f3, 1)
    yield from pair(f2, f3, 3, {})
    yield from pair(f3, s02, 1, {})
    yield from pair(f3, f1, 1, {})


_SIGNS = [a.sign * b.sign for a, b in zip(_operands(lambda i: (0, 0), True), _operands(lambda i: (0, 0), False))]


def _block_product(product, keep):
    count = iter(range(NOP))

    def m(sign=1):
        k = next(count)
        return _Signed(sign * _SIGNS[k], product(k))

    def park(slot, v):
        fetch = keep(slot, v.v)
        return lambda: _Signed(v.sign, fetch())

    def diag(slot):
        x = park(slot, m())
        y = m(-1)
        return (x, park(slot + 1, y)), x() + y

    def pair(da, db, slot=None):
        xs = m()
        ab = park(12, xs - da[1]() - db[1]())
        if slot:
            xs = park(slot, xs)
        ys = m(-1)
        ba = park(13, ys - da[0]() - db[0]())
        if slot:
            ys = park(slot + 1, ys)
        g = m()
        return ab() - g, ba() + g, (xs, ys)

    def steps():
        d0, c = diag(0)
        yield 0, 0, c
        d1, c = diag(2)
        yield 1, 1, c
        ab, ba, _ = pair(d0, d1)
        yield 0, 1, ab
        yield 1, 0, ba
        d2, c = diag(4)
        yield 2, 2, c
        ab, ba, _ = pair(d1, d2)
        yield 1, 2, ab
        yield 2, 1, ba
        ab, ba, d02 = pair(d2, d0, 8)
        yield 2, 0, ab
        yield 0, 2, ba
        d3, c = diag(6)
        yield 3, 3, c
        ab, ba, _ = pair(d2, d3)
        c23, c32 = park(10, ab), park(11, ba)
        yield 2, 3, ab
        yield 3, 2, ba
        ab, ba, _ = pair(d3, d02)
        yield 3, 0, ab - c32()
        yield 0, 3, ba - c23()
        ab, ba, _ = pair(d3, d1)
        yield 3, 1, ab
        yield 1, 3, ba

    for i, j, c in steps():
        assert c.sign > 0
        yield i, j, c.v


class _Tasks:
    def __init__(self):
        self.q = []

    def add(self, gen):
        self.q.append(gen)

    def step(self, n=1):
        while n > 0 and self.q:
            try:
                next(self.q[0])
                n -= 1
            except StopIteration:
                self.q.pop(0)

    def drain(self):
        while self.q:
            self.step()


def make(S=2048, PR=1, FROWS=128, FLAGS=None, PROF=0, MODE='', NOSIDE=0, LNP=(1, 1), LNG=2, PGAP=1, BGAP=1, FPAT=(1,), BROWS=16,
         TSTEP=1, PD0=1, PDA=2, PDB=1, APAT='LBPLLPLPPPLPLL.L.LLPL.LPLL', QPAT='BBBB.BBBBBBBBB.BBLBLBBBB.L', BPAT='PPPB.LLLPLLBBPPPLPLBPLLPP.LLLPLLLLLLPPLLPLLBLLLBLLLL',
         L0PAT='4', P0PAT='.99999977777777777777777777', W1AT=14, W1PAT='335', T0PAT='3P33PP3P33P3P3PP3PPPPP3PPP' 'BB63BB6B3BB6B6P3BB666BPBB3' '22LLL22LLL2LL222LLLL2L2LL2', DEPTH=4, WAT=1, B1PAT='PPPB.LLLPLLBBPPPLPLBPBPPPP',
         BEND='LPL.LPLLPPPBPPPBPPPBPPPBPP' 'LLLLLLLLLLLLLLLLLLLLLLLLLL' '..........................', TWICE=range(16, 66, 3), B0PAT='L.LLLL.LLLL.LLLL.LLLL.LLL.' 'LLL.LLLLLLBPBPBPBPBPBPBPBP', CUTS=(), CUTA=(), STATIC=0, WBAT=2, WAAT=16, HOLD=1, STASH=0, FPROBE=1, FSPLIT=3, OUTPIN=0, BPIN=0, STYLE=0, SKIP='', OAPIN=1, OAREL=1, HEAD=15, KVD=4, NDD=4):
    NTILE = S // TT
    STOP = 1 if MODE == 'P' else 0
    MODE = '' if STOP else MODE
    NSTASH = 32
    XR = S // 4
    SF = NTILE + 3 * NG + 4
    SO = SF + 3 * NFC
    XS = 0
    AKV = XS + (NOP + 3) * KH * XR
    AQ = AKV + NOP * KH * 4 * L
    BO = AQ + NOP * KH * 2 * L
    PRB = BO + NOP * 2 * HK
    END = PRB + 16
    NSUB = HK // FROWS
    NPART = (32 + 8 * NFC) * NSUB
    GU = S
    WD = GU + NFC * D
    WO = WD + FF
    ANCHOR = WO + D

    def kernel(x_hbm, wqkv_hbm, wphi_hbm, wo_hbm, wr_hbm, wg_hbm, wu_hbm, wd_hbm, out_hbm,
               wide, w_v, wphi_v, wr_v, fm_v, part, st, ar, stage, hold, feat, oa0, oa1, kvl, kv_acc, out_v, xb, hb, sems, split):

        def x_rows(row0, rows):
            return x_hbm.at[0, pl.ds(row0, rows)], wide.at[pl.ds(row0, rows)]

        def w_cols(c):
            return wqkv_hbm.at[:, pl.ds(c * L, L)], w_v.at[c]

        def kv_cols(gp):
            return [w_cols(o + g) for g in (2 * gp, 2 * gp + 1) for o in (NG, 2 * NG)]

        def ffn_chunk(c):
            cols = pl.ds(c * FC, FC)
            rows = pl.ds(GU + c * D, D)
            return [(wg_hbm.at[:, cols], wide.at[rows, pl.ds(0, FC)]),
                    (wu_hbm.at[:, cols], wide.at[rows, pl.ds(FC, FC)]),
                    (wd_hbm.at[cols], wide.at[pl.ds(WD + c * FC, FC)])]

        loads = {
            'x0': [(wr_hbm, wr_v), x_rows(0, 2 * L)],
            'x2': [(wphi_hbm.at[pl.ds(0, 8)], wphi_v.at[pl.ds(0, 8)]), x_rows(2 * L, 2 * L)],
            'wa': kv_cols(0)[:2],
            'wb': kv_cols(0)[2:],
            'w1': [(wphi_hbm.at[pl.ds(8, H - 8)], wphi_v.at[pl.ds(8, H - 8)])] + kv_cols(1),
            'w2': kv_cols(2),
            'x1': [x_rows(TT, TT)] + kv_cols(3),
            'wo': [x_rows(n * TT, TT) for n in range(2, NTILE)] + [(wo_hbm, wide.at[pl.ds(WO, D)])],
            'wq': [w_cols(g) for g in range(NG)] + [p for c in range(FSPLIT) for p in ffn_chunk(c)],
            'f': [p for c in range(FSPLIT, NFC) for p in ffn_chunk(c)],
        }
        if MODE:
            loads = {'x0': loads['x0']}

        def copies(name):
            return [pltpu.make_async_copy(src, dst, sems.at[list(loads).index(name)]) for src, dst in loads[name]]

        def out_copy(src0, dst0, rows, col0, cols):
            return pltpu.make_async_copy(out_v.at[pl.ds(src0, rows), pl.ds(col0, cols)],
                                         out_hbm.at[0, pl.ds(dst0, rows), pl.ds(col0, cols)], sems.at[0])

        for name in loads:
            for cp in copies(name):
                cp.start(priority=PR)

        def wait(name, cps=None):
            if name not in loads and (MODE or not cps):
                return
            if PROF:
                with jax.named_scope(name):
                    for cp in cps() if cps else copies(name):
                        cp.wait()
            else:
                for cp in cps() if cps else copies(name):
                    cp.wait()

        ar_w = ar.bitcast(U32)
        probes = set()
        ready = set()
        pending = []

        wait('x0')
        wr1 = wr_v[...].astype(F32).reshape(1, D)
        zero = pl.multiple_of(jnp.max(jnp.where(jnp.abs(wr1) < 0.0, pltpu.bitcast(wr1, jnp.int32), 0)), 16)
        never = zero > 0
        ar[pl.ds(PRB, 16), :] = jnp.zeros((16, L), BF)
        part[NPART] = jnp.zeros((8, L), F32)
        st[64] = jnp.zeros((16, L), F32)
        hold[14, pl.ds(0, 8), :] = jnp.zeros((8, L), F32)
        feat[NSTASH, pl.ds(0, 16), :] = jnp.zeros((16, L), BF)
        out_v[pl.ds(S, 16), pl.ds(0, 2 * L)] = jnp.zeros((16, 2 * L), BF)
        stage[32, pl.ds(0, 16), :] = jnp.zeros((16, L), BF)
        for oa in (oa0, oa1):
            oa[(NOP + 3) * KH, pl.ds(0, 16), :] = jnp.zeros((16, L), BF)

        def fold_matrices(groups):
            rr = lax.broadcasted_iota(jnp.int32, (L, DH), 0)
            ff = lax.broadcasted_iota(jnp.int32, (L, DH), 1)
            sel = jnp.where(((rr & 63) >> 1) == ff, 1.0, 0.0).astype(BF)
            r2 = lax.broadcasted_iota(jnp.int32, (L, L), 0)
            c2 = lax.broadcasted_iota(jnp.int32, (L, L), 1)
            own = ((r2 >> 6) * 2 + (r2 & 1)) == (c2 >> 5)
            for g in groups:
                a = wphi_v[4 * g:4 * g + 4].reshape(L, DH)
                fm_v[g] = jnp.where(own, _dot(sel, a, NT), 0.0).astype(BF)

        def put(row, v):
            probes.add('ar')
            ar[pl.ds(row, v.shape[0]), :] = v.astype(BF)

        def slabs(start, stride, k, row0, rows):
            return jnp.concatenate(
                [ar_w[pl.ds((start + s * stride) // 2 + k * (KH * stride // 2) + row0, rows // 2), :]
                 for s in range(KH)], axis=1)

        def folded(g, c, s):
            w = _unpack(w_v.bitcast(U32)[c, pl.ds(s * L // 2, L // 2), :])
            return _dot(_unpack(fm_v.bitcast(U32)[g]), w, NT) * (2.0 * LOG2E)

        def build(load, store, slots=range(NOP)):
            for r0 in range(0, L, 16):
                for k, v in enumerate(_operands(lambda i: [_unpack(load(k, r0)).astype(F32) for k in RAWL[i]], True)):
                    if k in slots and k not in STAGE:
                        store(k, r0, v.v)
                    if k == slots[-1]:
                        break
                yield

        def arena_build(row_of, slots=range(NOP)):
            return build(lambda k, r0: stage.bitcast(U32)[row_of(k)[1], pl.ds(r0 // 2, 8), :],
                         lambda k, r0, v: put(row_of(k)[0] + r0, v), slots)

        def put_plain(row_of, k, v):
            probes.add('stage')
            v = v.astype(BF)
            stage[row_of(k)[1]] = v
            if k < NOP:
                ar[pl.ds(row_of(k)[0], L), :] = v

        def kv_rows(gp, s):
            return lambda k: (AKV + ((k * KH + s) * 4 + gp) * L, 8 * s + STAGE.get(k, 0))

        def plain_kv(gp, s, which=(0, 1)):
            for i in which:
                g = 2 * gp + i
                for h in range(2):
                    put_plain(kv_rows(gp, s), RAWL[2 * i][h], folded(g, NG + g, h * KH + s))
                    put_plain(kv_rows(gp, s), RAWL[2 * i + 1][h], w_v[2 * NG + g, pl.ds(h * HK + s * L, L), :].T)

        def prep_kv(gp):
            for s in range(KH):
                plain_kv(gp, s)
                yield
                yield from arena_build(kv_rows(gp, s))

        def q_groups(gp):
            return (2 * gp, KH + 2 * gp, 2 * gp + 1, KH + 2 * gp + 1)

        def prep_q():
            for gp in range(2):
                for s in range(KH):
                    def row_of(k):
                        return AQ + ((k * KH + s) * 2 + gp) * L, 8 * s + STAGE.get(k, 0)
                    for i, g in enumerate(q_groups(gp)):
                        for h in range(2):
                            put_plain(row_of, RAWL[i][h], folded(g, g, h * KH + s))
                        if i % 2:
                            yield
                    yield from arena_build(row_of)
                ready.add(('q', gp))

        def prep_o():
            for c in range(2):
                for r0 in range(0, HK, 16):
                    blk = [wide[pl.ds(WO + h * HK + r0, 16), pl.ds(c * HK, HK)].astype(F32) for h in range(2)]
                    for k, v in enumerate(_operands(lambda j: [b[:, j * L:(j + 1) * L] for b in blk], False)):
                        put(BO + (k * 2 + c) * HK + r0, v.v)
                    yield

        wr = jnp.broadcast_to(wr1, (16, D))
        best = [jnp.full((16, 1), -jnp.inf, F32), jnp.zeros((16, 1), jnp.int32)]

        def row_mean(n, c, j):
            xf = wide[pl.ds(n * TT + j * L + c * 16, 16), :].astype(F32)
            mean = jnp.sum(xf, axis=1, keepdims=True) * (1.0 / D)
            probes.add('st')
            st[8 * c + 2 * j] = jnp.broadcast_to(mean, (16, L))

        def row_stats(n, c, j):
            r0 = n * TT + j * L + c * 16
            d = wide[pl.ds(r0, 16), :].astype(F32) - jnp.concatenate([st[8 * c + 2 * j]] * (D // L), axis=1)
            var = jnp.sum(d * d, axis=1, keepdims=True) * (1.0 / D)
            rs = _rcp(_rnd(jnp.sqrt(_rnd(_rnd(var) + 1e-5))))
            r = jnp.sum(d * wr, axis=1, keepdims=True) * rs
            up = (r > best[0]) | ((r == best[0]) & (r0 < best[1]))
            best[0] = jnp.where(up, r, best[0])
            best[1] = jnp.where(up, r0, best[1])
            probes.add('st')
            st[8 * c + 2 * j + 1] = jnp.broadcast_to(0.5 * rs, (16, L))

        def token_operands(n, c, s):
            row = XS + s * XR + n * L + c * 16

            def block(j):
                b = [(wide[pl.ds(n * TT + j * L + c * 16, 16), pl.ds(h * HK + s * L, L)].astype(F32)
                      - st[8 * c + 2 * j]) * st[8 * c + 2 * j + 1] for h in range(2)]
                for k, v in zip(RAW[j], b):
                    if k >= NOP:
                        put(row + k * KH * XR, v)
                return b

            for k, v in enumerate(_operands(block, False)):
                put(row + k * KH * XR, v.v)
            return v.v

        def layernorm(n):
            for j in range(4):
                row_mean(n, 0, j)
            yield
            for c in range(L // 16):
                for j in range(4):
                    row_stats(n, c, j)
                    if j % 2:
                        yield
                if c + 1 < L // 16:
                    for j in range(4):
                        row_mean(n, c + 1, j)
                    yield
                for s in range(KH):
                    token_operands(n, c, s)
                    yield

        side = _Tasks()
        prep = _Tasks()
        tail = _Tasks()
        tail2 = _Tasks()
        count = [0]
        origin = [0]
        twice = set()
        delay = [PD0]
        flush = []
        timed = {}

        def soon(action):
            timed.setdefault(count[0] + WAT, []).append(action)

        release = [stage.at[32]]
        plan = [APAT]

        def tie(end):
            due = pending.pop(0) if len(pending) > delay[0] else ()
            for name in sorted(due):
                if name == 'ar':
                    seen = ar_w[pl.ds(PRB // 2 + zero, 8), :]
                elif name == 'part':
                    seen = pltpu.bitcast(part[NPART + zero], U32)
                elif name == 'st':
                    seen = pltpu.bitcast(st[64, pl.ds(zero, 8), :], U32)
                elif name == 'hold':
                    seen = pltpu.bitcast(hold[14, pl.ds(zero, 8), :], U32)
                elif name == 'feat':
                    seen = feat.bitcast(U32)[NSTASH, pl.ds(zero, 8), :]
                elif name == 'stage':
                    seen = stage.bitcast(U32)[32, pl.ds(zero, 8), :]
                elif name == 'out':
                    seen = pltpu.bitcast(out_v[pl.ds(S + zero, 16), pl.ds(0, L)], U32)
                else:
                    seen = (oa0, oa1)[name == 'oa1'].bitcast(U32)[(NOP + 3) * KH, pl.ds(zero, 8), :]
                end = jnp.where(never, seen, end)
            return end

        def gate(words):
            if STYLE != 1:
                return words
            last_rows = jnp.concatenate([tie(words[-8:, :L]), words[-8:, L:]], axis=1)
            return jnp.concatenate([words[:-8], last_rows], axis=0)

        def gap(m):
            count[0] += 1
            for action in timed.pop(count[0], ()):
                action()
            if STYLE == 0:
                h = 8 * HEAD
                tied = pltpu.bitcast(tie(pltpu.bitcast(m[h:h + 8], U32)), F32)
                m = jnp.concatenate([v for v in (m[:h], tied, m[h + 8:]) if v.shape[0]], axis=0)
            if STYLE == 2:
                m8 = pltpu.bitcast(tie(pltpu.bitcast(m[:8], U32)), F32)
                wide[pl.ds(ANCHOR + zero, 8), pl.ds(0, 2 * L)] = jnp.concatenate([m8, m[8:16]], axis=1).astype(BF)
            elif side.q or prep.q or (OUTPIN and tail2.q):
                wide[pl.ds(ANCHOR + zero, 8), pl.ds(0, 2 * L)] = jnp.concatenate([m[:8], m[8:16]], axis=1).astype(BF)
            if prep.q and release:
                release[0][pl.ds(zero + 16, 16), :] = m[:16].astype(BF)
            tail.step(2 if count[0] in twice else 1)
            tail2.step()
            todo = plan[0][(count[0] - origin[0] - 1) % len(plan[0])]
            side.step({'L': 1, 'B': 1, '2': 2, '6': 1}.get(todo, 0))
            prep.step({'P': 1, 'B': 1, '3': 2, '6': 2, '5': 3, '7': 4, '9': 8}.get(todo, 0))
            pending.append(set(probes))
            probes.clear()
            return m

        def cut():
            pl.semaphore_signal(split, 1)
            pl.semaphore_wait(split, 1)

        def after(gaps, gen):
            start = count[0] + gaps

            def held():
                while count[0] < start and not flush:
                    yield
                yield from gen
            return held()

        turn = [0]

        def stash(v):
            if not STASH:
                return lambda: v
            slot = turn[0] % NSTASH
            turn[0] += 1
            probes.add('feat')
            feat[slot, pl.ds(0, v.shape[0]), :] = v
            return lambda: _unpack(feat.bitcast(U32)[slot, pl.ds(0, v.shape[0] // 2), :])

        def unit(lhs, rhs, dims, on_block):
            def keep(slot, v):
                if HOLD == 0 or (HOLD == 1 and slot < 12):
                    return lambda: v
                probes.add('hold')
                hold[slot] = v
                return lambda: hold[slot]

            for i, j, c in _block_product(lambda k: gap(_dot(_unpack(gate(lhs(k))), _unpack(rhs(k)), dims)), keep):
                on_block(i, j, c)

        def drain_tail():
            flush.append(1)
            tail.drain()
            flush.clear()

        route = {}

        def router():
            rmax = jnp.max(best[0])
            pos = best[1] + lax.broadcasted_iota(jnp.int32, (16, 1), 0)
            idx = jnp.min(jnp.where(best[0] == rmax, pos, S - 1))
            last = idx // TT
            blk = (idx // L) % 4
            row0 = pl.multiple_of((last * L + ((idx % L) // 16) * 16) // 2, 8)
            hit = lax.broadcasted_iota(jnp.int32, (16, HK), 0) == idx % 16
            route.update(rmax=rmax, idx=idx, last=last)
            for h in range(2):
                k = sum(jnp.where(blk == j, RAW[j][h], 0) for j in range(4))
                rows = _unpack(slabs(XS, XR, k, row0, 16)).astype(F32)
                row = 2.0 * jnp.sum(jnp.where(hit, rows, 0.0), axis=0, keepdims=True)
                for s in range(KH):
                    xb[pl.ds(h * HK + s * L, L), :] = jnp.broadcast_to(row[:, s * L:(s + 1) * L], (L, L)).T
                    yield

        def kv_unit(gp, n):
            seen, acc = {}, {}

            def combine(g, phis, vts):
                for pp in range(2):
                    upd = _dot(vts[pp](), phis[pp](), NT)
                    p = 2 * g + pp
                    acc[p] = acc.get(p, ()) + (upd,)
                    if len(acc[p]) == 4:
                        upd = _tree(list(acc[p]), jnp.add)
                        kv_acc[p] = upd if n == 0 else kv_acc[p] + upd
                    yield

            def on_block(i, j, c):
                g = 2 * gp + i // 2
                if i % 2:
                    seen[i, j] = [stash(jnp.concatenate([c[pp * 64:(pp + 1) * 64], jnp.ones((16, L), F32)],
                                                        axis=0).astype(BF)) for pp in range(2)]
                else:
                    seen[i, j] = [stash(_key_features(c[pp * 64:(pp + 1) * 64])) for pp in range(2)]
                if (i ^ 1, j) in seen:
                    tail.add(after(KVD, combine(g, seen[i & 2, j], seen[i | 1, j])))

            def weights(k):
                while not MODE and (gp, n) == (0, 0) and k in (7, 15) and k not in ready:
                    assert count[0] >= WBAT
                    prep.step()
                    note('first forced', k)
                return slabs(AKV, 4 * L, k, gp * L // 2, L)

            unit(weights,
                 lambda k: slabs(XS, XR, k, n * L // 2, L), NT, on_block)

        def first_layernorm():
            def fence():
                wide[pl.ds(ANCHOR + zero, 8), pl.ds(0, 2 * L)] = jnp.zeros((8, 2 * L), BF)

            for j0 in (0, 2):
                if j0:
                    wait('x2')
                    fold_matrices(range(2))
                for part_of in (row_mean, row_stats):
                    for c in range(L // 16):
                        for j in (j0, j0 + 1):
                            part_of(0, c, j)
                    fence()
            done = []
            for c in range(L // 16):
                for s in range(KH):
                    if len(done) == WAAT:
                        wait('wa')
                        for t in range(KH):
                            plain_kv(0, t, (0,))
                            prep.add(arena_build(kv_rows(0, t), range(7)))
                    if len(done) >= DEPTH:
                        v = done[-DEPTH]
                        wide[pl.ds(ANCHOR + zero, 8), pl.ds(0, 2 * L)] = jnp.concatenate([v, v], axis=1).astype(BF)
                    token_operands(0, c, s)
                    prep.step(2)
                    done.append(pltpu.bitcast(ar_w[pl.ds(PRB // 2 + zero, 8), :], F32))

        def more_weights():
            while count[0] < WBAT:
                yield
            wait('wb')
            for s in range(KH):
                plain_kv(0, s, (1,))
                yield
            for slots in (range(7, 15), range(15, NOP)):
                for s in range(KH):
                    yield from arena_build(kv_rows(0, s), slots)
                ready.add(slots[0])
            while count[0] < W1AT:
                yield
            wait('w1')
            fold_matrices(range(2, NG))
            plan[0] = W1PAT
            yield from prep_kv(1)

        ffn_out = []
        fcount = [0]

        def matvec(row0, col0, vec, k0, slot):
            acc = [[None, None], [None, None]]
            for k in range(k0, k0 + FROWS, 8):
                vk = vec[pl.ds(k, 8), :]
                wk = wide[pl.ds(row0 + k, 8), pl.ds(col0, 2 * L)].astype(F32)
                for t in range(2):
                    pr = wk[:, t * L:(t + 1) * L] * vk
                    a = acc[t][(k // 8) % 2]
                    acc[t][(k // 8) % 2] = pr if a is None else a + pr
            fcount[0] += 1
            if fcount[0] % FPROBE == 0:
                probes.add('part')
            for t in range(2):
                part[slot(t)] = acc[t][0] + acc[t][1]

        def total(slots):
            return _tree([part[s] for s in slots], jnp.add)

        def ffn():
            def gu_slot(c, t, p):
                return ((c % 2) * 8 + t) * 2 * NSUB + p

            def y_slot(c, t, p):
                return 32 * NSUB + (t * NFC + c) * NSUB + p

            def down(c, half):
                for t in (4 * half, 4 * half + 2):
                    for p in range(NSUB):
                        matvec(WD + c * FC, t * L, hb.at[c], p * FROWS, lambda u: y_slot(c, t + u, p))
                        yield

            def result(half):
                gate = 0.5 / (1.0 + jnp.exp(-jnp.full((8, L), route['rmax'], F32)))
                for t in range(4 * half, 4 * half + 4):
                    yt = sum(total([y_slot(c, t, p) for p in range(NSUB)]) for c in range(NFC))
                    ffn_out.append(jnp.broadcast_to(jnp.sum(yt, axis=0, keepdims=True), (8, L)) * gate)

            for c in range(NFC):
                while c == FSPLIT and not late_weights:
                    yield
                for t in range(0, 8, 2):
                    for p in range(2 * NSUB):
                        matvec(GU + c * D, t * L, xb, p * FROWS, lambda u: gu_slot(c, t + u, p))
                        yield
                for t in range(4):
                    gt = jnp.sum(total([gu_slot(c, t, p) for p in range(2 * NSUB)]), axis=0, keepdims=True)
                    ut = jnp.sum(total([gu_slot(c, 4 + t, p) for p in range(2 * NSUB)]), axis=0, keepdims=True)
                    hb[c, pl.ds(t * L, L), :] = jnp.broadcast_to(_silu(gt) * ut, (L, L)).T
                yield
                if c > 0:
                    yield from down(c - 1, 0)
            yield from down(0, 1)
            yield from down(NFC - 1, 0)
            result(0)
            note('ffn half at', count[0])
            yield
            for c in range(1, NFC):
                yield from down(c, 1)
            result(1)
            note('ffn done at', count[0])

        def start_side_work(n, gp):
            if n == 0 and gp == 1:
                wait('w2')
                prep.add(prep_kv(2))
                plan[0] = '.' * NOP + T0PAT
            elif n == 0 and gp == 2:
                wait('x1')
                prep.add(prep_kv(3))
                side.add(layernorm(1))
            elif n > 0 and gp == 0:
                plan[0] = APAT
                delay[0] = PDA
                if n == 1:
                    wait('wo')
                    prep.add(prep_o())
                if n + 1 < NTILE:
                    side.add(layernorm(n + 1))
                else:
                    wait('wq')
                    plan[0] = QPAT
                    side.add(router())
                    side.add(ffn())
                    prep.add(prep_q())

        late_weights = []
        if not MODE:
            first_layernorm()
            prep.drain()
            prep.add(more_weights())
            plan[0] = P0PAT
        for n in range({'': NTILE, 'A': NTILE - 1, 'B': 0}[MODE]):
            for gp in range(4):
                if MODE:
                    if gp == 0 and NOSIDE != 1:
                        side.drain()
                        if NOSIDE != 5:
                            side.add(layernorm(n + 1))
                        if n == 0 and NOSIDE == 4:
                            prep.add(prep_o())
                        if NOSIDE == 5:
                            prep.drain()
                            plan[0] = QPAT
                            side.add(ffn())
                            prep.add(prep_q())
                else:
                    while n == 0 and gp and prep.q:
                        prep.step()
                        note('prep_kv forced', gp)
                    while n and not gp and side.q:
                        side.step()
                        note('layernorm forced', n)
                    soon(lambda n=n, gp=gp: start_side_work(n, gp))
                    if (n, gp) in CUTA:
                        soon(cut)
                kv_unit(gp, n)
            if STOP:
                drain_tail()
                side.drain()
                seen = ar[pl.ds(PRB + zero, 16), :]
                out_v[pl.ds(0, 16), pl.ds(0, L)] = (seen.astype(F32) + best[0] + best[1]).astype(BF)
                return
        if MODE == 'A':
            if NOSIDE != 5:
                side.drain()
            else:
                prep.drain()
            drain_tail()
            out_v[pl.ds(0, 16), pl.ds(0, 1)] = (best[0] + best[1]).astype(BF)
            return
        if MODE == 'B':
            route.update(rmax=jnp.max(wr1), idx=zero, last=zero >> 4)
        rmax, idx, last = route['rmax'], route['idx'], route['last']

        def finish_kv():
            r3 = lax.broadcasted_iota(jnp.int32, (80, L), 0)
            c3 = lax.broadcasted_iota(jnp.int32, (80, L), 1)
            keep = jnp.where(r3 < 64, r3 >> 5, r3 & 1) == (c3 & 1)
            double = jnp.where(r3 < 64, 2.0, 1.0)
            for p in range(NP):
                kvl[p] = jnp.where(keep, kv_acc[p] * double, 0.0).astype(BF)
            yield

        if not MODE:
            tail.add(finish_kv())

        def tile_of(n):
            return n if STATIC else (last + 1 + n) % NTILE

        built, started = {}, set()

        def mult(v, m):
            return v if isinstance(v, int) else pl.multiple_of(v, m)

        def operands(n, gp):
            oa = (oa0, oa1)[n % 2]
            release[:] = [oa.at[(NOP + 3) * KH]] if OAREL else []
            for slab in (2 * gp, 2 * gp + 1):
                def store(k, r0, v):
                    if OAPIN:
                        probes.add(f'oa{n % 2}')
                    oa[k * KH + slab, pl.ds(r0, 16), :] = v.astype(BF)
                yield from build(lambda k, r0: oa.bitcast(U32)[k * KH + slab, pl.ds(r0 // 2, 8), :], store)
            built[n] = built.get(n, 0) + 1

        def token_words(n):
            return ar_w.at[pl.ds(mult(tile_of(n) * (L // 2), L // 2), ((NOP + 3) * KH * XR - XR + L) // 2)]

        def q_unit(gp, n):
            started.add(n)
            while not MODE and ('q', gp) not in ready:
                prep.step()
                note('prep_q forced', gp)
            left = [16]
            oa = (oa0, oa1)[n % 2]

            def attend(i, j, feats):
                p0 = 2 * q_groups(gp)[i]
                rows_out = []
                for pp, (phi, scale) in enumerate(feats):
                    nd = _dot(_unpack(kvl.bitcast(U32)[p0 + pp]), phi(), NN)
                    inv = _rcp(nd[64:72] + 1e-6 * scale)
                    for jj in range(2):
                        rd = jnp.broadcast_to(inv[jj:jj + 1], (8, L))
                        rows_out += [nd[jj * DH + 8 * q:jj * DH + 8 * q + 8] * rd for q in range(4)]
                    if pp == 0:
                        yield
                oa[RAWL[j][i % 2] * KH + 2 * gp + i // 2] = jnp.concatenate(rows_out, axis=0).T.astype(BF)
                left[0] -= 1
                if not left[0] and 'b' not in SKIP:
                    prep.add(operands(n, gp))
                yield

            def on_block(i, j, c):
                feats = [_query_features(c[pp * 64:(pp + 1) * 64]) for pp in range(2)]
                tail.add(after(NDD, attend(i, j, [(stash(phi), scale) for phi, scale in feats])))

            tokens = token_words(n)
            unit(lambda k: slabs(AQ, 2 * L, k, gp * L // 2, L),
                 lambda k: jnp.concatenate([tokens[pl.ds((k * KH + s) * XR // 2, L // 2), :] for s in range(KH)], axis=1),
                 NT, on_block)

        def o_unit(c, n):
            t = tile_of(n)
            tokens = token_words(n)
            x_tile = wide.at[pl.ds(mult(t * TT, TT), TT)]
            left = [16]

            def finish(j, col, s):
                cols = pl.ds(c * HK + col * L, L)
                xn = _unpack(tokens[pl.ds((RAW[j][c] * KH + col) * XR // 2, L // 2), :]).astype(F32)
                if n == NTILE - 1:
                    rid = lax.broadcasted_iota(jnp.int32, (L, L), 0) + j * L
                    yv = jnp.concatenate([ffn_out[c * KH + col]] * (L // 8), axis=0)
                    xn = xn + jnp.where(rid == idx % TT, yv, 0.0)
                if OUTPIN:
                    probes.add('out')
                sh = s * xn
                out_v[pl.ds(n * TT + j * L, L), cols] = (x_tile[pl.ds(j * L, L), cols].astype(F32) + sh + sh * jnp.tanh(xn)).astype(BF)
                left[0] -= 1
                if (n, c) == (NTILE - 1, 1):
                    out_copy(n * TT + j * L, mult(t * TT + j * L, L), L, cols.start, L).start()
                elif not left[0]:
                    out_copy(n * TT, mult(t * TT, TT), TT, c * HK, HK).start()
                yield

            def dummy(j, col, s):
                out_v[pl.ds(j * L, L), pl.ds(col * L, L)] = s.astype(BF)
                left[0] -= 1
                if not left[0]:
                    out_copy(n * TT, mult(t * TT, TT), TT, c * HK, HK).start()
                yield

            while n == NTILE - 1 and len(ffn_out) < 4 * (c + 1):
                side.step()
                note('ffn forced', c)
            if c == 0:
                if n == NTILE - 1:
                    drain_tail()
                while built.get(n, 0) < 2 and 'b' not in SKIP and n in started:
                    (prep if prep.q else tail).step()
                    note('build forced', n)
            oa = (oa0, oa1)[n % 2].bitcast(U32)
            unit(lambda k: jnp.concatenate([oa[k * KH + s] for s in range(KH)], axis=1),
                 lambda k: ar_w[pl.ds((BO + (k * 2 + c) * HK) // 2, HK // 2), :], NN,
                 lambda j, col, s: tail2.add(finish(j, col, s)) if 'f' not in SKIP else tail2.add(dummy(j, col, s)))

        if MODE and not NOSIDE:
            side.add(ffn())
            late_weights.append(1)
            prep.add(after(10, operands(0, 1)))
        twice.update(count[0] + t for t in TWICE)
        plan[0] = BPAT if MODE else B0PAT + B1PAT + BPAT[NOP:] + BPAT * 4 + BPAT[:NOP] + BEND
        delay[0] = PDB
        origin[0] = count[0]
        if MODE != 'B':
            q_unit(0, 0)
            soon(lambda: wait('f'))
            soon(lambda: late_weights.append(1))
            q_unit(1, 0)
        for n in range(1, NTILE - (MODE == 'B')):
            for gp in range(2):
                if (n, gp) in CUTS:
                    soon(cut)
                q_unit(gp, n)
                o_unit(gp, n - 1)
        if MODE != 'B':
            for c in range(2):
                if (NTILE, c) in CUTS:
                    soon(cut)
                o_unit(c, NTILE - 1)
        drain_tail()
        tail2.drain()
        prep.drain()
        wait('out', lambda: [out_copy(0, 0, TT, 0, HK) for k in range(2 * NTILE - 1)]
             + [out_copy(0, 0, L, 0, L) for k in range(16)])

    @jax.jit
    def run(A_x, A_wqkv, A_w_phi, A_wo, B_x, B_w_r, B_w_gate, B_w_up, B_w_down):
        any_spec = pl.BlockSpec(memory_space=pl.ANY)
        return pl.pallas_call(
            kernel,
            out_shape=jax.ShapeDtypeStruct(A_x.shape, A_x.dtype),
            in_specs=[any_spec] * 8,
            out_specs=any_spec,
            scratch_shapes=[
                pltpu.VMEM((ANCHOR + 8, D), BF),
                pltpu.VMEM((3 * NG, D, L), BF),
                pltpu.VMEM((H, DH, DH), BF),
                pltpu.VMEM((D,), BF),
                pltpu.VMEM((NG, L, L), BF),
                pltpu.VMEM((NPART + 1, 8, L), F32),
                pltpu.VMEM((65, 16, L), F32),
                pltpu.VMEM((END, L), BF),
                pltpu.VMEM((33, L, L), BF),
                pltpu.VMEM((15, L, L), F32),
                pltpu.VMEM((NSTASH + 1, L, L), BF),
                pltpu.VMEM(((NOP + 3) * KH + 1, L, L), BF),
                pltpu.VMEM(((NOP + 3) * KH + 1, L, L), BF),
                pltpu.VMEM((NP, 80, L), BF),
                pltpu.VMEM((NP, 80, L), F32),
                pltpu.VMEM((S + 16, D), BF),
                pltpu.VMEM((D, L), F32),
                pltpu.VMEM((NFC, FC, L), F32),
                pltpu.SemaphoreType.DMA((10,)),
                pltpu.SemaphoreType.REGULAR,
            ],
            compiler_params=pltpu.CompilerParams(vmem_limit_bytes=120 << 20, flags=FLAGS),
            name="hedgehog_mod",
        )(A_x, A_wqkv, A_w_phi, A_wo, B_w_r, B_w_gate, B_w_up, B_w_down)

    return run


_run = make()


@jax.jit
def pallas_recurrent_scan__linear_kernel_hedgehog__moe_arch_mod__prompt_kernel(
    A_x, A_wqkv, A_w_phi, A_wo, B_x, B_w_r, B_w_gate, B_w_up, B_w_down,
):
    return _run(A_x, A_wqkv, A_w_phi, A_wo, B_x, B_w_r, B_w_gate, B_w_up, B_w_down)
```

```python
import jax
import jax.numpy as jnp
from jax import lax
import jax.experimental.pallas as pl
import jax.experimental.pallas.tpu as pltpu

BF = jnp.bfloat16
F32 = jnp.float32
U32 = jnp.uint32
NN = (((1,), (0,)), ((), ()))
NT = (((1,), (1,)), ((), ()))
LOG2E = 1.4426950408889634

S, D, H, DH, FF = 2048, 1024, 32, 32, 3584
L = 128
HK = D // 2
KH = HK // L
NG = H // 4
NP = H // 2
TT = 4 * L
NTILE = S // TT
FC = 4 * L
NFC = FF // FC
FROWS = 128
NSUB = HK // FROWS
EARLY = 3
NOP = 26
RAW = ((1, 26), (27, 2), (7, 8), (16, 28))
RAWL = ((26, 0), (3, 27), (7, 8), (28, 15))
STAGE = {k: i for i, k in enumerate(sum(RAWL, ()))}

XR = S // 4
XS = 16
AKV = XS + (NOP + 3) * KH * XR
AQ = AKV + NOP * KH * 4 * L
BO = AQ + NOP * KH * 2 * L
SPARE = BO + NOP * 2 * HK
GU = S
WD = GU + NFC * D
WO = WD + FF
ANCHOR = WO + D
NPART = (32 + 8 * NFC) * NSUB
OSPARE = (NOP + 3) * KH

PIECES = {'.': (0, 0), 'L': (1, 0), '2': (2, 0), 'P': (0, 1), '3': (0, 2), '5': (0, 3), '9': (0, 8),
          'B': (1, 1), '6': (1, 2)}
FIRST_PLAN = '.935555555533355535535533P'
TILE0_PLAN = '.' * NOP + 'PP33PP3P33P333PP3PPPPP3PPP' '3B63BB6BBBB6B6P3BBB666PBB3' '2L2LLL22L22LL222LLLL2LLL2L'
NORM_PLAN = 'PBPLLPLPPPLLLL.L.LBLL.LL.P'
QUERY_PLAN = 'LBBBBBLBBBBB.BBBBBBBBBBLP.'
Q_PLAN, O_PLAN = 'PLB..LLLPLPBPLPLBPBLPLLLP.', 'LBBPLLLLPBPPLLPLLBLLLLLLL.'
OUT_PLAN = ('L.LLLL.LLLL.LLLL.LLLL.LLL.' 'LLL.LLLLLLBPBPBPBPBPBPBPBP' 'PLB..LLLPLPBPLPLBPBPPPBPPP'
            + O_PLAN + (Q_PLAN + O_PLAN) * 4 + Q_PLAN + 'LBBPLLLLPBBPPBPPBPPBPPBPPP' + 'L' * NOP + '.' * NOP)


def _dot(a, b, dims):
    return lax.dot_general(a, b, dims, preferred_element_type=F32)


def _unpack(words):
    return pltpu.bitcast(words, BF)


def _rnd(v):
    return v.astype(BF).astype(F32)


def _rcp(v):
    return pltpu.reciprocal(v, approx=True)


def _silu(v):
    h = 0.5 * v
    return h + h * jnp.tanh(h)


def _total(v):
    while len(v) > 1:
        v = [v[i] + v[i + 1] for i in range(0, len(v), 2)]
    return v[0]


def _pair_reduce(v, reduce, op):
    r = reduce(v, axis=0)
    r = op(r, pltpu.roll(r, 2, 0))
    return op(r, pltpu.roll(r, 4, 0))


def _dual_exp(p):
    v = p.reshape(8, 8, L)
    ep = jnp.exp2(v - _pair_reduce(v, jnp.max, jnp.maximum))
    en = jnp.exp2(_pair_reduce(v, jnp.min, jnp.minimum) - v)
    return ep, en, _pair_reduce(ep, jnp.sum, jnp.add), _pair_reduce(en, jnp.sum, jnp.add)


def _key_features(p):
    ep, en, sp, sn = _dual_exp(p)
    return jnp.concatenate([ep * _rcp(sp), en * _rcp(sn)], axis=0).reshape(L, L).astype(BF)


def _query_features(p):
    ep, en, sp, sn = _dual_exp(p)
    return jnp.concatenate([ep, en * (sp * _rcp(sn))], axis=0).reshape(L, L).astype(BF), sp


class _Signed:
    def __init__(self, sign, v):
        self.sign, self.v = sign, v

    def __neg__(self):
        return _Signed(-self.sign, self.v)

    def __add__(self, o):
        if self.sign == o.sign:
            return _Signed(self.sign, self.v + o.v)
        return _Signed(1, self.v - o.v if self.sign > 0 else o.v - self.v)

    def __sub__(self, o):
        return self + (-o)


def _nxt(k, d=1):
    return (k - 1 + d) % 3 + 1


def _operands(block, left):
    lo, hi = (1, 2) if left else (2, 1)

    def forms(i):
        x, y = block(i)
        if left:
            return {1: _Signed(1, x), 2: _Signed(-1, y), 3: _Signed(1, y - x)}
        return {1: _Signed(1, y), 2: _Signed(1, x), 3: _Signed(-1, x + y)}

    def diag(g, k):
        yield g[_nxt(k, lo)]
        yield g[_nxt(k, hi)]

    def pair(ga, gb, k, s):
        m = _nxt(k, 2)
        yield gb[k] - ga[_nxt(k)] if left else ga[_nxt(k)] - gb[k]
        for n in (_nxt(m, lo), _nxt(m, hi)):
            s[n] = ga[n] + gb[n]
            yield s[n]

    f0 = forms(0)
    yield from diag(f0, 1)
    f1 = forms(1)
    yield from diag(f1, 2)
    yield from pair(f0, f1, 1, {})
    f2 = forms(2)
    yield from diag(f2, 3)
    yield from pair(f1, f2, 2, {})
    s02 = {}
    yield from pair(f2, f0, 3, s02)
    s02[2] = f0[2] + f2[2]
    f3 = forms(3)
    yield from diag(f3, 1)
    yield from pair(f2, f3, 3, {})
    yield from pair(f3, s02, 1, {})
    yield from pair(f3, f1, 1, {})


_SIGNS = [a.sign * b.sign for a, b in zip(_operands(lambda i: (0, 0), True), _operands(lambda i: (0, 0), False))]


def _block_product(product):
    count = iter(range(NOP))

    def m(sign=1):
        k = next(count)
        return _Signed(sign * _SIGNS[k], product(k))

    def diag(i):
        x, y = m(), m(-1)
        yield i, i, x + y
        return x, y

    def pair(a, b, da, db, less=(None, None)):
        g = m()
        xs = m()
        ab = xs - da[1] - db[1] - g
        yield a, b, ab if less[0] is None else ab - less[0]
        ys = m(-1)
        ba = ys - da[0] - db[0] + g
        yield b, a, ba if less[1] is None else ba - less[1]
        return (xs, ys), (ab, ba)

    def steps():
        d0 = yield from diag(0)
        d1 = yield from diag(1)
        yield from pair(0, 1, d0, d1)
        d2 = yield from diag(2)
        yield from pair(1, 2, d1, d2)
        d02, _ = yield from pair(2, 0, d2, d0)
        d3 = yield from diag(3)
        _, (c23, c32) = yield from pair(2, 3, d2, d3)
        yield from pair(3, 0, d3, d02, (c32, c23))
        yield from pair(3, 1, d3, d1)

    for i, j, c in steps():
        assert c.sign > 0
        yield i, j, c.v


class _Tasks:
    def __init__(self):
        self.q = []

    def add(self, gen):
        self.q.append(gen)

    def step(self, n=1):
        while n > 0 and self.q:
            try:
                next(self.q[0])
                n -= 1
            except StopIteration:
                self.q.pop(0)

    def drain(self):
        while self.q:
            self.step()


def _kernel(x_hbm, wqkv_hbm, wphi_hbm, wo_hbm, wr_hbm, wg_hbm, wu_hbm, wd_hbm, out_hbm,
            wide, w_v, wphi_v, wr_v, fm_v, part, st, ar, stage, oa0, oa1, kvl, kv_acc, out_v, xb, hb, sems):

    def x_rows(row0, rows):
        return x_hbm.at[0, pl.ds(row0, rows)], wide.at[pl.ds(row0, rows)]

    def w_cols(c):
        return wqkv_hbm.at[:, pl.ds(c * L, L)], w_v.at[c]

    def kv_cols(gp):
        return [w_cols(o + g) for g in (2 * gp, 2 * gp + 1) for o in (NG, 2 * NG)]

    def phi_heads(h0, heads):
        return wphi_hbm.at[pl.ds(h0, heads)], wphi_v.at[pl.ds(h0, heads)]

    def ffn_chunk(c):
        cols = pl.ds(c * FC, FC)
        rows = pl.ds(GU + c * D, D)
        return [(wg_hbm.at[:, cols], wide.at[rows, pl.ds(0, FC)]),
                (wu_hbm.at[:, cols], wide.at[rows, pl.ds(FC, FC)]),
                (wd_hbm.at[cols], wide.at[pl.ds(WD + c * FC, FC)])]

    loads = {
        'x00': [(wr_hbm, wr_v), x_rows(0, L)],
        'x01': [x_rows(L, L)],
        'x02': [x_rows(2 * L, L)],
        'x03': [x_rows(3 * L, L)],
        'kv0a': [phi_heads(0, 8)] + kv_cols(0)[:2],
        'kv0b': kv_cols(0)[2:],
        'kv1': [phi_heads(8, H - 8)] + kv_cols(1),
        'kv2': kv_cols(2),
        'kv3': [x_rows(TT, TT)] + kv_cols(3),
        'wo': [x_rows(n * TT, TT) for n in range(2, NTILE)] + [(wo_hbm, wide.at[pl.ds(WO, D)])],
        'wq': [w_cols(g) for g in range(NG)] + [p for c in range(EARLY) for p in ffn_chunk(c)],
        'ffn': [p for c in range(EARLY, NFC) for p in ffn_chunk(c)],
    }

    def copies(name):
        return [pltpu.make_async_copy(src, dst, sems.at[list(loads).index(name)]) for src, dst in loads[name]]

    def wait(name):
        for cp in copies(name):
            cp.wait()

    def out_copy(src0, dst0, rows, col0, cols):
        return pltpu.make_async_copy(out_v.at[pl.ds(src0, rows), pl.ds(col0, cols)],
                                     out_hbm.at[0, pl.ds(dst0, rows), pl.ds(col0, cols)], sems.at[0])

    for name in loads:
        for cp in copies(name):
            cp.start(priority=1)

    ar_w = ar.bitcast(U32)
    stored = set()
    ready = set()

    wait('x00')
    wr1 = wr_v[...].astype(F32).reshape(1, D)
    zero = pl.multiple_of(jnp.max(jnp.where(jnp.abs(wr1) < 0.0, pltpu.bitcast(wr1, jnp.int32), 0)), 16)
    never = zero > 0
    ar[pl.ds(SPARE, 16), :] = jnp.zeros((16, L), BF)
    part[NPART] = jnp.zeros((8, L), F32)
    st[64] = jnp.zeros((16, L), F32)
    stage[32, pl.ds(0, 16), :] = jnp.zeros((16, L), BF)
    for oa in (oa0, oa1):
        oa[OSPARE, pl.ds(0, 16), :] = jnp.zeros((16, L), BF)

    def fold_matrices(groups):
        rr = lax.broadcasted_iota(jnp.int32, (L, DH), 0)
        ff = lax.broadcasted_iota(jnp.int32, (L, DH), 1)
        sel = jnp.where(((rr & 63) >> 1) == ff, 1.0, 0.0).astype(BF)
        r2 = lax.broadcasted_iota(jnp.int32, (L, L), 0)
        c2 = lax.broadcasted_iota(jnp.int32, (L, L), 1)
        own = ((r2 >> 6) * 2 + (r2 & 1)) == (c2 >> 5)
        for g in groups:
            a = wphi_v[4 * g:4 * g + 4].reshape(L, DH)
            fm_v[g] = jnp.where(own, _dot(sel, a, NT), 0.0).astype(BF)

    def put(row, v):
        stored.add('ar')
        ar[pl.ds(row, v.shape[0]), :] = v.astype(BF)

    def slabs(start, stride, k, row0, rows):
        return jnp.concatenate(
            [ar_w[pl.ds((start + s * stride) // 2 + k * (KH * stride // 2) + row0, rows // 2), :]
             for s in range(KH)], axis=1)

    def folded(g, c, s):
        w = _unpack(w_v.bitcast(U32)[c, pl.ds(s * L // 2, L // 2), :])
        return _dot(_unpack(fm_v.bitcast(U32)[g]), w, NT) * (2.0 * LOG2E)

    def build(load, store, slots=range(NOP)):
        for r0 in range(0, L, 16):
            for k, v in enumerate(_operands(lambda i: [_unpack(load(k, r0)).astype(F32) for k in RAWL[i]], True)):
                if k in slots and k not in STAGE:
                    store(k, r0, v.v)
                if k == slots[-1]:
                    break
            yield

    def arena_build(row_of, slots=range(NOP)):
        return build(lambda k, r0: stage.bitcast(U32)[row_of(k)[1], pl.ds(r0 // 2, 8), :],
                     lambda k, r0, v: put(row_of(k)[0] + r0, v), slots)

    def put_plain(row_of, k, v):
        stored.add('stage')
        v = v.astype(BF)
        stage[row_of(k)[1]] = v
        if k < NOP:
            ar[pl.ds(row_of(k)[0], L), :] = v

    def kv_rows(gp, s):
        return lambda k: (AKV + ((k * KH + s) * 4 + gp) * L, 8 * s + STAGE.get(k, 0))

    def plain_kv(gp, s, which=(0, 1)):
        for i in which:
            g = 2 * gp + i
            for h in range(2):
                put_plain(kv_rows(gp, s), RAWL[2 * i][h], folded(g, NG + g, h * KH + s))
                put_plain(kv_rows(gp, s), RAWL[2 * i + 1][h], w_v[2 * NG + g, pl.ds(h * HK + s * L, L), :].T)

    def prep_kv(gp):
        for s in range(KH):
            plain_kv(gp, s)
            yield
            yield from arena_build(kv_rows(gp, s))

    def q_groups(gp):
        return (2 * gp, KH + 2 * gp, 2 * gp + 1, KH + 2 * gp + 1)

    def prep_q():
        for gp in range(2):
            for s in range(KH):
                def row_of(k):
                    return AQ + ((k * KH + s) * 2 + gp) * L, 8 * s + STAGE.get(k, 0)
                for i, g in enumerate(q_groups(gp)):
                    for h in range(2):
                        put_plain(row_of, RAWL[i][h], folded(g, g, h * KH + s))
                    if i % 2:
                        yield
                yield from arena_build(row_of)
            ready.add(('q', gp))

    def prep_o():
        for c in range(2):
            for r0 in range(0, HK, 16):
                blk = [wide[pl.ds(WO + h * HK + r0, 16), pl.ds(c * HK, HK)].astype(F32) for h in range(2)]
                for k, v in enumerate(_operands(lambda j: [b[:, j * L:(j + 1) * L] for b in blk], False)):
                    put(BO + (k * 2 + c) * HK + r0, v.v)
                yield

    wr = jnp.broadcast_to(wr1, (16, D))
    best = [jnp.full((16, 1), -jnp.inf, F32), jnp.zeros((16, 1), jnp.int32)]

    def row_mean(n, c, j):
        xf = wide[pl.ds(n * TT + j * L + c * 16, 16), :].astype(F32)
        mean = jnp.sum(xf, axis=1, keepdims=True) * (1.0 / D)
        stored.add('st')
        st[8 * c + 2 * j] = jnp.broadcast_to(mean, (16, L))

    def row_stats(n, c, j):
        r0 = n * TT + j * L + c * 16
        d = wide[pl.ds(r0, 16), :].astype(F32) - jnp.concatenate([st[8 * c + 2 * j]] * (D // L), axis=1)
        var = jnp.sum(d * d, axis=1, keepdims=True) * (1.0 / D)
        rs = _rcp(_rnd(jnp.sqrt(_rnd(_rnd(var) + 1e-5))))
        r = jnp.sum(d * wr, axis=1, keepdims=True) * rs
        up = (r > best[0]) | ((r == best[0]) & (r0 < best[1]))
        best[0] = jnp.where(up, r, best[0])
        best[1] = jnp.where(up, r0, best[1])
        stored.add('st')
        st[8 * c + 2 * j + 1] = jnp.broadcast_to(0.5 * rs, (16, L))
        st[64, pl.ds(8, 8), :] = jnp.broadcast_to(jnp.maximum(best[0][:8], best[0][8:]), (8, L))

    def token_operands(n, c, s):
        row = XS + s * XR + n * L + c * 16

        def block(j):
            b = [(wide[pl.ds(n * TT + j * L + c * 16, 16), pl.ds(h * HK + s * L, L)].astype(F32)
                  - st[8 * c + 2 * j]) * st[8 * c + 2 * j + 1] for h in range(2)]
            for k, v in zip(RAW[j], b):
                if k >= NOP:
                    put(row + k * KH * XR, v)
            return b

        for k, v in enumerate(_operands(block, False)):
            put(row + k * KH * XR, v.v)

    def layernorm(n):
        for j in range(4):
            row_mean(n, 0, j)
        yield
        for c in range(L // 16):
            for j in range(4):
                row_stats(n, c, j)
                if j % 2:
                    yield
            if c + 1 < L // 16:
                for j in range(4):
                    row_mean(n, c + 1, j)
                yield
            for s in range(KH):
                token_operands(n, c, s)
                yield

    side, prep, tail, tail2 = _Tasks(), _Tasks(), _Tasks(), _Tasks()
    count = [0]
    plan = [FIRST_PLAN, 0]
    delay = [1]
    timed, pending, twice, flush = {}, [], set(), []
    release = [stage.at[32]]

    def anchor(v):
        wide[pl.ds(ANCHOR + zero, 8), pl.ds(0, 2 * L)] = v.astype(BF)

    def probe(name):
        if name == 'ar':
            return ar_w[pl.ds(SPARE // 2 + zero, 8), :]
        if name == 'part':
            return pltpu.bitcast(part[NPART + zero], U32)
        if name == 'st':
            return pltpu.bitcast(st[64, pl.ds(zero, 8), :], U32)
        if name == 'stage':
            return stage.bitcast(U32)[32, pl.ds(zero, 8), :]
        return (oa0, oa1)[name == 'oa1'].bitcast(U32)[OSPARE, pl.ds(zero, 8), :]

    def gap(m):
        count[0] += 1
        for action in timed.pop(count[0], ()):
            action()
        tied = pltpu.bitcast(m[96:104], U32)
        for name in sorted(pending.pop(0) if len(pending) > delay[0] else ()):
            tied = jnp.where(never, probe(name), tied)
        m = jnp.concatenate([m[:96], pltpu.bitcast(tied, F32), m[104:]], axis=0)
        if side.q or prep.q:
            anchor(jnp.concatenate([m[:8], m[8:16]], axis=1))
        if prep.q:
            release[0][pl.ds(zero + 16, 16), :] = m[:16].astype(BF)
        tail.step(2 if count[0] in twice else 1)
        tail2.step()
        todo = PIECES[plan[0][(count[0] - plan[1] - 1) % len(plan[0])]]
        side.step(todo[0])
        prep.step(todo[1])
        pending.append(sorted(stored))
        stored.clear()
        return m

    def soon(action):
        timed.setdefault(count[0] + 1, []).append(action)

    def after(products, gen):
        start = count[0] + products

        def held():
            while count[0] < start and not flush:
                yield
            yield from gen
        return held()

    def drain_tail():
        flush.append(1)
        tail.drain()
        flush.clear()

    def unit(lhs, rhs, dims, on_block):
        for i, j, c in _block_product(lambda k: gap(_dot(_unpack(lhs(k)), _unpack(rhs(k)), dims))):
            on_block(i, j, c)

    route, ffn_out = {}, []

    def router():
        rmax = jnp.max(best[0])
        pos = best[1] + lax.broadcasted_iota(jnp.int32, (16, 1), 0)
        idx = jnp.min(jnp.where(best[0] == rmax, pos, S - 1))
        last = idx // TT
        blk = (idx // L) % 4
        row0 = pl.multiple_of((last * L + ((idx % L) // 16) * 16) // 2, 8)
        hit = lax.broadcasted_iota(jnp.int32, (16, HK), 0) == idx % 16
        route.update(rmax=rmax, idx=idx, last=last)
        for h in range(2):
            k = sum(jnp.where(blk == j, RAW[j][h], 0) for j in range(4))
            rows = _unpack(slabs(XS, XR, k, row0, 16)).astype(F32)
            row = 2.0 * jnp.sum(jnp.where(hit, rows, 0.0), axis=0, keepdims=True)
            for s in range(KH):
                xb[pl.ds(h * HK + s * L, L), :] = jnp.broadcast_to(row[:, s * L:(s + 1) * L], (L, L)).T
                yield

    def matvec(row0, col0, vec, k0, slot):
        vk = vec[pl.ds(k0, FROWS), :]
        wk = wide[pl.ds(row0 + k0, FROWS), pl.ds(col0, 2 * L)].astype(F32)
        pr = wk * jnp.concatenate([vk, vk], axis=1)
        acc = jnp.sum(pr.reshape(FROWS // 8, 8, 2 * L), axis=0)
        stored.add('part')
        for t in range(2):
            part[slot(t)] = acc[:, t * L:(t + 1) * L]

    def ffn():
        def gu_slot(c, t, p):
            return ((c % 2) * 8 + t) * 2 * NSUB + p

        def y_slot(c, t, p):
            return 32 * NSUB + (t * NFC + c) * NSUB + p

        def column(c, t):
            return jnp.sum(_total([part[gu_slot(c, t, p)] for p in range(2 * NSUB)]), axis=0, keepdims=True)

        def down(c, half):
            for t in (4 * half, 4 * half + 2):
                for p in range(NSUB):
                    matvec(WD + c * FC, t * L, hb.at[c], p * FROWS, lambda u: y_slot(c, t + u, p))
                    yield

        def result(half):
            gate = 0.5 / (1.0 + jnp.exp(-jnp.full((8, L), route['rmax'], F32)))
            for t in range(4 * half, 4 * half + 4):
                yt = sum(_total([part[y_slot(c, t, p)] for p in range(NSUB)]) for c in range(NFC))
                ffn_out.append(jnp.broadcast_to(jnp.sum(yt, axis=0, keepdims=True), (8, L)) * gate)

        for c in range(NFC):
            while c == EARLY and 'ffn' not in ready:
                yield
            for t in range(0, 8, 2):
                for p in range(2 * NSUB):
                    matvec(GU + c * D, t * L, xb, p * FROWS, lambda u: gu_slot(c, t + u, p))
                    yield
            for t in range(4):
                gate, up = column(c, t), column(c, 4 + t)
                hb[c, pl.ds(t * L, L), :] = jnp.broadcast_to(_silu(gate) * up, (L, L)).T
            yield
            if c > 0:
                yield from down(c - 1, 0)
        yield from down(0, 1)
        yield from down(NFC - 1, 0)
        result(0)
        yield
        for c in range(1, NFC):
            yield from down(c, 1)
        result(1)

    def kv_unit(gp, n):
        seen, acc = {}, {}

        def combine(g, phis, vts):
            for pp in range(2):
                p = 2 * g + pp
                acc[p] = acc.get(p, []) + [_dot(vts[pp], phis[pp], NT)]
                if len(acc[p]) == 4:
                    upd = _total(acc[p])
                    kv_acc[p] = upd if n == 0 else kv_acc[p] + upd
                yield

        def on_block(i, j, c):
            if i % 2:
                seen[i, j] = [jnp.concatenate([c[pp * 64:(pp + 1) * 64], jnp.ones((16, L), F32)], axis=0).astype(BF)
                              for pp in range(2)]
            else:
                seen[i, j] = [_key_features(c[pp * 64:(pp + 1) * 64]) for pp in range(2)]
            if (i ^ 1, j) in seen:
                tail.add(after(3, combine(2 * gp + i // 2, seen[i & 2, j], seen[i | 1, j])))

        def weights(k):
            while (gp, n) == (0, 0) and k in (7, 15) and k not in ready:
                prep.step()
            return slabs(AKV, 4 * L, k, gp * L // 2, L)

        unit(weights, lambda k: slabs(XS, XR, k, n * L // 2, L), NT, on_block)

    def first_tokens():
        for j in range(4):
            if j:
                wait(f'x0{j}')
            for part_of in (row_mean, row_stats):
                for c in range(L // 16):
                    part_of(0, c, j)
                anchor(jnp.zeros((8, 2 * L), BF))
        done = []
        for c in range(L // 16):
            for s in range(KH):
                if len(done) == 20:
                    wait('kv0a')
                    fold_matrices(range(2))
                    for t in range(KH):
                        plain_kv(0, t, (0,))
                        prep.add(arena_build(kv_rows(0, t), range(7)))
                if len(done) >= 3:
                    anchor(jnp.concatenate([done[-3], done[-3]], axis=1))
                token_operands(0, c, s)
                prep.step(2)
                done.append(pltpu.bitcast(probe('ar'), F32))
        prep.drain()

    def more_weights():
        while count[0] < 3:
            yield
        wait('kv0b')
        for s in range(KH):
            plain_kv(0, s, (1,))
            yield
        for slots in (range(7, 15), range(15, NOP)):
            for s in range(KH):
                yield from arena_build(kv_rows(0, s), slots)
            ready.add(slots[0])
        while count[0] < 16:
            yield
        wait('kv1')
        fold_matrices(range(2, NG))
        yield from prep_kv(1)

    def start_side_work(n, gp):
        if (n, gp) == (0, 1):
            wait('kv2')
            prep.add(prep_kv(2))
            plan[0] = TILE0_PLAN
        elif (n, gp) == (0, 2):
            wait('kv3')
            prep.add(prep_kv(3))
            side.add(layernorm(1))
        elif n > 0 and gp == 0:
            plan[0] = NORM_PLAN
            delay[0] = 2
            if n == 1:
                wait('wo')
                prep.add(prep_o())
            if n + 1 < NTILE:
                side.add(layernorm(n + 1))
            else:
                wait('wq')
                plan[0] = QUERY_PLAN
                side.add(router())
                side.add(ffn())
                prep.add(prep_q())

    first_tokens()
    prep.add(more_weights())
    for n in range(NTILE):
        for gp in range(4):
            if n == 0 and gp:
                prep.drain()
            if n and not gp:
                side.drain()
            soon(lambda n=n, gp=gp: start_side_work(n, gp))
            kv_unit(gp, n)
    idx, last = route['idx'], route['last']

    def finish_kv():
        r = lax.broadcasted_iota(jnp.int32, (80, L), 0)
        c = lax.broadcasted_iota(jnp.int32, (80, L), 1)
        keep = jnp.where(r < 64, r >> 5, r & 1) == (c & 1)
        double = jnp.where(r < 64, 2.0, 1.0)
        for p in range(NP):
            kvl[p] = jnp.where(keep, kv_acc[p] * double, 0.0).astype(BF)
        yield

    tail.add(finish_kv())

    built = {}

    def tile_of(n):
        return (last + 1 + n) % NTILE

    def token_words(n):
        return ar_w.at[pl.ds(pl.multiple_of(XS // 2 + tile_of(n) * (L // 2), 8), ((NOP + 3) * KH * XR - XR + L) // 2)]

    def o_operands(n, gp):
        oa = (oa0, oa1)[n % 2]
        release[0] = oa.at[OSPARE]
        for slab in (2 * gp, 2 * gp + 1):
            def store(k, r0, v):
                stored.add(f'oa{n % 2}')
                oa[k * KH + slab, pl.ds(r0, 16), :] = v.astype(BF)
            yield from build(lambda k, r0: oa.bitcast(U32)[k * KH + slab, pl.ds(r0 // 2, 8), :], store)
        built[n] = built.get(n, 0) + 1

    def q_unit(gp, n):
        while ('q', gp) not in ready:
            prep.step()
        left = [16]
        oa = (oa0, oa1)[n % 2]

        def attend(i, j, feats):
            rows = []
            for pp, (phi, scale) in enumerate(feats):
                nd = _dot(_unpack(kvl.bitcast(U32)[2 * q_groups(gp)[i] + pp]), phi, NN)
                inv = _rcp(nd[64:72] + 1e-6 * scale)
                for head in range(2):
                    rd = jnp.broadcast_to(inv[head:head + 1], (8, L))
                    rows += [nd[head * DH + 8 * q:head * DH + 8 * q + 8] * rd for q in range(4)]
                if pp == 0:
                    yield
            oa[RAWL[j][i % 2] * KH + 2 * gp + i // 2] = jnp.concatenate(rows, axis=0).T.astype(BF)
            left[0] -= 1
            if not left[0]:
                prep.add(o_operands(n, gp))
            yield

        def on_block(i, j, c):
            tail.add(after(4, attend(i, j, [_query_features(c[pp * 64:(pp + 1) * 64]) for pp in range(2)])))

        tokens = token_words(n)
        unit(lambda k: slabs(AQ, 2 * L, k, gp * L // 2, L),
             lambda k: jnp.concatenate([tokens[pl.ds((k * KH + s) * XR // 2, L // 2), :] for s in range(KH)], axis=1),
             NT, on_block)

    def o_unit(c, n):
        t = tile_of(n)
        tokens = token_words(n)
        x_tile = wide.at[pl.ds(pl.multiple_of(t * TT, TT), TT)]
        left = [16]

        def finish(j, col, s):
            cols = pl.ds(c * HK + col * L, L)
            half = _unpack(tokens[pl.ds((RAW[j][c] * KH + col) * XR // 2, L // 2), :]).astype(F32)
            if n == NTILE - 1:
                rid = lax.broadcasted_iota(jnp.int32, (L, L), 0) + j * L
                y = jnp.concatenate([ffn_out[c * KH + col]] * (L // 8), axis=0)
                half = half + jnp.where(rid == idx % TT, y, 0.0)
            sh = s * half
            out_v[pl.ds(n * TT + j * L, L), cols] = (
                x_tile[pl.ds(j * L, L), cols].astype(F32) + sh + sh * jnp.tanh(half)).astype(BF)
            left[0] -= 1
            if (n, c) == (NTILE - 1, 1):
                out_copy(n * TT + j * L, pl.multiple_of(t * TT + j * L, L), L, cols.start, L).start()
            elif not left[0]:
                out_copy(n * TT, pl.multiple_of(t * TT, TT), TT, c * HK, HK).start()
            yield

        while n == NTILE - 1 and len(ffn_out) < 4 * (c + 1):
            side.step()
        if c == 0:
            if n == NTILE - 1:
                drain_tail()
            while built.get(n, 0) < 2:
                (prep if prep.q else tail).step()
        oa = (oa0, oa1)[n % 2].bitcast(U32)
        unit(lambda k: jnp.concatenate([oa[k * KH + s] for s in range(KH)], axis=1),
             lambda k: ar_w[pl.ds((BO + (k * 2 + c) * HK) // 2, HK // 2), :], NN,
             lambda j, col, s: tail2.add(finish(j, col, s)))

    twice.update(count[0] + t for t in range(12, 60, 2))
    plan[:] = [OUT_PLAN, count[0]]
    delay[0] = 1
    q_unit(0, 0)
    soon(lambda: wait('ffn'))
    soon(lambda: ready.add('ffn'))
    q_unit(1, 0)
    for n in range(1, NTILE):
        for gp in range(2):
            q_unit(gp, n)
            o_unit(gp, n - 1)
    for c in range(2):
        o_unit(c, NTILE - 1)
    drain_tail()
    tail2.drain()
    for _ in range(2 * NTILE - 1):
        out_copy(0, 0, TT, 0, HK).wait()
    for _ in range(16):
        out_copy(0, 0, L, 0, L).wait()


@jax.jit
def pallas_recurrent_scan__linear_kernel_hedgehog__moe_arch_mod__prompt_kernel(
    A_x: jax.Array,
    A_wqkv: jax.Array,
    A_w_phi: jax.Array,
    A_wo: jax.Array,
    B_x: jax.Array,
    B_w_r: jax.Array,
    B_w_gate: jax.Array,
    B_w_up: jax.Array,
    B_w_down: jax.Array,
):
    del B_x
    hbm = pl.BlockSpec(memory_space=pl.ANY)
    return pl.pallas_call(
        _kernel,
        out_shape=jax.ShapeDtypeStruct(A_x.shape, A_x.dtype),
        in_specs=[hbm] * 8,
        out_specs=hbm,
        scratch_shapes=[
            pltpu.VMEM((ANCHOR + 8, D), BF),
            pltpu.VMEM((3 * NG, D, L), BF),
            pltpu.VMEM((H, DH, DH), BF),
            pltpu.VMEM((D,), BF),
            pltpu.VMEM((NG, L, L), BF),
            pltpu.VMEM((NPART + 1, 8, L), F32),
            pltpu.VMEM((65, 16, L), F32),
            pltpu.VMEM((SPARE + 16, L), BF),
            pltpu.VMEM((33, L, L), BF),
            pltpu.VMEM((OSPARE + 1, L, L), BF),
            pltpu.VMEM((OSPARE + 1, L, L), BF),
            pltpu.VMEM((NP, 80, L), BF),
            pltpu.VMEM((NP, 80, L), F32),
            pltpu.VMEM((S, D), BF),
            pltpu.VMEM((D, L), F32),
            pltpu.VMEM((NFC, FC, L), F32),
            pltpu.SemaphoreType.DMA((12,)),
        ],
        compiler_params=pltpu.CompilerParams(vmem_limit_bytes=120 << 20),
        name="hedgehog_mod",
    )(A_x, A_wqkv, A_w_phi, A_wo, B_w_r, B_w_gate, B_w_up, B_w_down)
```

```python
import jax
import jax.numpy as jnp
from jax import lax
import jax.experimental.pallas as pl
import jax.experimental.pallas.tpu as pltpu

BF = jnp.bfloat16
F32 = jnp.float32
U32 = jnp.uint32
NN = (((1,), (0,)), ((), ()))
NT = (((1,), (1,)), ((), ()))
LOG2E = 1.4426950408889634

S, D, H, DH, FF = 2048, 1024, 32, 32, 3584
L = 128
HK = D // 2
KH = HK // L
NG = H // 4
NP = H // 2
TT = 4 * L
NTILE = S // TT
FC = 4 * L
NFC = FF // FC
FROWS = 128
NSUB = HK // FROWS
EARLY = 3
NOP = 26
RAW = ((1, 26), (27, 2), (7, 8), (16, 28))
RAWL = ((26, 0), (3, 27), (7, 8), (28, 15))
STAGE = {k: i for i, k in enumerate(sum(RAWL, ()))}

XR = S // 4
XS = 16
AKV = XS + (NOP + 3) * KH * XR
AQ = AKV + NOP * KH * 4 * L
BO = AQ + NOP * KH * 2 * L
SPARE = BO + NOP * 2 * HK
GU = S
WD = GU + NFC * D
WO = WD + FF
ANCHOR = WO + D
NPART = (32 + 8 * NFC) * NSUB
OSPARE = (NOP + 3) * KH

PIECES = {'.': (0, 0), 'L': (1, 0), '2': (2, 0), 'P': (0, 1), '3': (0, 2), '5': (0, 3), '9': (0, 8),
          'B': (1, 1), '6': (1, 2)}
FIRST_PLAN = '.935555555533355535535533P'
TILE0_PLAN = '.' * NOP + 'PP33PP3P33P333PP3PPPPP3PPP' '3B63BB6BBBB6B6P3BBB666PBB3' '2L2LLL22L22LL222LLLL2LLL2L'
NORM_PLAN = 'PBPLLPLPPPLLLL.L.LBLL.LL.P'
QUERY_PLAN = 'LBBBBBLBBBBB.BBBBBBBBBBLP.'
OUT_PLAN = ('L.L.LL.LLLL.LLLLLLLLL.LLL.' 'LLL.LLLLLLBPBPBPBPPPBPBPBB'
            '.LBP.LPBPLBPPLPBLPPPLLPPBP' 'LBBPLP.LLBPPB.BLPBLPLLLLL.'
            + 'PLLL.LL.BLPBPLPLBLLLPLLLPL' 'LBBPLPPLPBPPB.PLLBLLLLLLL.' * 4
            + 'B.LLLLBLBLPPLLPLLP.LPLLLPL' 'LBBLLLBPPBBPPBPPBPPLPPBPPP'
            'LLLLLLLLLLLLLLLLLLLLLLLLLL' '..........................')
DOT_PLAN = ('11221111111111122211111222' '22111211211222112211121222'
            '12121211111111111111111111' '11111111111111121111111111'
            + '11111112111211111112111221' '11211111111111111111111111' * 4
            + '21111111111112112212111111' '11211111111111111111111111'
            '11111111111111111111111111' '11111111111111111111111111')


def _dot(a, b, dims):
    return lax.dot_general(a, b, dims, preferred_element_type=F32)


def _unpack(words):
    return pltpu.bitcast(words, BF)


def _rnd(v):
    return v.astype(BF).astype(F32)


def _rcp(v):
    return pltpu.reciprocal(v, approx=True)


def _silu(v):
    h = 0.5 * v
    return h + h * jnp.tanh(h)


def _total(v):
    while len(v) > 1:
        v = [v[i] + v[i + 1] for i in range(0, len(v), 2)]
    return v[0]


def _pair_reduce(v, reduce, op):
    r = reduce(v, axis=0)
    r = op(r, pltpu.roll(r, 2, 0))
    return op(r, pltpu.roll(r, 4, 0))


def _dual_exp(p):
    v = p.reshape(8, 8, L)
    ep = jnp.exp2(v - _pair_reduce(v, jnp.max, jnp.maximum))
    en = jnp.exp2(_pair_reduce(v, jnp.min, jnp.minimum) - v)
    return ep, en, _pair_reduce(ep, jnp.sum, jnp.add), _pair_reduce(en, jnp.sum, jnp.add)


def _key_features(p):
    ep, en, sp, sn = _dual_exp(p)
    return jnp.concatenate([ep * _rcp(sp), en * _rcp(sn)], axis=0).reshape(L, L).astype(BF)


def _query_features(p):
    ep, en, sp, sn = _dual_exp(p)
    return jnp.concatenate([ep, en * (sp * _rcp(sn))], axis=0).reshape(L, L).astype(BF), sp


class _Signed:
    def __init__(self, sign, v):
        self.sign, self.v = sign, v

    def __neg__(self):
        return _Signed(-self.sign, self.v)

    def __add__(self, o):
        if self.sign == o.sign:
            return _Signed(self.sign, self.v + o.v)
        return _Signed(1, self.v - o.v if self.sign > 0 else o.v - self.v)

    def __sub__(self, o):
        return self + (-o)


def _nxt(k, d=1):
    return (k - 1 + d) % 3 + 1


def _operands(block, left):
    lo, hi = (1, 2) if left else (2, 1)

    def forms(i):
        x, y = block(i)
        if left:
            return {1: _Signed(1, x), 2: _Signed(-1, y), 3: _Signed(1, y - x)}
        return {1: _Signed(1, y), 2: _Signed(1, x), 3: _Signed(-1, x + y)}

    def diag(g, k):
        yield g[_nxt(k, lo)]
        yield g[_nxt(k, hi)]

    def pair(ga, gb, k, s):
        m = _nxt(k, 2)
        yield gb[k] - ga[_nxt(k)] if left else ga[_nxt(k)] - gb[k]
        for n in (_nxt(m, lo), _nxt(m, hi)):
            s[n] = ga[n] + gb[n]
            yield s[n]

    f0 = forms(0)
    yield from diag(f0, 1)
    f1 = forms(1)
    yield from diag(f1, 2)
    yield from pair(f0, f1, 1, {})
    f2 = forms(2)
    yield from diag(f2, 3)
    yield from pair(f1, f2, 2, {})
    s02 = {}
    yield from pair(f2, f0, 3, s02)
    s02[2] = f0[2] + f2[2]
    f3 = forms(3)
    yield from diag(f3, 1)
    yield from pair(f2, f3, 3, {})
    yield from pair(f3, s02, 1, {})
    yield from pair(f3, f1, 1, {})


_SIGNS = [a.sign * b.sign for a, b in zip(_operands(lambda i: (0, 0), True), _operands(lambda i: (0, 0), False))]


def _block_product(product):
    count = iter(range(NOP))

    def m(sign=1):
        k = next(count)
        return _Signed(sign * _SIGNS[k], product(k))

    def diag(i):
        x, y = m(), m(-1)
        yield i, i, x + y
        return x, y

    def pair(a, b, da, db, less=(None, None)):
        g = m()
        xs = m()
        ab = xs - da[1] - db[1] - g
        yield a, b, ab if less[0] is None else ab - less[0]
        ys = m(-1)
        ba = ys - da[0] - db[0] + g
        yield b, a, ba if less[1] is None else ba - less[1]
        return (xs, ys), (ab, ba)

    def steps():
        d0 = yield from diag(0)
        d1 = yield from diag(1)
        yield from pair(0, 1, d0, d1)
        d2 = yield from diag(2)
        yield from pair(1, 2, d1, d2)
        d02, _ = yield from pair(2, 0, d2, d0)
        d3 = yield from diag(3)
        _, (c23, c32) = yield from pair(2, 3, d2, d3)
        yield from pair(3, 0, d3, d02, (c32, c23))
        yield from pair(3, 1, d3, d1)

    for i, j, c in steps():
        assert c.sign > 0
        yield i, j, c.v


class _Tasks:
    def __init__(self):
        self.q = []

    def add(self, gen):
        self.q.append(gen)

    def step(self, n=1):
        while n > 0 and self.q:
            try:
                next(self.q[0])
                n -= 1
            except StopIteration:
                self.q.pop(0)

    def drain(self):
        while self.q:
            self.step()


def _kernel(x_hbm, wqkv_hbm, wphi_hbm, wo_hbm, wr_hbm, wg_hbm, wu_hbm, wd_hbm, out_hbm,
            wide, w_v, wphi_v, wr_v, fm_v, part, st, ar, stage, oa0, oa1, kvl, kv_acc, out_v, xb, hb, sems):

    def x_rows(row0, rows):
        return x_hbm.at[0, pl.ds(row0, rows)], wide.at[pl.ds(row0, rows)]

    def w_cols(c):
        return wqkv_hbm.at[:, pl.ds(c * L, L)], w_v.at[c]

    def kv_cols(gp):
        return [w_cols(o + g) for g in (2 * gp, 2 * gp + 1) for o in (NG, 2 * NG)]

    def phi_heads(h0, heads):
        return wphi_hbm.at[pl.ds(h0, heads)], wphi_v.at[pl.ds(h0, heads)]

    def ffn_chunk(c):
        cols = pl.ds(c * FC, FC)
        rows = pl.ds(GU + c * D, D)
        return [(wg_hbm.at[:, cols], wide.at[rows, pl.ds(0, FC)]),
                (wu_hbm.at[:, cols], wide.at[rows, pl.ds(FC, FC)]),
                (wd_hbm.at[cols], wide.at[pl.ds(WD + c * FC, FC)])]

    loads = {
        'x00': [(wr_hbm, wr_v), x_rows(0, L)],
        'x01': [x_rows(L, L)],
        'x02': [x_rows(2 * L, L)],
        'x03': [x_rows(3 * L, L)],
        'kv0a': [phi_heads(0, 8)] + kv_cols(0)[:2],
        'kv0b': kv_cols(0)[2:],
        'kv1': [phi_heads(8, H - 8)] + kv_cols(1),
        'kv2': kv_cols(2),
        'kv3': [x_rows(TT, TT)] + kv_cols(3),
        'wo': [x_rows(n * TT, TT) for n in range(2, NTILE)] + [(wo_hbm, wide.at[pl.ds(WO, D)])],
        'wq': [w_cols(g) for g in range(NG)] + [p for c in range(EARLY) for p in ffn_chunk(c)],
        'ffn': [p for c in range(EARLY, NFC) for p in ffn_chunk(c)],
    }

    def copies(name):
        return [pltpu.make_async_copy(src, dst, sems.at[list(loads).index(name)]) for src, dst in loads[name]]

    def wait(name):
        for cp in copies(name):
            cp.wait()

    def out_copy(src0, dst0, rows, col0, cols):
        return pltpu.make_async_copy(out_v.at[pl.ds(src0, rows), pl.ds(col0, cols)],
                                     out_hbm.at[0, pl.ds(dst0, rows), pl.ds(col0, cols)], sems.at[0])

    for name in loads:
        for cp in copies(name):
            cp.start(priority=1)

    ar_w = ar.bitcast(U32)
    stored = set()
    ready = set()

    wait('x00')
    wr1 = wr_v[...].astype(F32).reshape(1, D)
    zero = pl.multiple_of(jnp.max(jnp.where(jnp.abs(wr1) < 0.0, pltpu.bitcast(wr1, jnp.int32), 0)), 16)
    never = zero > 0
    ar[pl.ds(SPARE, 16), :] = jnp.zeros((16, L), BF)
    part[NPART] = jnp.zeros((8, L), F32)
    st[64] = jnp.zeros((16, L), F32)
    stage[32, pl.ds(0, 16), :] = jnp.zeros((16, L), BF)
    for oa in (oa0, oa1):
        oa[OSPARE, pl.ds(0, 16), :] = jnp.zeros((16, L), BF)

    def fold_matrices(groups):
        rr = lax.broadcasted_iota(jnp.int32, (L, DH), 0)
        ff = lax.broadcasted_iota(jnp.int32, (L, DH), 1)
        sel = jnp.where(((rr & 63) >> 1) == ff, 1.0, 0.0).astype(BF)
        r2 = lax.broadcasted_iota(jnp.int32, (L, L), 0)
        c2 = lax.broadcasted_iota(jnp.int32, (L, L), 1)
        own = ((r2 >> 6) * 2 + (r2 & 1)) == (c2 >> 5)
        for g in groups:
            a = wphi_v[4 * g:4 * g + 4].reshape(L, DH)
            fm_v[g] = jnp.where(own, _dot(sel, a, NT), 0.0).astype(BF)

    def put(row, v):
        stored.add('ar')
        ar[pl.ds(row, v.shape[0]), :] = v.astype(BF)

    def slabs(start, stride, k, row0, rows):
        return jnp.concatenate(
            [ar_w[pl.ds((start + s * stride) // 2 + k * (KH * stride // 2) + row0, rows // 2), :]
             for s in range(KH)], axis=1)

    def folded(g, c, s):
        w = _unpack(w_v.bitcast(U32)[c, pl.ds(s * L // 2, L // 2), :])
        return _dot(_unpack(fm_v.bitcast(U32)[g]), w, NT) * (2.0 * LOG2E)

    def build(load, store, slots=range(NOP)):
        for r0 in range(0, L, 16):
            for k, v in enumerate(_operands(lambda i: [_unpack(load(k, r0)).astype(F32) for k in RAWL[i]], True)):
                if k in slots and k not in STAGE:
                    store(k, r0, v.v)
                if k == slots[-1]:
                    break
            yield

    def arena_build(row_of, slots=range(NOP)):
        return build(lambda k, r0: stage.bitcast(U32)[row_of(k)[1], pl.ds(r0 // 2, 8), :],
                     lambda k, r0, v: put(row_of(k)[0] + r0, v), slots)

    def put_plain(row_of, k, v):
        stored.add('stage')
        v = v.astype(BF)
        stage[row_of(k)[1]] = v
        if k < NOP:
            ar[pl.ds(row_of(k)[0], L), :] = v

    def kv_rows(gp, s):
        return lambda k: (AKV + ((k * KH + s) * 4 + gp) * L, 8 * s + STAGE.get(k, 0))

    def plain_kv(gp, s, which=(0, 1)):
        for i in which:
            g = 2 * gp + i
            for h in range(2):
                put_plain(kv_rows(gp, s), RAWL[2 * i][h], folded(g, NG + g, h * KH + s))
                put_plain(kv_rows(gp, s), RAWL[2 * i + 1][h], w_v[2 * NG + g, pl.ds(h * HK + s * L, L), :].T)

    def prep_kv(gp):
        for s in range(KH):
            plain_kv(gp, s)
            yield
            yield from arena_build(kv_rows(gp, s))

    def q_groups(gp):
        return (2 * gp, KH + 2 * gp, 2 * gp + 1, KH + 2 * gp + 1)

    def prep_q():
        for gp in range(2):
            for s in range(KH):
                def row_of(k):
                    return AQ + ((k * KH + s) * 2 + gp) * L, 8 * s + STAGE.get(k, 0)
                for i, g in enumerate(q_groups(gp)):
                    for h in range(2):
                        put_plain(row_of, RAWL[i][h], folded(g, g, h * KH + s))
                    if i % 2:
                        yield
                yield from arena_build(row_of)
            ready.add(('q', gp))

    def prep_o():
        for c in range(2):
            for r0 in range(0, HK, 16):
                blk = [wide[pl.ds(WO + h * HK + r0, 16), pl.ds(c * HK, HK)].astype(F32) for h in range(2)]
                for k, v in enumerate(_operands(lambda j: [b[:, j * L:(j + 1) * L] for b in blk], False)):
                    put(BO + (k * 2 + c) * HK + r0, v.v)
                yield

    wr = jnp.broadcast_to(wr1, (16, D))
    best = [jnp.full((16, 1), -jnp.inf, F32), jnp.zeros((16, 1), jnp.int32)]

    def row_mean(n, c, j):
        xf = wide[pl.ds(n * TT + j * L + c * 16, 16), :].astype(F32)
        mean = jnp.sum(xf, axis=1, keepdims=True) * (1.0 / D)
        stored.add('st')
        st[8 * c + 2 * j] = jnp.broadcast_to(mean, (16, L))

    def row_stats(n, c, j):
        r0 = n * TT + j * L + c * 16
        d = wide[pl.ds(r0, 16), :].astype(F32) - jnp.concatenate([st[8 * c + 2 * j]] * (D // L), axis=1)
        var = jnp.sum(d * d, axis=1, keepdims=True) * (1.0 / D)
        rs = _rcp(_rnd(jnp.sqrt(_rnd(_rnd(var) + 1e-5))))
        r = jnp.sum(d * wr, axis=1, keepdims=True) * rs
        up = (r > best[0]) | ((r == best[0]) & (r0 < best[1]))
        best[0] = jnp.where(up, r, best[0])
        best[1] = jnp.where(up, r0, best[1])
        stored.add('st')
        st[8 * c + 2 * j + 1] = jnp.broadcast_to(0.5 * rs, (16, L))
        st[64, pl.ds(8, 8), :] = jnp.broadcast_to(jnp.maximum(best[0][:8], best[0][8:]), (8, L))

    def token_operands(n, c, s):
        row = XS + s * XR + n * L + c * 16

        def block(j):
            b = [(wide[pl.ds(n * TT + j * L + c * 16, 16), pl.ds(h * HK + s * L, L)].astype(F32)
                  - st[8 * c + 2 * j]) * st[8 * c + 2 * j + 1] for h in range(2)]
            for k, v in zip(RAW[j], b):
                if k >= NOP:
                    put(row + k * KH * XR, v)
            return b

        for k, v in enumerate(_operands(block, False)):
            put(row + k * KH * XR, v.v)

    def layernorm(n):
        for j in range(4):
            row_mean(n, 0, j)
        yield
        for c in range(L // 16):
            for j in range(4):
                row_stats(n, c, j)
                if j % 2:
                    yield
            if c + 1 < L // 16:
                for j in range(4):
                    row_mean(n, c + 1, j)
                yield
            for s in range(KH):
                token_operands(n, c, s)
                yield

    side, prep, tail, tail2 = _Tasks(), _Tasks(), _Tasks(), _Tasks()
    count = [0]
    plan = [FIRST_PLAN, 0]
    delay = [1]
    timed, pending, dots, flush = {}, [], {}, []
    release = [stage.at[32]]

    def anchor(v):
        wide[pl.ds(ANCHOR + zero, 8), pl.ds(0, 2 * L)] = v.astype(BF)

    def probe(name):
        if name == 'ar':
            return ar_w[pl.ds(SPARE // 2 + zero, 8), :]
        if name == 'part':
            return pltpu.bitcast(part[NPART + zero], U32)
        if name == 'st':
            return pltpu.bitcast(st[64, pl.ds(zero, 8), :], U32)
        if name == 'stage':
            return stage.bitcast(U32)[32, pl.ds(zero, 8), :]
        return (oa0, oa1)[name == 'oa1'].bitcast(U32)[OSPARE, pl.ds(zero, 8), :]

    def gap(m):
        count[0] += 1
        for action in timed.pop(count[0], ()):
            action()
        tied = pltpu.bitcast(m[96:104], U32)
        for name in sorted(pending.pop(0) if len(pending) > delay[0] else ()):
            tied = jnp.where(never, probe(name), tied)
        m = jnp.concatenate([m[:96], pltpu.bitcast(tied, F32), m[104:]], axis=0)
        if side.q or prep.q:
            anchor(jnp.concatenate([m[:8], m[8:16]], axis=1))
        if prep.q:
            release[0][pl.ds(zero + 16, 16), :] = m[:16].astype(BF)
        tail.step(dots.get(count[0], 1))
        tail2.step()
        todo = PIECES[plan[0][(count[0] - plan[1] - 1) % len(plan[0])]]
        side.step(todo[0])
        prep.step(todo[1])
        pending.append(sorted(stored))
        stored.clear()
        return m

    def soon(action):
        timed.setdefault(count[0] + 1, []).append(action)

    def after(products, gen):
        start = count[0] + products

        def held():
            while count[0] < start and not flush:
                yield
            yield from gen
        return held()

    def drain_tail():
        flush.append(1)
        tail.drain()
        flush.clear()

    def unit(lhs, rhs, dims, on_block):
        for i, j, c in _block_product(lambda k: gap(_dot(_unpack(lhs(k)), _unpack(rhs(k)), dims))):
            on_block(i, j, c)

    route, ffn_out = {}, []

    def router():
        rmax = jnp.max(best[0])
        pos = best[1] + lax.broadcasted_iota(jnp.int32, (16, 1), 0)
        idx = jnp.min(jnp.where(best[0] == rmax, pos, S - 1))
        last = idx // TT
        blk = (idx // L) % 4
        row0 = pl.multiple_of((last * L + ((idx % L) // 16) * 16) // 2, 8)
        hit = lax.broadcasted_iota(jnp.int32, (16, HK), 0) == idx % 16
        route.update(rmax=rmax, idx=idx, last=last)
        for h in range(2):
            k = sum(jnp.where(blk == j, RAW[j][h], 0) for j in range(4))
            rows = _unpack(slabs(XS, XR, k, row0, 16)).astype(F32)
            row = 2.0 * jnp.sum(jnp.where(hit, rows, 0.0), axis=0, keepdims=True)
            for s in range(KH):
                xb[pl.ds(h * HK + s * L, L), :] = jnp.broadcast_to(row[:, s * L:(s + 1) * L], (L, L)).T
                yield

    def matvec(row0, col0, vec, k0, slot):
        vk = vec[pl.ds(k0, FROWS), :]
        wk = wide[pl.ds(row0 + k0, FROWS), pl.ds(col0, 2 * L)].astype(F32)
        pr = wk * jnp.concatenate([vk, vk], axis=1)
        acc = jnp.sum(pr.reshape(FROWS // 8, 8, 2 * L), axis=0)
        stored.add('part')
        for t in range(2):
            part[slot(t)] = acc[:, t * L:(t + 1) * L]

    def ffn():
        def gu_slot(c, t, p):
            return ((c % 2) * 8 + t) * 2 * NSUB + p

        def y_slot(c, t, p):
            return 32 * NSUB + (t * NFC + c) * NSUB + p

        def column(c, t):
            return jnp.sum(_total([part[gu_slot(c, t, p)] for p in range(2 * NSUB)]), axis=0, keepdims=True)

        def down(c, half):
            for t in (4 * half, 4 * half + 2):
                for p in range(NSUB):
                    matvec(WD + c * FC, t * L, hb.at[c], p * FROWS, lambda u: y_slot(c, t + u, p))
                    yield

        def result(half):
            gate = 0.5 / (1.0 + jnp.exp(-jnp.full((8, L), route['rmax'], F32)))
            for t in range(4 * half, 4 * half + 4):
                yt = sum(_total([part[y_slot(c, t, p)] for p in range(NSUB)]) for c in range(NFC))
                ffn_out.append(jnp.broadcast_to(jnp.sum(yt, axis=0, keepdims=True), (8, L)) * gate)

        for c in range(NFC):
            while c == EARLY and 'ffn' not in ready:
                yield
            for t in range(0, 8, 2):
                for p in range(2 * NSUB):
                    matvec(GU + c * D, t * L, xb, p * FROWS, lambda u: gu_slot(c, t + u, p))
                    yield
            for t in range(4):
                gate, up = column(c, t), column(c, 4 + t)
                hb[c, pl.ds(t * L, L), :] = jnp.broadcast_to(_silu(gate) * up, (L, L)).T
            yield
            if c > 0:
                yield from down(c - 1, 0)
        yield from down(0, 1)
        yield from down(NFC - 1, 0)
        result(0)
        yield
        for c in range(1, NFC):
            yield from down(c, 1)
        result(1)

    def kv_unit(gp, n):
        seen, acc = {}, {}

        def combine(g, phis, vts):
            for pp in range(2):
                p = 2 * g + pp
                acc[p] = acc.get(p, []) + [_dot(vts[pp], phis[pp], NT)]
                if len(acc[p]) == 4:
                    upd = _total(acc[p])
                    kv_acc[p] = upd if n == 0 else kv_acc[p] + upd
                yield

        def on_block(i, j, c):
            if i % 2:
                seen[i, j] = [jnp.concatenate([c[pp * 64:(pp + 1) * 64], jnp.ones((16, L), F32)], axis=0).astype(BF)
                              for pp in range(2)]
            else:
                seen[i, j] = [_key_features(c[pp * 64:(pp + 1) * 64]) for pp in range(2)]
            if (i ^ 1, j) in seen:
                tail.add(after(3, combine(2 * gp + i // 2, seen[i & 2, j], seen[i | 1, j])))

        def weights(k):
            while (gp, n) == (0, 0) and k in (7, 15) and k not in ready:
                prep.step()
            return slabs(AKV, 4 * L, k, gp * L // 2, L)

        unit(weights, lambda k: slabs(XS, XR, k, n * L // 2, L), NT, on_block)

    def first_tokens():
        for j in range(4):
            if j:
                wait(f'x0{j}')
            for part_of in (row_mean, row_stats):
                for c in range(L // 16):
                    part_of(0, c, j)
                anchor(jnp.zeros((8, 2 * L), BF))
        done = []
        for c in range(L // 16):
            for s in range(KH):
                if len(done) == 20:
                    wait('kv0a')
                    fold_matrices(range(2))
                    for t in range(KH):
                        plain_kv(0, t, (0,))
                        prep.add(arena_build(kv_rows(0, t), range(7)))
                if len(done) >= 3:
                    anchor(jnp.concatenate([done[-3], done[-3]], axis=1))
                token_operands(0, c, s)
                prep.step(2)
                done.append(pltpu.bitcast(probe('ar'), F32))
        prep.drain()

    def more_weights():
        while count[0] < 3:
            yield
        wait('kv0b')
        for s in range(KH):
            plain_kv(0, s, (1,))
            yield
        for slots in (range(7, 15), range(15, NOP)):
            for s in range(KH):
                yield from arena_build(kv_rows(0, s), slots)
            ready.add(slots[0])
        while count[0] < 16:
            yield
        wait('kv1')
        fold_matrices(range(2, NG))
        yield from prep_kv(1)

    def start_side_work(n, gp):
        if (n, gp) == (0, 1):
            wait('kv2')
            prep.add(prep_kv(2))
            plan[0] = TILE0_PLAN
        elif (n, gp) == (0, 2):
            wait('kv3')
            prep.add(prep_kv(3))
            side.add(layernorm(1))
        elif n > 0 and gp == 0:
            plan[0] = NORM_PLAN
            delay[0] = 2
            if n == 1:
                wait('wo')
                prep.add(prep_o())
            if n + 1 < NTILE:
                side.add(layernorm(n + 1))
            else:
                wait('wq')
                plan[0] = QUERY_PLAN
                side.add(router())
                side.add(ffn())
                prep.add(prep_q())

    first_tokens()
    prep.add(more_weights())
    for n in range(NTILE):
        for gp in range(4):
            if n == 0 and gp:
                prep.drain()
            if n and not gp:
                side.drain()
            soon(lambda n=n, gp=gp: start_side_work(n, gp))
            kv_unit(gp, n)
    idx, last = route['idx'], route['last']

    def finish_kv():
        r = lax.broadcasted_iota(jnp.int32, (80, L), 0)
        c = lax.broadcasted_iota(jnp.int32, (80, L), 1)
        keep = jnp.where(r < 64, r >> 5, r & 1) == (c & 1)
        double = jnp.where(r < 64, 2.0, 1.0)
        for p in range(NP):
            kvl[p] = jnp.where(keep, kv_acc[p] * double, 0.0).astype(BF)
        yield

    tail.add(finish_kv())

    built = {}

    def tile_of(n):
        return (last + 1 + n) % NTILE

    def token_words(n):
        return ar_w.at[pl.ds(pl.multiple_of(XS // 2 + tile_of(n) * (L // 2), 8), ((NOP + 3) * KH * XR - XR + L) // 2)]

    def o_operands(n, gp):
        oa = (oa0, oa1)[n % 2]
        release[0] = oa.at[OSPARE]
        for slab in (2 * gp, 2 * gp + 1):
            def store(k, r0, v):
                stored.add(f'oa{n % 2}')
                oa[k * KH + slab, pl.ds(r0, 16), :] = v.astype(BF)
            yield from build(lambda k, r0: oa.bitcast(U32)[k * KH + slab, pl.ds(r0 // 2, 8), :], store)
        built[n] = built.get(n, 0) + 1

    def q_unit(gp, n):
        while ('q', gp) not in ready:
            prep.step()
        left = [16]
        oa = (oa0, oa1)[n % 2]

        def attend(i, j, feats):
            rows = []
            for pp, (phi, scale) in enumerate(feats):
                nd = _dot(_unpack(kvl.bitcast(U32)[2 * q_groups(gp)[i] + pp]), phi, NN)
                inv = _rcp(nd[64:72] + 1e-6 * scale)
                for head in range(2):
                    rd = jnp.broadcast_to(inv[head:head + 1], (8, L))
                    rows += [nd[head * DH + 8 * q:head * DH + 8 * q + 8] * rd for q in range(4)]
                if pp == 0:
                    yield
            oa[RAWL[j][i % 2] * KH + 2 * gp + i // 2] = jnp.concatenate(rows, axis=0).T.astype(BF)
            left[0] -= 1
            if not left[0]:
                prep.add(o_operands(n, gp))
            yield

        def on_block(i, j, c):
            tail.add(after(4, attend(i, j, [_query_features(c[pp * 64:(pp + 1) * 64]) for pp in range(2)])))

        tokens = token_words(n)
        unit(lambda k: slabs(AQ, 2 * L, k, gp * L // 2, L),
             lambda k: jnp.concatenate([tokens[pl.ds((k * KH + s) * XR // 2, L // 2), :] for s in range(KH)], axis=1),
             NT, on_block)

    def o_unit(c, n):
        t = tile_of(n)
        tokens = token_words(n)
        x_tile = wide.at[pl.ds(pl.multiple_of(t * TT, TT), TT)]
        left = [16]

        def finish(j, col, s):
            cols = pl.ds(c * HK + col * L, L)
            half = _unpack(tokens[pl.ds((RAW[j][c] * KH + col) * XR // 2, L // 2), :]).astype(F32)
            if n == NTILE - 1:
                rid = lax.broadcasted_iota(jnp.int32, (L, L), 0) + j * L
                y = jnp.concatenate([ffn_out[c * KH + col]] * (L // 8), axis=0)
                half = half + jnp.where(rid == idx % TT, y, 0.0)
            sh = s * half
            out_v[pl.ds(n * TT + j * L, L), cols] = (
                x_tile[pl.ds(j * L, L), cols].astype(F32) + sh + sh * jnp.tanh(half)).astype(BF)
            left[0] -= 1
            if (n, c) == (NTILE - 1, 1):
                out_copy(n * TT + j * L, pl.multiple_of(t * TT + j * L, L), L, cols.start, L).start()
            elif not left[0]:
                out_copy(n * TT, pl.multiple_of(t * TT, TT), TT, c * HK, HK).start()
            yield

        while n == NTILE - 1 and len(ffn_out) < 4 * (c + 1):
            side.step()
        if c == 0:
            if n == NTILE - 1:
                drain_tail()
            while built.get(n, 0) < 2:
                (prep if prep.q else tail).step()
        oa = (oa0, oa1)[n % 2].bitcast(U32)
        unit(lambda k: jnp.concatenate([oa[k * KH + s] for s in range(KH)], axis=1),
             lambda k: ar_w[pl.ds((BO + (k * 2 + c) * HK) // 2, HK // 2), :], NN,
             lambda j, col, s: tail2.add(finish(j, col, s)))

    dots.update((count[0] + 1 + t, int(n)) for t, n in enumerate(DOT_PLAN))
    plan[:] = [OUT_PLAN, count[0]]
    delay[0] = 1
    q_unit(0, 0)
    soon(lambda: wait('ffn'))
    soon(lambda: ready.add('ffn'))
    q_unit(1, 0)
    for n in range(1, NTILE):
        for gp in range(2):
            q_unit(gp, n)
            o_unit(gp, n - 1)
    for c in range(2):
        o_unit(c, NTILE - 1)
    drain_tail()
    tail2.drain()
    for _ in range(2 * NTILE - 1):
        out_copy(0, 0, TT, 0, HK).wait()
    for _ in range(16):
        out_copy(0, 0, L, 0, L).wait()


@jax.jit
def pallas_recurrent_scan__linear_kernel_hedgehog__moe_arch_mod__prompt_kernel(
    A_x: jax.Array,
    A_wqkv: jax.Array,
    A_w_phi: jax.Array,
    A_wo: jax.Array,
    B_x: jax.Array,
    B_w_r: jax.Array,
    B_w_gate: jax.Array,
    B_w_up: jax.Array,
    B_w_down: jax.Array,
):
    del B_x
    hbm = pl.BlockSpec(memory_space=pl.ANY)
    return pl.pallas_call(
        _kernel,
        out_shape=jax.ShapeDtypeStruct(A_x.shape, A_x.dtype),
        in_specs=[hbm] * 8,
        out_specs=hbm,
        scratch_shapes=[
            pltpu.VMEM((ANCHOR + 8, D), BF),
            pltpu.VMEM((3 * NG, D, L), BF),
            pltpu.VMEM((H, DH, DH), BF),
            pltpu.VMEM((D,), BF),
            pltpu.VMEM((NG, L, L), BF),
            pltpu.VMEM((NPART + 1, 8, L), F32),
            pltpu.VMEM((65, 16, L), F32),
            pltpu.VMEM((SPARE + 16, L), BF),
            pltpu.VMEM((33, L, L), BF),
            pltpu.VMEM((OSPARE + 1, L, L), BF),
            pltpu.VMEM((OSPARE + 1, L, L), BF),
            pltpu.VMEM((NP, 80, L), BF),
            pltpu.VMEM((NP, 80, L), F32),
            pltpu.VMEM((S, D), BF),
            pltpu.VMEM((D, L), F32),
            pltpu.VMEM((NFC, FC, L), F32),
            pltpu.SemaphoreType.DMA((12,)),
        ],
        compiler_params=pltpu.CompilerParams(vmem_limit_bytes=120 << 20),
        name="hedgehog_mod",
    )(A_x, A_wqkv, A_w_phi, A_wo, B_w_r, B_w_gate, B_w_up, B_w_down)
```

```python
import jax
import jax.numpy as jnp
from jax import lax
import jax.experimental.pallas as pl
import jax.experimental.pallas.tpu as pltpu

BF = jnp.bfloat16
F32 = jnp.float32
U32 = jnp.uint32
NN = (((1,), (0,)), ((), ()))
NT = (((1,), (1,)), ((), ()))
LOG2E = 1.4426950408889634

S, D, H, DH, FF = 2048, 1024, 32, 32, 3584
L = 128
HK = D // 2
KH = HK // L
NG = H // 4
NP = H // 2
TT = 4 * L
NTILE = S // TT
FC = 4 * L
NFC = FF // FC
FROWS = 128
NSUB = HK // FROWS
EARLY = 3
NOP = 26
RAW = ((1, 26), (27, 2), (7, 8), (16, 28))
RAWL = ((26, 0), (3, 27), (7, 8), (28, 15))
STAGE = {k: i for i, k in enumerate(sum(RAWL, ()))}

XR = S // 4
XS = 0
AKV = XS + (NOP + 3) * KH * XR
AQ = AKV + NOP * KH * 4 * L
BO = AQ + NOP * KH * 2 * L
SPARE = BO + NOP * 2 * HK
GU = S
WD = GU + NFC * D
WO = WD + FF
ANCHOR = WO + D
OPART = (32 + 8 * NFC) * NSUB
NPART = OPART + 16 * NSUB
OSPARE = (NOP + 3) * KH

PIECES = {'.': (0, 0), 'L': (1, 0), '2': (2, 0), 'P': (0, 1), '3': (0, 2), '5': (0, 3), '9': (0, 8),
          'B': (1, 1), '6': (1, 2), 'E': (0, 0)}
FIRST_PLAN = '.935555555533355535535533P'
TILE0_PLAN = '.' * NOP + 'PP33PP3P33P333PP3PPPPP3PPP' '3B63BB6BBBB6B6P3BBB666PBB3' '2L2LLL22L22LL222LLLL2LLL2L'
NORM_PLAN = 'PBPLLPLPPPLLLL.L.LBLL.LL.P'
QUERY_PLAN = 'LBBBBBLBBBBB.BBBBBBBBBBLP.'
OUT_PLAN = ('L.L.LL.LLLL.LLLLLLLLL.LLL.' 'LBLLLL.LLLBPBPBLPPPPBPBPBB'
            '.LBP.LPLPLBPPLPBLPPPBLPPBP' 'LBLPLP.LLBPP.BBLBBLPL.LBL.'
            + ('LL.LLLLLBBPLPLP.BPLLPLPLBL' 'LPLLLBPLPBLPL.PLLBPLBLLBLL') * 4
            + 'LLLPLLBLBL.PLBLLPPLLPLLLBL' 'BBBLLLBPPBLPLBPPBPPPPPBPPP'
            'ELELELELLLELELELELLLEEEEEL' 'LEEEEEEEEEEEEEEEEEEEEEEEE.')
DOT_PLAN = ('11221121111111112211111222' '22111211211222112211121222'
            '12121211111111111111111111' '11111111111111121111111111'
            + ('11111112111211111112111121' '11211111111111111211111111') * 4
            + '11121211112211111211111111' '11211111111111111111111111'
            '11111111111111111111111111' '11111111111111111111111111')


def _dot(a, b, dims):
    return lax.dot_general(a, b, dims, preferred_element_type=F32)


def _unpack(words):
    return pltpu.bitcast(words, BF)


def _rnd(v):
    return v.astype(BF).astype(F32)


def _rcp(v):
    return pltpu.reciprocal(v, approx=True)


def _silu(v):
    h = 0.5 * v
    return h + h * jnp.tanh(h)


def _total(v):
    while len(v) > 1:
        v = [v[i] + v[i + 1] for i in range(0, len(v), 2)]
    return v[0]


def _pair_reduce(v, reduce, op):
    r = reduce(v, axis=0)
    r = op(r, pltpu.roll(r, 2, 0))
    return op(r, pltpu.roll(r, 4, 0))


def _dual_exp(p):
    v = p.reshape(8, 8, L)
    ep = jnp.exp2(v - _pair_reduce(v, jnp.max, jnp.maximum))
    en = jnp.exp2(_pair_reduce(v, jnp.min, jnp.minimum) - v)
    return ep, en, _pair_reduce(ep, jnp.sum, jnp.add), _pair_reduce(en, jnp.sum, jnp.add)


def _key_features(p):
    ep, en, sp, sn = _dual_exp(p)
    return jnp.concatenate([ep * _rcp(sp), en * _rcp(sn)], axis=0).reshape(L, L).astype(BF)


def _query_features(p):
    ep, en, sp, sn = _dual_exp(p)
    return jnp.concatenate([ep, en * (sp * _rcp(sn))], axis=0).reshape(L, L).astype(BF), sp


class _Signed:
    def __init__(self, sign, v):
        self.sign, self.v = sign, v

    def __neg__(self):
        return _Signed(-self.sign, self.v)

    def __add__(self, o):
        if self.sign == o.sign:
            return _Signed(self.sign, self.v + o.v)
        return _Signed(1, self.v - o.v if self.sign > 0 else o.v - self.v)

    def __sub__(self, o):
        return self + (-o)


def _nxt(k, d=1):
    return (k - 1 + d) % 3 + 1


def _operands(block, left):
    lo, hi = (1, 2) if left else (2, 1)

    def forms(i):
        x, y = block(i)
        if left:
            return {1: _Signed(1, x), 2: _Signed(-1, y), 3: _Signed(1, y - x)}
        return {1: _Signed(1, y), 2: _Signed(1, x), 3: _Signed(-1, x + y)}

    def diag(g, k):
        yield g[_nxt(k, lo)]
        yield g[_nxt(k, hi)]

    def pair(ga, gb, k, s):
        m = _nxt(k, 2)
        yield gb[k] - ga[_nxt(k)] if left else ga[_nxt(k)] - gb[k]
        for n in (_nxt(m, lo), _nxt(m, hi)):
            s[n] = ga[n] + gb[n]
            yield s[n]

    f0 = forms(0)
    yield from diag(f0, 1)
    f1 = forms(1)
    yield from diag(f1, 2)
    yield from pair(f0, f1, 1, {})
    f2 = forms(2)
    yield from diag(f2, 3)
    yield from pair(f1, f2, 2, {})
    s02 = {}
    yield from pair(f2, f0, 3, s02)
    s02[2] = f0[2] + f2[2]
    f3 = forms(3)
    yield from diag(f3, 1)
    yield from pair(f2, f3, 3, {})
    yield from pair(f3, s02, 1, {})
    yield from pair(f3, f1, 1, {})


_SIGNS = [a.sign * b.sign for a, b in zip(_operands(lambda i: (0, 0), True), _operands(lambda i: (0, 0), False))]


def _block_product(product):
    count = iter(range(NOP))

    def m(sign=1):
        k = next(count)
        return _Signed(sign * _SIGNS[k], product(k))

    def diag(i):
        x, y = m(), m(-1)
        yield i, i, x + y
        return x, y

    def pair(a, b, da, db, less=(None, None)):
        g = m()
        xs = m()
        ab = xs - da[1] - db[1] - g
        yield a, b, ab if less[0] is None else ab - less[0]
        ys = m(-1)
        ba = ys - da[0] - db[0] + g
        yield b, a, ba if less[1] is None else ba - less[1]
        return (xs, ys), (ab, ba)

    def steps():
        d0 = yield from diag(0)
        d1 = yield from diag(1)
        yield from pair(0, 1, d0, d1)
        d2 = yield from diag(2)
        yield from pair(1, 2, d1, d2)
        d02, _ = yield from pair(2, 0, d2, d0)
        d3 = yield from diag(3)
        _, (c23, c32) = yield from pair(2, 3, d2, d3)
        yield from pair(3, 0, d3, d02, (c32, c23))
        yield from pair(3, 1, d3, d1)

    for i, j, c in steps():
        assert c.sign > 0
        yield i, j, c.v


class _Tasks:
    def __init__(self):
        self.q = []

    def add(self, gen):
        self.q.append(gen)

    def step(self, n=1):
        while n > 0 and self.q:
            try:
                next(self.q[0])
                n -= 1
            except StopIteration:
                self.q.pop(0)

    def drain(self):
        while self.q:
            self.step()


def _kernel(x_hbm, wqkv_hbm, wphi_hbm, wo_hbm, wr_hbm, wg_hbm, wu_hbm, wd_hbm, out_hbm,
            wide, w_v, wphi_v, wr_v, fm_v, part, st, ar, stage, oa0, oa1, kvl, kv_acc, out_v, xb, ob, hb, sems):

    def x_rows(row0, rows):
        return x_hbm.at[0, pl.ds(row0, rows)], wide.at[pl.ds(row0, rows)]

    def w_cols(c):
        return wqkv_hbm.at[:, pl.ds(c * L, L)], w_v.at[c]

    def kv_cols(gp):
        return [w_cols(o + g) for g in (2 * gp, 2 * gp + 1) for o in (NG, 2 * NG)]

    def phi_heads(h0, heads):
        return wphi_hbm.at[pl.ds(h0, heads)], wphi_v.at[pl.ds(h0, heads)]

    def ffn_chunk(c):
        cols = pl.ds(c * FC, FC)
        rows = pl.ds(GU + c * D, D)
        return [(wg_hbm.at[:, cols], wide.at[rows, pl.ds(0, FC)]),
                (wu_hbm.at[:, cols], wide.at[rows, pl.ds(FC, FC)]),
                (wd_hbm.at[cols], wide.at[pl.ds(WD + c * FC, FC)])]

    loads = {
        'x00': [(wr_hbm, wr_v), x_rows(0, L)],
        'x01': [x_rows(L, L)],
        'x02': [x_rows(2 * L, L)],
        'x03': [x_rows(3 * L, L)],
        'kv0a': [phi_heads(0, 8)] + kv_cols(0)[:2],
        'kv0b': kv_cols(0)[2:],
        'kv1': [phi_heads(8, H - 8)] + kv_cols(1),
        'kv2': kv_cols(2),
        'kv3': [x_rows(TT, TT)] + kv_cols(3),
        'wo': [x_rows(n * TT, TT) for n in range(2, NTILE)] + [(wo_hbm, wide.at[pl.ds(WO, D)])],
        'wq': [w_cols(g) for g in range(NG)] + [p for c in range(EARLY) for p in ffn_chunk(c)],
        'ffn': [p for c in range(EARLY, NFC) for p in ffn_chunk(c)],
    }

    def copies(name):
        return [pltpu.make_async_copy(src, dst, sems.at[list(loads).index(name)]) for src, dst in loads[name]]

    def wait(name):
        for cp in copies(name):
            cp.wait()

    def out_copy(src0, dst0, rows, col0, cols, sem):
        return pltpu.make_async_copy(out_v.at[pl.ds(src0, rows), pl.ds(col0, cols)],
                                     out_hbm.at[0, pl.ds(dst0, rows), pl.ds(col0, cols)], sems.at[sem])

    for name in loads:
        for cp in copies(name):
            cp.start(priority=1)

    ar_w = ar.bitcast(U32)
    stored = set()
    ready = set()

    wait('x00')
    wr1 = wr_v[...].astype(F32).reshape(1, D)
    zero = pl.multiple_of(jnp.max(jnp.where(jnp.abs(wr1) < 0.0, pltpu.bitcast(wr1, jnp.int32), 0)), 16)
    never = zero > 0
    ar[pl.ds(SPARE, 16), :] = jnp.zeros((16, L), BF)
    part[NPART] = jnp.zeros((8, L), F32)
    st[64] = jnp.zeros((16, L), F32)
    stage[32, pl.ds(0, 16), :] = jnp.zeros((16, L), BF)
    for oa in (oa0, oa1):
        oa[OSPARE, pl.ds(0, 16), :] = jnp.zeros((16, L), BF)

    def fold_matrices(groups):
        rr = lax.broadcasted_iota(jnp.int32, (L, DH), 0)
        ff = lax.broadcasted_iota(jnp.int32, (L, DH), 1)
        sel = jnp.where(((rr & 63) >> 1) == ff, 1.0, 0.0).astype(BF)
        r2 = lax.broadcasted_iota(jnp.int32, (L, L), 0)
        c2 = lax.broadcasted_iota(jnp.int32, (L, L), 1)
        own = ((r2 >> 6) * 2 + (r2 & 1)) == (c2 >> 5)
        for g in groups:
            a = wphi_v[4 * g:4 * g + 4].reshape(L, DH)
            fm_v[g] = jnp.where(own, _dot(sel, a, NT), 0.0).astype(BF)

    def put(row, v):
        stored.add('ar')
        ar[pl.ds(row, v.shape[0]), :] = v.astype(BF)

    def slabs(start, stride, k, row0, rows):
        return jnp.concatenate(
            [ar_w[pl.ds((start + s * stride) // 2 + k * (KH * stride // 2) + row0, rows // 2), :]
             for s in range(KH)], axis=1)

    def folded(g, c, s):
        w = _unpack(w_v.bitcast(U32)[c, pl.ds(s * L // 2, L // 2), :])
        return _dot(_unpack(fm_v.bitcast(U32)[g]), w, NT) * (2.0 * LOG2E)

    def build(load, store, slots=range(NOP)):
        for r0 in range(0, L, 16):
            for k, v in enumerate(_operands(lambda i: [_unpack(load(k, r0)).astype(F32) for k in RAWL[i]], True)):
                if k in slots and k not in STAGE:
                    store(k, r0, v.v)
                if k == slots[-1]:
                    break
            yield

    def arena_build(row_of, slots=range(NOP)):
        return build(lambda k, r0: stage.bitcast(U32)[row_of(k)[1], pl.ds(r0 // 2, 8), :],
                     lambda k, r0, v: put(row_of(k)[0] + r0, v), slots)

    def put_plain(row_of, k, v):
        stored.add('stage')
        v = v.astype(BF)
        stage[row_of(k)[1]] = v
        if k < NOP:
            ar[pl.ds(row_of(k)[0], L), :] = v

    def kv_rows(gp, s):
        return lambda k: (AKV + ((k * KH + s) * 4 + gp) * L, 8 * s + STAGE.get(k, 0))

    def plain_kv(gp, s, which=(0, 1)):
        for i in which:
            g = 2 * gp + i
            for h in range(2):
                put_plain(kv_rows(gp, s), RAWL[2 * i][h], folded(g, NG + g, h * KH + s))
                put_plain(kv_rows(gp, s), RAWL[2 * i + 1][h], w_v[2 * NG + g, pl.ds(h * HK + s * L, L), :].T)

    def prep_kv(gp):
        for s in range(KH):
            plain_kv(gp, s)
            yield
            yield from arena_build(kv_rows(gp, s))

    def q_groups(gp):
        return (2 * gp, KH + 2 * gp, 2 * gp + 1, KH + 2 * gp + 1)

    def prep_q():
        for gp in range(2):
            for s in range(KH):
                def row_of(k):
                    return AQ + ((k * KH + s) * 2 + gp) * L, 8 * s + STAGE.get(k, 0)
                for i, g in enumerate(q_groups(gp)):
                    for h in range(2):
                        put_plain(row_of, RAWL[i][h], folded(g, g, h * KH + s))
                    if i % 2:
                        yield
                yield from arena_build(row_of)
            ready.add(('q', gp))

    def prep_o():
        for c in range(2):
            for r0 in range(0, HK, 16):
                blk = [wide[pl.ds(WO + h * HK + r0, 16), pl.ds(c * HK, HK)].astype(F32) for h in range(2)]
                for k, v in enumerate(_operands(lambda j: [b[:, j * L:(j + 1) * L] for b in blk], False)):
                    put(BO + (k * 2 + c) * HK + r0, v.v)
                yield

    wr = jnp.broadcast_to(wr1, (16, D))
    best = [jnp.full((16, 1), -jnp.inf, F32), jnp.zeros((16, 1), jnp.int32)]

    def row_mean(n, c, j):
        xf = wide[pl.ds(n * TT + j * L + c * 16, 16), :].astype(F32)
        mean = jnp.sum(xf, axis=1, keepdims=True) * (1.0 / D)
        stored.add('st')
        st[8 * c + 2 * j] = jnp.broadcast_to(mean, (16, L))

    def row_stats(n, c, j):
        r0 = n * TT + j * L + c * 16
        d = wide[pl.ds(r0, 16), :].astype(F32) - jnp.concatenate([st[8 * c + 2 * j]] * (D // L), axis=1)
        var = jnp.sum(d * d, axis=1, keepdims=True) * (1.0 / D)
        rs = _rcp(_rnd(jnp.sqrt(_rnd(_rnd(var) + 1e-5))))
        r = jnp.sum(d * wr, axis=1, keepdims=True) * rs
        up = (r > best[0]) | ((r == best[0]) & (r0 < best[1]))
        best[0] = jnp.where(up, r, best[0])
        best[1] = jnp.where(up, r0, best[1])
        stored.add('st')
        st[8 * c + 2 * j + 1] = jnp.broadcast_to(0.5 * rs, (16, L))
        st[64, pl.ds(8, 8), :] = jnp.broadcast_to(jnp.maximum(best[0][:8], best[0][8:]), (8, L))

    def token_operands(n, c, s):
        row = XS + s * XR + n * L + c * 16

        def block(j):
            b = [(wide[pl.ds(n * TT + j * L + c * 16, 16), pl.ds(h * HK + s * L, L)].astype(F32)
                  - st[8 * c + 2 * j]) * st[8 * c + 2 * j + 1] for h in range(2)]
            for k, v in zip(RAW[j], b):
                if k >= NOP:
                    put(row + k * KH * XR, v)
            return b

        for k, v in enumerate(_operands(block, False)):
            put(row + k * KH * XR, v.v)

    def layernorm(n):
        for j in range(4):
            row_mean(n, 0, j)
        yield
        for c in range(L // 16):
            for j in range(4):
                row_stats(n, c, j)
                if j % 2:
                    yield
            if c + 1 < L // 16:
                for j in range(4):
                    row_mean(n, c + 1, j)
                yield
            for s in range(KH):
                token_operands(n, c, s)
                yield

    side, prep, tail, tail2, extra = _Tasks(), _Tasks(), _Tasks(), _Tasks(), _Tasks()
    count = [0]
    plan = [FIRST_PLAN, 0]
    delay = [1]
    timed, pending, dots, flush = {}, [], {}, []
    release = [stage.at[32]]

    def anchor(v):
        wide[pl.ds(ANCHOR + zero, 8), pl.ds(0, 2 * L)] = v.astype(BF)

    def probe(name):
        if name == 'ar':
            return ar_w[pl.ds(SPARE // 2 + zero, 8), :]
        if name == 'part':
            return pltpu.bitcast(part[NPART + zero], U32)
        if name == 'st':
            return pltpu.bitcast(st[64, pl.ds(zero, 8), :], U32)
        if name == 'stage':
            return stage.bitcast(U32)[32, pl.ds(zero, 8), :]
        return (oa0, oa1)[name == 'oa1'].bitcast(U32)[OSPARE, pl.ds(zero, 8), :]

    def gap(m):
        count[0] += 1
        for action in timed.pop(count[0], ()):
            action()
        tied = pltpu.bitcast(m[96:104], U32)
        for name in sorted(pending.pop(0) if len(pending) > delay[0] else ()):
            tied = jnp.where(never, probe(name), tied)
        m = jnp.concatenate([m[:96], pltpu.bitcast(tied, F32), m[104:]], axis=0)
        if side.q or prep.q or extra.q:
            anchor(jnp.concatenate([m[:8], m[8:16]], axis=1))
        if prep.q:
            release[0][pl.ds(zero + 16, 16), :] = m[:16].astype(BF)
        tail.step(dots.get(count[0], 1))
        tail2.step()
        todo = plan[0][(count[0] - plan[1] - 1) % len(plan[0])]
        side.step(PIECES[todo][0])
        prep.step(PIECES[todo][1])
        extra.step(todo == 'E')
        pending.append(sorted(stored))
        stored.clear()
        return m

    def soon(action):
        timed.setdefault(count[0] + 1, []).append(action)

    def after(products, gen):
        start = count[0] + products

        def held():
            while count[0] < start and not flush:
                yield
            yield from gen
        return held()

    def drain_tail():
        flush.append(1)
        tail.drain()
        flush.clear()

    def unit(lhs, rhs, dims, on_block):
        for i, j, c in _block_product(lambda k: gap(_dot(_unpack(lhs(k)), _unpack(rhs(k)), dims))):
            on_block(i, j, c)

    route = {}

    def router():
        rmax = jnp.max(best[0])
        pos = best[1] + lax.broadcasted_iota(jnp.int32, (16, 1), 0)
        idx = jnp.min(jnp.where(best[0] == rmax, pos, S - 1))
        tile = idx // TT
        blk = (idx // L) % 4
        word = pl.multiple_of(((idx % L) // 16) * 8, 8)
        hit = lax.broadcasted_iota(jnp.int32, (16, HK), 0) == idx % 16
        route.update(rmax=rmax, idx=idx, tile=tile, block=blk, word=word)
        halves = []
        for h in range(2):
            k = sum(jnp.where(blk == j, RAW[j][h], 0) for j in range(4))
            rows = _unpack(slabs(XS, XR, k, tile * (L // 2) + word, 16)).astype(F32)
            row = 2.0 * jnp.sum(jnp.where(hit, rows, 0.0), axis=0, keepdims=True)
            halves.append(row)
            route['row'] = jnp.concatenate(halves, axis=1)
            for s in range(KH):
                xb[pl.ds(h * HK + s * L, L), :] = jnp.broadcast_to(row[:, s * L:(s + 1) * L], (L, L)).T
                yield

    def matvec(row0, col0, vec, k0, slot):
        vk = vec[pl.ds(k0, FROWS), :]
        wk = wide[pl.ds(row0 + k0, FROWS), pl.ds(col0, 2 * L)].astype(F32)
        pr = wk * jnp.concatenate([vk, vk], axis=1)
        acc = jnp.sum(pr.reshape(FROWS // 8, 8, 2 * L), axis=0)
        stored.add('part')
        for t in range(2):
            part[slot(t)] = acc[:, t * L:(t + 1) * L]

    def ffn():
        def gu_slot(c, t, p):
            return ((c % 2) * 8 + t) * 2 * NSUB + p

        def y_slot(c, t, p):
            return 32 * NSUB + (t * NFC + c) * NSUB + p

        def column(c, t):
            return jnp.sum(_total([part[gu_slot(c, t, p)] for p in range(2 * NSUB)]), axis=0, keepdims=True)

        def down(c):
            for t in range(0, 8, 2):
                for p in range(NSUB):
                    matvec(WD + c * FC, t * L, hb.at[c], p * FROWS, lambda u: y_slot(c, t + u, p))
                    yield

        for c in range(NFC):
            while c == EARLY and 'ffn' not in ready:
                yield
            for t in range(0, 8, 2):
                for p in range(2 * NSUB):
                    matvec(GU + c * D, t * L, xb, p * FROWS, lambda u: gu_slot(c, t + u, p))
                    yield
            for t in range(4):
                gate, up = column(c, t), column(c, 4 + t)
                hb[c, pl.ds(t * L, L), :] = jnp.broadcast_to(_silu(gate) * up, (L, L)).T
            yield
            if c > 0:
                yield from down(c - 1)
        yield
        yield from down(NFC - 1)
        y = [sum(_total([part[y_slot(c, t, p)] for p in range(NSUB)]) for c in range(NFC)) for t in range(8)]
        gate = 1.0 / (1.0 + jnp.exp(-jnp.full((1, D), route['rmax'], F32)))
        route['y'] = jnp.sum(jnp.concatenate(y, axis=1), axis=0, keepdims=True) * gate

    def kv_unit(gp, n):
        seen, acc = {}, {}

        def combine(g, phis, vts):
            for pp in range(2):
                p = 2 * g + pp
                acc[p] = acc.get(p, []) + [_dot(vts[pp], phis[pp], NT)]
                if len(acc[p]) == 4:
                    upd = _total(acc[p])
                    kv_acc[p] = upd if n == 0 else kv_acc[p] + upd
                yield

        def on_block(i, j, c):
            if i % 2:
                seen[i, j] = [jnp.concatenate([c[pp * 64:(pp + 1) * 64], jnp.ones((16, L), F32)], axis=0).astype(BF)
                              for pp in range(2)]
            else:
                seen[i, j] = [_key_features(c[pp * 64:(pp + 1) * 64]) for pp in range(2)]
            if (i ^ 1, j) in seen:
                tail.add(after(3, combine(2 * gp + i // 2, seen[i & 2, j], seen[i | 1, j])))

        def weights(k):
            while (gp, n) == (0, 0) and k in (7, 15) and k not in ready:
                prep.step()
            return slabs(AKV, 4 * L, k, gp * L // 2, L)

        unit(weights, lambda k: slabs(XS, XR, k, n * L // 2, L), NT, on_block)

    def first_tokens():
        for j in range(4):
            if j:
                wait(f'x0{j}')
            for part_of in (row_mean, row_stats):
                for c in range(L // 16):
                    part_of(0, c, j)
                anchor(jnp.zeros((8, 2 * L), BF))
        done = []
        for c in range(L // 16):
            for s in range(KH):
                if len(done) == 20:
                    wait('kv0a')
                    fold_matrices(range(2))
                    for t in range(KH):
                        plain_kv(0, t, (0,))
                        prep.add(arena_build(kv_rows(0, t), range(7)))
                if len(done) >= 3:
                    anchor(jnp.concatenate([done[-3], done[-3]], axis=1))
                token_operands(0, c, s)
                prep.step(2)
                done.append(pltpu.bitcast(probe('ar'), F32))
        prep.drain()

    def more_weights():
        while count[0] < 3:
            yield
        wait('kv0b')
        for s in range(KH):
            plain_kv(0, s, (1,))
            yield
        for slots in (range(7, 15), range(15, NOP)):
            for s in range(KH):
                yield from arena_build(kv_rows(0, s), slots)
            ready.add(slots[0])
        while count[0] < 16:
            yield
        wait('kv1')
        fold_matrices(range(2, NG))
        yield from prep_kv(1)

    def start_side_work(n, gp):
        if (n, gp) == (0, 1):
            wait('kv2')
            prep.add(prep_kv(2))
            plan[0] = TILE0_PLAN
        elif (n, gp) == (0, 2):
            wait('kv3')
            prep.add(prep_kv(3))
            side.add(layernorm(1))
        elif n > 0 and gp == 0:
            plan[0] = NORM_PLAN
            delay[0] = 2
            if n == 1:
                wait('wo')
                prep.add(prep_o())
            if n + 1 < NTILE:
                side.add(layernorm(n + 1))
            else:
                wait('wq')
                plan[0] = QUERY_PLAN
                side.add(router())
                side.add(ffn())
                prep.add(prep_q())

    first_tokens()
    prep.add(more_weights())
    for n in range(NTILE):
        for gp in range(4):
            if n == 0 and gp:
                prep.drain()
            if n and not gp:
                side.drain()
            soon(lambda n=n, gp=gp: start_side_work(n, gp))
            kv_unit(gp, n)

    def finish_kv():
        r = lax.broadcasted_iota(jnp.int32, (80, L), 0)
        c = lax.broadcasted_iota(jnp.int32, (80, L), 1)
        keep = jnp.where(r < 64, r >> 5, r & 1) == (c & 1)
        double = jnp.where(r < 64, 2.0, 1.0)
        for p in range(NP):
            kvl[p] = jnp.where(keep, kv_acc[p] * double, 0.0).astype(BF)
        yield

    tail.add(finish_kv())

    built = {}

    caught = [jnp.zeros((8, L), U32)] * (2 * KH)

    def catch_row(n, gp):
        for slab in (2 * gp, 2 * gp + 1):
            for h in range(2):
                k = sum(jnp.where(route['block'] == j, RAWL[j][h], 0) for j in range(4))
                words = (oa0, oa1)[n % 2].bitcast(U32)[k * KH + slab, pl.ds(route['word'], 8), :]
                caught[h * KH + slab] = jnp.where(route['tile'] == n, words, caught[h * KH + slab])

    def routed_projection():
        hit = lax.broadcasted_iota(jnp.int32, (16, L), 0) == route['idx'] % 16
        for t in range(2 * KH):
            row = jnp.sum(jnp.where(hit, _unpack(caught[t]).astype(F32), 0.0), axis=0, keepdims=True)
            ob[pl.ds(t * L, L), :] = jnp.broadcast_to(row, (L, L)).T
            if t % 2:
                yield
        for t in range(0, 8, 2):
            for p in range(2 * NSUB):
                matvec(WO, t * L, ob, p * FROWS, lambda u: OPART + (t + u) * 2 * NSUB + p)
                yield
        s = [_total([part[OPART + t * 2 * NSUB + p] for p in range(2 * NSUB)]) for t in range(8)]
        route['s'] = jnp.sum(jnp.concatenate(s, axis=1), axis=0, keepdims=True)

    def o_operands(n, gp):
        oa = (oa0, oa1)[n % 2]
        release[0] = oa.at[OSPARE]
        for slab in (2 * gp, 2 * gp + 1):
            def store(k, r0, v):
                stored.add(f'oa{n % 2}')
                oa[k * KH + slab, pl.ds(r0, 16), :] = v.astype(BF)
            yield from build(lambda k, r0: oa.bitcast(U32)[k * KH + slab, pl.ds(r0 // 2, 8), :], store)
        built[n] = built.get(n, 0) + 1

    def q_unit(gp, n):
        while ('q', gp) not in ready:
            prep.step()
        left = [16]
        oa = (oa0, oa1)[n % 2]

        def attend(i, j, feats):
            rows = []
            for pp, (phi, scale) in enumerate(feats):
                nd = _dot(_unpack(kvl.bitcast(U32)[2 * q_groups(gp)[i] + pp]), phi, NN)
                inv = _rcp(nd[64:72] + 1e-6 * scale)
                for head in range(2):
                    rd = jnp.broadcast_to(inv[head:head + 1], (8, L))
                    rows += [nd[head * DH + 8 * q:head * DH + 8 * q + 8] * rd for q in range(4)]
                if pp == 0:
                    yield
            oa[RAWL[j][i % 2] * KH + 2 * gp + i // 2] = jnp.concatenate(rows, axis=0).T.astype(BF)
            left[0] -= 1
            if not left[0]:
                catch_row(n, gp)
                prep.add(o_operands(n, gp))
                if (n, gp) == (NTILE - 1, 1):
                    extra.add(routed_projection())
            yield

        def on_block(i, j, c):
            tail.add(after(4, attend(i, j, [_query_features(c[pp * 64:(pp + 1) * 64]) for pp in range(2)])))

        unit(lambda k: slabs(AQ, 2 * L, k, gp * L // 2, L),
             lambda k: slabs(XS, XR, k, n * L // 2, L), NT, on_block)

    def o_unit(c, n):
        left = [16]

        def finish(j, col, s):
            rows = pl.ds(n * TT + j * L, L)
            cols = pl.ds(c * HK + col * L, L)
            half = _unpack(ar_w[pl.ds((XS + (RAW[j][c] * KH + col) * XR + n * L) // 2, L // 2), :]).astype(F32)
            sh = s * half
            out_v[rows, cols] = (wide[rows, cols].astype(F32) + sh + sh * jnp.tanh(half)).astype(BF)
            left[0] -= 1
            if (n, c) == (NTILE - 1, 1):
                out_copy(rows.start, rows.start, L, cols.start, L, 1).start()
            elif not left[0]:
                out_copy(n * TT, n * TT, TT, c * HK, HK, int(n == NTILE - 1)).start()
            yield

        if c == 0:
            if n == NTILE - 1:
                drain_tail()
            while built.get(n, 0) < 2:
                (prep if prep.q else tail).step()
        oa = (oa0, oa1)[n % 2].bitcast(U32)
        unit(lambda k: jnp.concatenate([oa[k * KH + s] for s in range(KH)], axis=1),
             lambda k: ar_w[pl.ds((BO + (k * 2 + c) * HK) // 2, HK // 2), :], NN,
             lambda j, col, s: tail2.add(finish(j, col, s)))

    dots.update((count[0] + 1 + t, int(n)) for t, n in enumerate(DOT_PLAN))
    plan[:] = [OUT_PLAN, count[0]]
    delay[0] = 1
    q_unit(0, 0)
    soon(lambda: wait('ffn'))
    soon(lambda: ready.add('ffn'))
    q_unit(1, 0)
    for n in range(1, NTILE):
        for gp in range(2):
            q_unit(gp, n)
            o_unit(gp, n - 1)
    for c in range(2):
        o_unit(c, NTILE - 1)
    drain_tail()
    tail2.drain()
    side.drain()
    extra.drain()

    row0 = pl.multiple_of((route['idx'] // 16) * 16, 16)
    half = 0.5 * (route['row'] + route['y'])
    sh = route['s'] * half
    fixed = wide[pl.ds(row0, 16), :].astype(F32) + (sh + sh * jnp.tanh(half))
    hit = lax.broadcasted_iota(jnp.int32, (16, D), 0) == route['idx'] % 16
    out_v[pl.ds(S, 16), :] = jnp.where(hit, fixed, out_v[pl.ds(row0, 16), :].astype(F32)).astype(BF)
    rows_copy = out_copy(S, row0, 16, 0, D, 2)
    for _ in range(2 * NTILE - 2):
        out_copy(0, 0, TT, 0, HK, 0).wait()
    pl.when(route['tile'] != NTILE - 1)(rows_copy.start)
    out_copy(0, 0, TT, 0, HK, 1).wait()
    for _ in range(16):
        out_copy(0, 0, L, 0, L, 1).wait()
    pl.when(route['tile'] == NTILE - 1)(rows_copy.start)
    rows_copy.wait()


@jax.jit
def pallas_recurrent_scan__linear_kernel_hedgehog__moe_arch_mod__prompt_kernel(
    A_x: jax.Array,
    A_wqkv: jax.Array,
    A_w_phi: jax.Array,
    A_wo: jax.Array,
    B_x: jax.Array,
    B_w_r: jax.Array,
    B_w_gate: jax.Array,
    B_w_up: jax.Array,
    B_w_down: jax.Array,
):
    del B_x
    hbm = pl.BlockSpec(memory_space=pl.ANY)
    return pl.pallas_call(
        _kernel,
        out_shape=jax.ShapeDtypeStruct(A_x.shape, A_x.dtype),
        in_specs=[hbm] * 8,
        out_specs=hbm,
        scratch_shapes=[
            pltpu.VMEM((ANCHOR + 8, D), BF),
            pltpu.VMEM((3 * NG, D, L), BF),
            pltpu.VMEM((H, DH, DH), BF),
            pltpu.VMEM((D,), BF),
            pltpu.VMEM((NG, L, L), BF),
            pltpu.VMEM((NPART + 1, 8, L), F32),
            pltpu.VMEM((65, 16, L), F32),
            pltpu.VMEM((SPARE + 16, L), BF),
            pltpu.VMEM((33, L, L), BF),
            pltpu.VMEM((OSPARE + 1, L, L), BF),
            pltpu.VMEM((OSPARE + 1, L, L), BF),
            pltpu.VMEM((NP, 80, L), BF),
            pltpu.VMEM((NP, 80, L), F32),
            pltpu.VMEM((S + 16, D), BF),
            pltpu.VMEM((D, L), F32),
            pltpu.VMEM((D, L), F32),
            pltpu.VMEM((NFC, FC, L), F32),
            pltpu.SemaphoreType.DMA((12,)),
        ],
        compiler_params=pltpu.CompilerParams(vmem_limit_bytes=120 << 20),
        name="hedgehog_mod",
    )(A_x, A_wqkv, A_w_phi, A_wo, B_w_r, B_w_gate, B_w_up, B_w_down)
```

```python
import jax
import jax.numpy as jnp
from jax import lax
import jax.experimental.pallas as pl
import jax.experimental.pallas.tpu as pltpu

BF = jnp.bfloat16
F32 = jnp.float32
U32 = jnp.uint32
NN = (((1,), (0,)), ((), ()))
NT = (((1,), (1,)), ((), ()))
LOG2E = 1.4426950408889634

S, D, H, DH, FF = 2048, 1024, 32, 32, 3584
L = 128
HK = D // 2
KH = HK // L
NG = H // 4
NP = H // 2
TT = 4 * L
NTILE = S // TT
FC = 4 * L
NFC = FF // FC
FROWS = 128
NSUB = HK // FROWS
EARLY = 3
NOP = 26
RAW = ((1, 26), (27, 2), (7, 8), (16, 28))
RAWL = ((26, 0), (3, 27), (7, 8), (28, 15))
STAGE = {k: i for i, k in enumerate(sum(RAWL, ()))}

XR = S // 4
XS = 0
AKV = XS + (NOP + 3) * KH * XR
AQ = AKV + NOP * KH * 4 * L
BO = AQ + NOP * KH * 2 * L
SPARE = BO + NOP * 2 * HK
GU = S
WD = GU + NFC * D
WO = WD + FF
ANCHOR = WO + D
OPART = (32 + 8 * NFC) * NSUB
NPART = OPART + 16 * NSUB
OSPARE = (NOP + 3) * KH

PIECES = {'.': (0, 0), 'L': (1, 0), '2': (2, 0), 'P': (0, 1), '3': (0, 2), '5': (0, 3), '9': (0, 8),
          'B': (1, 1), '6': (1, 2), 'E': (0, 0)}
FIRST_PLAN = '.935555555533355535535533P'
TILE0_PLAN = '.' * NOP + 'PP33PP3P33P333PP3PPPPP3PPP' '3B63BB6BBBB6B6P3BBB666PBB3' '2L2LLL22L22LL222LLLL2LLL2L'
NORM_PLAN = 'PBPLLPLPPPLLLL.L.LBLL.LL.P'
QUERY_PLAN = 'LBBBBBLBBBBB.BBBBBBBBBBLP.'
OUT_PLAN = ('L.L.LL.LLLL.LLLLLLLLL.LLL.' 'LBLLLL.LLLBPBPBLPPPPBPBPBB'
            '.LBP.LPLPLBPPLPBLPPPBLPPBP' 'LBLPLP.LLBPP.BBLBBLPL.LBL.'
            + ('LL.LLLLLBBPLPLP.BPLLPLPLBL' 'LPLLLBPLPBLPL.PLLBPLBLLBLL') * 4
            + 'LLLPLLBLBL.PLBLLPPLLPLLLBL' 'BBBLLLBPPBLPLBPPBPPPPPBPPP'
            'ELELELELLLELELELELLLEEEEEL' 'LEEEEEEEEEEEEEEEEEEEEEEEE.')
DOT_PLAN = ('11221121111111112211111222' '22111211211222112211121222'
            '12121211111111111111111111' '11111111111111121111111111'
            + ('11111112111211111112111121' '11211111111111111211111111') * 4
            + '11121211112211111211111111' '11211111111111111111111111'
            '11111111111111111111111111' '11111111111111111111111111')


def _dot(a, b, dims):
    return lax.dot_general(a, b, dims, preferred_element_type=F32)


def _unpack(words):
    return pltpu.bitcast(words, BF)


def _rnd(v):
    return v.astype(BF).astype(F32)


def _rcp(v):
    return pltpu.reciprocal(v, approx=True)


def _silu(v):
    h = 0.5 * v
    return h + h * jnp.tanh(h)


def _total(v):
    while len(v) > 1:
        v = [v[i] + v[i + 1] for i in range(0, len(v), 2)]
    return v[0]


def _pair_reduce(v, reduce, op):
    r = reduce(v, axis=0)
    r = op(r, pltpu.roll(r, 2, 0))
    return op(r, pltpu.roll(r, 4, 0))


def _dual_exp(p):
    v = p.reshape(8, 8, L)
    ep = jnp.exp2(v - _pair_reduce(v, jnp.max, jnp.maximum))
    en = jnp.exp2(_pair_reduce(v, jnp.min, jnp.minimum) - v)
    return ep, en, _pair_reduce(ep, jnp.sum, jnp.add), _pair_reduce(en, jnp.sum, jnp.add)


def _key_features(p):
    ep, en, sp, sn = _dual_exp(p)
    return jnp.concatenate([ep * _rcp(sp), en * _rcp(sn)], axis=0).reshape(L, L).astype(BF)


def _query_features(p):
    ep, en, sp, sn = _dual_exp(p)
    return jnp.concatenate([ep, en * (sp * _rcp(sn))], axis=0).reshape(L, L).astype(BF), sp


class _Signed:
    def __init__(self, sign, v):
        self.sign, self.v = sign, v

    def __neg__(self):
        return _Signed(-self.sign, self.v)

    def __add__(self, o):
        if self.sign == o.sign:
            return _Signed(self.sign, self.v + o.v)
        return _Signed(1, self.v - o.v if self.sign > 0 else o.v - self.v)

    def __sub__(self, o):
        return self + (-o)


def _nxt(k, d=1):
    return (k - 1 + d) % 3 + 1


def _operands(block, left):
    lo, hi = (1, 2) if left else (2, 1)

    def forms(i):
        x, y = block(i)
        if left:
            return {1: _Signed(1, x), 2: _Signed(-1, y), 3: _Signed(1, y - x)}
        return {1: _Signed(1, y), 2: _Signed(1, x), 3: _Signed(-1, x + y)}

    def diag(g, k):
        yield g[_nxt(k, lo)]
        yield g[_nxt(k, hi)]

    def pair(ga, gb, k, s):
        m = _nxt(k, 2)
        yield gb[k] - ga[_nxt(k)] if left else ga[_nxt(k)] - gb[k]
        for n in (_nxt(m, lo), _nxt(m, hi)):
            s[n] = ga[n] + gb[n]
            yield s[n]

    f0 = forms(0)
    yield from diag(f0, 1)
    f1 = forms(1)
    yield from diag(f1, 2)
    yield from pair(f0, f1, 1, {})
    f2 = forms(2)
    yield from diag(f2, 3)
    yield from pair(f1, f2, 2, {})
    s02 = {}
    yield from pair(f2, f0, 3, s02)
    s02[2] = f0[2] + f2[2]
    f3 = forms(3)
    yield from diag(f3, 1)
    yield from pair(f2, f3, 3, {})
    yield from pair(f3, s02, 1, {})
    yield from pair(f3, f1, 1, {})


_SIGNS = [a.sign * b.sign for a, b in zip(_operands(lambda i: (0, 0), True), _operands(lambda i: (0, 0), False))]


def _block_product(product):
    count = iter(range(NOP))

    def m(sign=1):
        k = next(count)
        return _Signed(sign * _SIGNS[k], product(k))

    def diag(i):
        x, y = m(), m(-1)
        yield i, i, x + y
        return x, y

    def pair(a, b, da, db, less=(None, None)):
        g = m()
        xs = m()
        ab = xs - da[1] - db[1] - g
        yield a, b, ab if less[0] is None else ab - less[0]
        ys = m(-1)
        ba = ys - da[0] - db[0] + g
        yield b, a, ba if less[1] is None else ba - less[1]
        return (xs, ys), (ab, ba)

    def steps():
        d0 = yield from diag(0)
        d1 = yield from diag(1)
        yield from pair(0, 1, d0, d1)
        d2 = yield from diag(2)
        yield from pair(1, 2, d1, d2)
        d02, _ = yield from pair(2, 0, d2, d0)
        d3 = yield from diag(3)
        _, (c23, c32) = yield from pair(2, 3, d2, d3)
        yield from pair(3, 0, d3, d02, (c32, c23))
        yield from pair(3, 1, d3, d1)

    for i, j, c in steps():
        assert c.sign > 0
        yield i, j, c.v


class _Tasks:
    def __init__(self):
        self.q = []

    def add(self, gen):
        self.q.append(gen)

    def step(self, n=1):
        while n > 0 and self.q:
            try:
                next(self.q[0])
                n -= 1
            except StopIteration:
                self.q.pop(0)

    def drain(self):
        while self.q:
            self.step()


def _kernel(x_hbm, wqkv_hbm, wphi_hbm, wo_hbm, wr_hbm, wg_hbm, wu_hbm, wd_hbm, out_hbm,
            wide, w_v, wphi_v, wr_v, fm_v, part, st, ar, stage, oa0, oa1, kvl, kv_acc, out_v, xb, ob, hb, sems):

    def x_rows(row0, rows):
        return x_hbm.at[0, pl.ds(row0, rows)], wide.at[pl.ds(row0, rows)]

    def w_cols(c):
        return wqkv_hbm.at[:, pl.ds(c * L, L)], w_v.at[c]

    def kv_cols(gp):
        return [w_cols(o + g) for g in (2 * gp, 2 * gp + 1) for o in (NG, 2 * NG)]

    def phi_heads(h0, heads):
        return wphi_hbm.at[pl.ds(h0, heads)], wphi_v.at[pl.ds(h0, heads)]

    def ffn_chunk(c):
        cols = pl.ds(c * FC, FC)
        rows = pl.ds(GU + c * D, D)
        return [(wg_hbm.at[:, cols], wide.at[rows, pl.ds(0, FC)]),
                (wu_hbm.at[:, cols], wide.at[rows, pl.ds(FC, FC)]),
                (wd_hbm.at[cols], wide.at[pl.ds(WD + c * FC, FC)])]

    loads = {
        'x00': [(wr_hbm, wr_v), x_rows(0, L)],
        'x01': [x_rows(L, L)],
        'x02': [x_rows(2 * L, L)],
        'x03': [x_rows(3 * L, L)],
        'kv0a': [phi_heads(0, 8)] + kv_cols(0)[:2],
        'kv0b': kv_cols(0)[2:],
        'kv1': [phi_heads(8, H - 8)] + kv_cols(1),
        'kv2': kv_cols(2),
        'kv3': [x_rows(TT, TT)] + kv_cols(3),
        'wo': [x_rows(n * TT, TT) for n in range(2, NTILE)] + [(wo_hbm, wide.at[pl.ds(WO, D)])],
        'wq': [w_cols(g) for g in range(NG)] + [p for c in range(EARLY) for p in ffn_chunk(c)],
        'ffn': [p for c in range(EARLY, NFC) for p in ffn_chunk(c)],
    }

    def copies(name):
        return [pltpu.make_async_copy(src, dst, sems.at[list(loads).index(name)]) for src, dst in loads[name]]

    def wait(name):
        for cp in copies(name):
            cp.wait()

    def out_copy(src0, dst0, rows, col0, cols, sem):
        return pltpu.make_async_copy(out_v.at[pl.ds(src0, rows), pl.ds(col0, cols)],
                                     out_hbm.at[0, pl.ds(dst0, rows), pl.ds(col0, cols)], sems.at[sem])

    for name in loads:
        for cp in copies(name):
            cp.start(priority=1)

    ar_w = ar.bitcast(U32)
    stored = set()
    ready = set()

    wait('x00')
    wr1 = wr_v[...].astype(F32).reshape(1, D)
    zero = pl.multiple_of(jnp.max(jnp.where(jnp.abs(wr1) < 0.0, pltpu.bitcast(wr1, jnp.int32), 0)), 16)
    never = zero > 0
    ar[pl.ds(SPARE, 16), :] = jnp.zeros((16, L), BF)
    part[NPART] = jnp.zeros((8, L), F32)
    st[64] = jnp.zeros((16, L), F32)
    stage[32, pl.ds(0, 16), :] = jnp.zeros((16, L), BF)
    for oa in (oa0, oa1):
        oa[OSPARE, pl.ds(0, 16), :] = jnp.zeros((16, L), BF)

    def fold_matrices(groups):
        rr = lax.broadcasted_iota(jnp.int32, (L, DH), 0)
        ff = lax.broadcasted_iota(jnp.int32, (L, DH), 1)
        sel = jnp.where(((rr & 63) >> 1) == ff, 1.0, 0.0).astype(BF)
        r2 = lax.broadcasted_iota(jnp.int32, (L, L), 0)
        c2 = lax.broadcasted_iota(jnp.int32, (L, L), 1)
        own = ((r2 >> 6) * 2 + (r2 & 1)) == (c2 >> 5)
        for g in groups:
            a = wphi_v[4 * g:4 * g + 4].reshape(L, DH)
            fm_v[g] = jnp.where(own, _dot(sel, a, NT), 0.0).astype(BF)

    def put(row, v):
        stored.add('ar')
        ar[pl.ds(row, v.shape[0]), :] = v.astype(BF)

    def slabs(start, stride, k, row0, rows):
        return jnp.concatenate(
            [ar_w[pl.ds((start + s * stride) // 2 + k * (KH * stride // 2) + row0, rows // 2), :]
             for s in range(KH)], axis=1)

    def folded(g, c, s):
        w = _unpack(w_v.bitcast(U32)[c, pl.ds(s * L // 2, L // 2), :])
        return _dot(_unpack(fm_v.bitcast(U32)[g]), w, NT) * (2.0 * LOG2E)

    def build(load, store, slots=range(NOP)):
        for r0 in range(0, L, 16):
            for k, v in enumerate(_operands(lambda i: [_unpack(load(k, r0)).astype(F32) for k in RAWL[i]], True)):
                if k in slots and k not in STAGE:
                    store(k, r0, v.v)
                if k == slots[-1]:
                    break
            yield

    def arena_build(row_of, slots=range(NOP)):
        return build(lambda k, r0: stage.bitcast(U32)[row_of(k)[1], pl.ds(r0 // 2, 8), :],
                     lambda k, r0, v: put(row_of(k)[0] + r0, v), slots)

    def put_plain(row_of, k, v):
        stored.add('stage')
        v = v.astype(BF)
        stage[row_of(k)[1]] = v
        if k < NOP:
            ar[pl.ds(row_of(k)[0], L), :] = v

    def kv_rows(gp, s):
        return lambda k: (AKV + ((k * KH + s) * 4 + gp) * L, 8 * s + STAGE.get(k, 0))

    def plain_kv(gp, s, which=(0, 1)):
        for i in which:
            g = 2 * gp + i
            for h in range(2):
                put_plain(kv_rows(gp, s), RAWL[2 * i][h], folded(g, NG + g, h * KH + s))
                put_plain(kv_rows(gp, s), RAWL[2 * i + 1][h], w_v[2 * NG + g, pl.ds(h * HK + s * L, L), :].T)

    def prep_kv(gp):
        for s in range(KH):
            plain_kv(gp, s)
            yield
            yield from arena_build(kv_rows(gp, s))

    def q_groups(gp):
        return (2 * gp, KH + 2 * gp, 2 * gp + 1, KH + 2 * gp + 1)

    def prep_q():
        for gp in range(2):
            for s in range(KH):
                def row_of(k):
                    return AQ + ((k * KH + s) * 2 + gp) * L, 8 * s + STAGE.get(k, 0)
                for i, g in enumerate(q_groups(gp)):
                    for h in range(2):
                        put_plain(row_of, RAWL[i][h], folded(g, g, h * KH + s))
                    if i % 2:
                        yield
                yield from arena_build(row_of)
            ready.add(('q', gp))

    def prep_o():
        for c in range(2):
            for r0 in range(0, HK, 16):
                blk = [wide[pl.ds(WO + h * HK + r0, 16), pl.ds(c * HK, HK)].astype(F32) for h in range(2)]
                for k, v in enumerate(_operands(lambda j: [b[:, j * L:(j + 1) * L] for b in blk], False)):
                    put(BO + (k * 2 + c) * HK + r0, v.v)
                yield

    wr = jnp.broadcast_to(wr1, (16, D))
    best = [jnp.full((16, 1), -jnp.inf, F32), jnp.zeros((16, 1), jnp.int32)]

    def row_mean(n, c, j):
        xf = wide[pl.ds(n * TT + j * L + c * 16, 16), :].astype(F32)
        mean = jnp.sum(xf, axis=1, keepdims=True) * (1.0 / D)
        stored.add('st')
        st[8 * c + 2 * j] = jnp.broadcast_to(mean, (16, L))

    def row_stats(n, c, j):
        r0 = n * TT + j * L + c * 16
        d = wide[pl.ds(r0, 16), :].astype(F32) - jnp.concatenate([st[8 * c + 2 * j]] * (D // L), axis=1)
        var = jnp.sum(d * d, axis=1, keepdims=True) * (1.0 / D)
        rs = _rcp(_rnd(jnp.sqrt(_rnd(_rnd(var) + 1e-5))))
        r = jnp.sum(d * wr, axis=1, keepdims=True) * rs
        up = (r > best[0]) | ((r == best[0]) & (r0 < best[1]))
        best[0] = jnp.where(up, r, best[0])
        best[1] = jnp.where(up, r0, best[1])
        stored.add('st')
        st[8 * c + 2 * j + 1] = jnp.broadcast_to(0.5 * rs, (16, L))
        st[64, pl.ds(8, 8), :] = jnp.broadcast_to(jnp.maximum(best[0][:8], best[0][8:]), (8, L))

    def token_operands(n, c, s):
        row = XS + s * XR + n * L + c * 16

        def block(j):
            b = [(wide[pl.ds(n * TT + j * L + c * 16, 16), pl.ds(h * HK + s * L, L)].astype(F32)
                  - st[8 * c + 2 * j]) * st[8 * c + 2 * j + 1] for h in range(2)]
            for k, v in zip(RAW[j], b):
                if k >= NOP:
                    put(row + k * KH * XR, v)
            return b

        for k, v in enumerate(_operands(block, False)):
            put(row + k * KH * XR, v.v)

    def layernorm(n):
        for j in range(4):
            row_mean(n, 0, j)
        yield
        for c in range(L // 16):
            for j in range(4):
                row_stats(n, c, j)
                if j % 2:
                    yield
            if c + 1 < L // 16:
                for j in range(4):
                    row_mean(n, c + 1, j)
                yield
            for s in range(KH):
                token_operands(n, c, s)
                yield

    side, prep, tail, tail2, extra = _Tasks(), _Tasks(), _Tasks(), _Tasks(), _Tasks()
    count = [0]
    plan = [FIRST_PLAN, 0]
    delay = [1]
    timed, pending, dots, flush = {}, [], {}, []
    release = [stage.at[32]]

    def anchor(v):
        wide[pl.ds(ANCHOR + zero, 8), pl.ds(0, 2 * L)] = v.astype(BF)

    def probe(name):
        if name == 'ar':
            return ar_w[pl.ds(SPARE // 2 + zero, 8), :]
        if name == 'part':
            return pltpu.bitcast(part[NPART + zero], U32)
        if name == 'st':
            return pltpu.bitcast(st[64, pl.ds(zero, 8), :], U32)
        if name == 'stage':
            return stage.bitcast(U32)[32, pl.ds(zero, 8), :]
        return (oa0, oa1)[name == 'oa1'].bitcast(U32)[OSPARE, pl.ds(zero, 8), :]

    def gap(m):
        count[0] += 1
        for action in timed.pop(count[0], ()):
            action()
        tied = pltpu.bitcast(m[96:104], U32)
        for name in sorted(pending.pop(0) if len(pending) > delay[0] else ()):
            tied = jnp.where(never, probe(name), tied)
        m = jnp.concatenate([m[:96], pltpu.bitcast(tied, F32), m[104:]], axis=0)
        if side.q or prep.q or extra.q:
            anchor(jnp.concatenate([m[:8], m[8:16]], axis=1))
        if prep.q:
            release[0][pl.ds(zero + 16, 16), :] = m[:16].astype(BF)
        tail.step(dots.get(count[0], 1))
        tail2.step()
        todo = plan[0][(count[0] - plan[1] - 1) % len(plan[0])]
        side.step(PIECES[todo][0])
        prep.step(PIECES[todo][1])
        extra.step(todo == 'E')
        pending.append(sorted(stored))
        stored.clear()
        return m

    def soon(action):
        timed.setdefault(count[0] + 1, []).append(action)

    def after(products, gen):
        start = count[0] + products

        def held():
            while count[0] < start and not flush:
                yield
            yield from gen
        return held()

    def drain_tail():
        flush.append(1)
        tail.drain()
        flush.clear()

    def unit(lhs, rhs, dims, on_block):
        for i, j, c in _block_product(lambda k: gap(_dot(_unpack(lhs(k)), _unpack(rhs(k)), dims))):
            on_block(i, j, c)

    route = {}

    def router():
        slot = lax.broadcasted_iota(jnp.int32, (16, 1), 0)
        lane_rows = lax.broadcasted_iota(jnp.int32, (16, D), 0)
        rows = jnp.zeros((16, D), F32)
        for i in range(16):
            group = pl.multiple_of(jnp.max(jnp.where(slot == i, best[1], 0)), 16)
            rows = jnp.where(lane_rows == i, wide[pl.ds(group, 16), :].astype(F32), rows)
        mean = jnp.sum(rows, axis=1, keepdims=True) * (1.0 / D)
        var = jnp.sum((rows - mean) * (rows - mean), axis=1, keepdims=True) * (1.0 / D)
        xn = _rnd(_rnd(rows - _rnd(mean)) / _rnd(jnp.sqrt(_rnd(_rnd(var) + 1e-5))))
        score = _rnd(jnp.sum(xn * wr, axis=1, keepdims=True))
        rmax = jnp.max(score)
        idx = jnp.min(jnp.where(score == rmax, best[1] + slot, S - 1))
        row = jnp.sum(jnp.where(lane_rows == idx % 16, xn, 0.0), axis=0, keepdims=True)
        route.update(rmax=rmax, idx=idx, row=row, tile=idx // TT, block=(idx // L) % 4,
                     word=pl.multiple_of(((idx % L) // 16) * 8, 8))
        for t in range(D // L):
            xb[pl.ds(t * L, L), :] = jnp.broadcast_to(row[:, t * L:(t + 1) * L], (L, L)).T
            yield

    def matvec(row0, col0, vec, k0, slot):
        vk = vec[pl.ds(k0, FROWS), :]
        wk = wide[pl.ds(row0 + k0, FROWS), pl.ds(col0, 2 * L)].astype(F32)
        pr = wk * jnp.concatenate([vk, vk], axis=1)
        acc = jnp.sum(pr.reshape(FROWS // 8, 8, 2 * L), axis=0)
        stored.add('part')
        for t in range(2):
            part[slot(t)] = acc[:, t * L:(t + 1) * L]

    def ffn():
        def gu_slot(c, t, p):
            return ((c % 2) * 8 + t) * 2 * NSUB + p

        def y_slot(c, t, p):
            return 32 * NSUB + (t * NFC + c) * NSUB + p

        def column(c, t):
            return jnp.sum(_total([part[gu_slot(c, t, p)] for p in range(2 * NSUB)]), axis=0, keepdims=True)

        def down(c):
            for t in range(0, 8, 2):
                for p in range(NSUB):
                    matvec(WD + c * FC, t * L, hb.at[c], p * FROWS, lambda u: y_slot(c, t + u, p))
                    yield

        for c in range(NFC):
            while c == EARLY and 'ffn' not in ready:
                yield
            for t in range(0, 8, 2):
                for p in range(2 * NSUB):
                    matvec(GU + c * D, t * L, xb, p * FROWS, lambda u: gu_slot(c, t + u, p))
                    yield
            for t in range(4):
                gate, up = column(c, t), column(c, 4 + t)
                hb[c, pl.ds(t * L, L), :] = jnp.broadcast_to(_silu(gate) * up, (L, L)).T
            yield
            if c > 0:
                yield from down(c - 1)
        yield
        yield from down(NFC - 1)
        y = [sum(_total([part[y_slot(c, t, p)] for p in range(NSUB)]) for c in range(NFC)) for t in range(8)]
        gate = 1.0 / (1.0 + jnp.exp(-jnp.full((1, D), route['rmax'], F32)))
        route['y'] = jnp.sum(jnp.concatenate(y, axis=1), axis=0, keepdims=True) * gate

    def kv_unit(gp, n):
        seen, acc = {}, {}

        def combine(g, phis, vts):
            for pp in range(2):
                p = 2 * g + pp
                acc[p] = acc.get(p, []) + [_dot(vts[pp], phis[pp], NT)]
                if len(acc[p]) == 4:
                    upd = _total(acc[p])
                    kv_acc[p] = upd if n == 0 else kv_acc[p] + upd
                yield

        def on_block(i, j, c):
            if i % 2:
                seen[i, j] = [jnp.concatenate([c[pp * 64:(pp + 1) * 64], jnp.ones((16, L), F32)], axis=0).astype(BF)
                              for pp in range(2)]
            else:
                seen[i, j] = [_key_features(c[pp * 64:(pp + 1) * 64]) for pp in range(2)]
            if (i ^ 1, j) in seen:
                tail.add(after(3, combine(2 * gp + i // 2, seen[i & 2, j], seen[i | 1, j])))

        def weights(k):
            while (gp, n) == (0, 0) and k in (7, 15) and k not in ready:
                prep.step()
            return slabs(AKV, 4 * L, k, gp * L // 2, L)

        unit(weights, lambda k: slabs(XS, XR, k, n * L // 2, L), NT, on_block)

    def first_tokens():
        for j in range(4):
            if j:
                wait(f'x0{j}')
            for part_of in (row_mean, row_stats):
                for c in range(L // 16):
                    part_of(0, c, j)
                anchor(jnp.zeros((8, 2 * L), BF))
        done = []
        for c in range(L // 16):
            for s in range(KH):
                if len(done) == 20:
                    wait('kv0a')
                    fold_matrices(range(2))
                    for t in range(KH):
                        plain_kv(0, t, (0,))
                        prep.add(arena_build(kv_rows(0, t), range(7)))
                if len(done) >= 3:
                    anchor(jnp.concatenate([done[-3], done[-3]], axis=1))
                token_operands(0, c, s)
                prep.step(2)
                done.append(pltpu.bitcast(probe('ar'), F32))
        prep.drain()

    def more_weights():
        while count[0] < 3:
            yield
        wait('kv0b')
        for s in range(KH):
            plain_kv(0, s, (1,))
            yield
        for slots in (range(7, 15), range(15, NOP)):
            for s in range(KH):
                yield from arena_build(kv_rows(0, s), slots)
            ready.add(slots[0])
        while count[0] < 16:
            yield
        wait('kv1')
        fold_matrices(range(2, NG))
        yield from prep_kv(1)

    def start_side_work(n, gp):
        if (n, gp) == (0, 1):
            wait('kv2')
            prep.add(prep_kv(2))
            plan[0] = TILE0_PLAN
        elif (n, gp) == (0, 2):
            wait('kv3')
            prep.add(prep_kv(3))
            side.add(layernorm(1))
        elif n > 0 and gp == 0:
            plan[0] = NORM_PLAN
            delay[0] = 2
            if n == 1:
                wait('wo')
                prep.add(prep_o())
            if n + 1 < NTILE:
                side.add(layernorm(n + 1))
            else:
                wait('wq')
                plan[0] = QUERY_PLAN
                side.add(router())
                side.add(ffn())
                prep.add(prep_q())

    first_tokens()
    prep.add(more_weights())
    for n in range(NTILE):
        for gp in range(4):
            if n == 0 and gp:
                prep.drain()
            if n and not gp:
                side.drain()
            soon(lambda n=n, gp=gp: start_side_work(n, gp))
            kv_unit(gp, n)

    def finish_kv():
        r = lax.broadcasted_iota(jnp.int32, (80, L), 0)
        c = lax.broadcasted_iota(jnp.int32, (80, L), 1)
        keep = jnp.where(r < 64, r >> 5, r & 1) == (c & 1)
        double = jnp.where(r < 64, 2.0, 1.0)
        for p in range(NP):
            kvl[p] = jnp.where(keep, kv_acc[p] * double, 0.0).astype(BF)
        yield

    tail.add(finish_kv())

    built = {}

    caught = [jnp.zeros((8, L), U32)] * (2 * KH)

    def catch_row(n, gp):
        for slab in (2 * gp, 2 * gp + 1):
            for h in range(2):
                k = sum(jnp.where(route['block'] == j, RAWL[j][h], 0) for j in range(4))
                words = (oa0, oa1)[n % 2].bitcast(U32)[k * KH + slab, pl.ds(route['word'], 8), :]
                caught[h * KH + slab] = jnp.where(route['tile'] == n, words, caught[h * KH + slab])

    def routed_projection():
        hit = lax.broadcasted_iota(jnp.int32, (16, L), 0) == route['idx'] % 16
        for t in range(2 * KH):
            row = jnp.sum(jnp.where(hit, _unpack(caught[t]).astype(F32), 0.0), axis=0, keepdims=True)
            ob[pl.ds(t * L, L), :] = jnp.broadcast_to(row, (L, L)).T
            if t % 2:
                yield
        for t in range(0, 8, 2):
            for p in range(2 * NSUB):
                matvec(WO, t * L, ob, p * FROWS, lambda u: OPART + (t + u) * 2 * NSUB + p)
                yield
        s = [_total([part[OPART + t * 2 * NSUB + p] for p in range(2 * NSUB)]) for t in range(8)]
        route['s'] = jnp.sum(jnp.concatenate(s, axis=1), axis=0, keepdims=True)

    def o_operands(n, gp):
        oa = (oa0, oa1)[n % 2]
        release[0] = oa.at[OSPARE]
        for slab in (2 * gp, 2 * gp + 1):
            def store(k, r0, v):
                stored.add(f'oa{n % 2}')
                oa[k * KH + slab, pl.ds(r0, 16), :] = v.astype(BF)
            yield from build(lambda k, r0: oa.bitcast(U32)[k * KH + slab, pl.ds(r0 // 2, 8), :], store)
        built[n] = built.get(n, 0) + 1

    def q_unit(gp, n):
        while ('q', gp) not in ready:
            prep.step()
        left = [16]
        oa = (oa0, oa1)[n % 2]

        def attend(i, j, feats):
            rows = []
            for pp, (phi, scale) in enumerate(feats):
                nd = _dot(_unpack(kvl.bitcast(U32)[2 * q_groups(gp)[i] + pp]), phi, NN)
                inv = _rcp(nd[64:72] + 1e-6 * scale)
                for head in range(2):
                    rd = jnp.broadcast_to(inv[head:head + 1], (8, L))
                    rows += [nd[head * DH + 8 * q:head * DH + 8 * q + 8] * rd for q in range(4)]
                if pp == 0:
                    yield
            oa[RAWL[j][i % 2] * KH + 2 * gp + i // 2] = jnp.concatenate(rows, axis=0).T.astype(BF)
            left[0] -= 1
            if not left[0]:
                catch_row(n, gp)
                prep.add(o_operands(n, gp))
                if (n, gp) == (NTILE - 1, 1):
                    extra.add(routed_projection())
            yield

        def on_block(i, j, c):
            tail.add(after(4, attend(i, j, [_query_features(c[pp * 64:(pp + 1) * 64]) for pp in range(2)])))

        unit(lambda k: slabs(AQ, 2 * L, k, gp * L // 2, L),
             lambda k: slabs(XS, XR, k, n * L // 2, L), NT, on_block)

    def o_unit(c, n):
        left = [16]

        def finish(j, col, s):
            rows = pl.ds(n * TT + j * L, L)
            cols = pl.ds(c * HK + col * L, L)
            half = _unpack(ar_w[pl.ds((XS + (RAW[j][c] * KH + col) * XR + n * L) // 2, L // 2), :]).astype(F32)
            sh = s * half
            out_v[rows, cols] = (wide[rows, cols].astype(F32) + sh + sh * jnp.tanh(half)).astype(BF)
            left[0] -= 1
            if (n, c) == (NTILE - 1, 1):
                out_copy(rows.start, rows.start, L, cols.start, L, 1).start()
            elif not left[0]:
                out_copy(n * TT, n * TT, TT, c * HK, HK, int(n == NTILE - 1)).start()
            yield

        if c == 0:
            if n == NTILE - 1:
                drain_tail()
            while built.get(n, 0) < 2:
                (prep if prep.q else tail).step()
        oa = (oa0, oa1)[n % 2].bitcast(U32)
        unit(lambda k: jnp.concatenate([oa[k * KH + s] for s in range(KH)], axis=1),
             lambda k: ar_w[pl.ds((BO + (k * 2 + c) * HK) // 2, HK // 2), :], NN,
             lambda j, col, s: tail2.add(finish(j, col, s)))

    dots.update((count[0] + 1 + t, int(n)) for t, n in enumerate(DOT_PLAN))
    plan[:] = [OUT_PLAN, count[0]]
    delay[0] = 1
    q_unit(0, 0)
    soon(lambda: wait('ffn'))
    soon(lambda: ready.add('ffn'))
    q_unit(1, 0)
    for n in range(1, NTILE):
        for gp in range(2):
            q_unit(gp, n)
            o_unit(gp, n - 1)
    for c in range(2):
        o_unit(c, NTILE - 1)
    drain_tail()
    tail2.drain()
    side.drain()
    extra.drain()

    row0 = pl.multiple_of((route['idx'] // 16) * 16, 16)
    half = 0.5 * (route['row'] + route['y'])
    sh = route['s'] * half
    fixed = wide[pl.ds(row0, 16), :].astype(F32) + (sh + sh * jnp.tanh(half))
    hit = lax.broadcasted_iota(jnp.int32, (16, D), 0) == route['idx'] % 16
    out_v[pl.ds(S, 16), :] = jnp.where(hit, fixed, out_v[pl.ds(row0, 16), :].astype(F32)).astype(BF)
    rows_copy = out_copy(S, row0, 16, 0, D, 2)
    for _ in range(2 * NTILE - 2):
        out_copy(0, 0, TT, 0, HK, 0).wait()
    pl.when(route['tile'] != NTILE - 1)(rows_copy.start)
    out_copy(0, 0, TT, 0, HK, 1).wait()
    for _ in range(16):
        out_copy(0, 0, L, 0, L, 1).wait()
    pl.when(route['tile'] == NTILE - 1)(rows_copy.start)
    rows_copy.wait()


@jax.jit
def pallas_recurrent_scan__linear_kernel_hedgehog__moe_arch_mod__prompt_kernel(
    A_x: jax.Array,
    A_wqkv: jax.Array,
    A_w_phi: jax.Array,
    A_wo: jax.Array,
    B_x: jax.Array,
    B_w_r: jax.Array,
    B_w_gate: jax.Array,
    B_w_up: jax.Array,
    B_w_down: jax.Array,
):
    del B_x
    hbm = pl.BlockSpec(memory_space=pl.ANY)
    return pl.pallas_call(
        _kernel,
        out_shape=jax.ShapeDtypeStruct(A_x.shape, A_x.dtype),
        in_specs=[hbm] * 8,
        out_specs=hbm,
        scratch_shapes=[
            pltpu.VMEM((ANCHOR + 8, D), BF),
            pltpu.VMEM((3 * NG, D, L), BF),
            pltpu.VMEM((H, DH, DH), BF),
            pltpu.VMEM((D,), BF),
            pltpu.VMEM((NG, L, L), BF),
            pltpu.VMEM((NPART + 1, 8, L), F32),
            pltpu.VMEM((65, 16, L), F32),
            pltpu.VMEM((SPARE + 16, L), BF),
            pltpu.VMEM((33, L, L), BF),
            pltpu.VMEM((OSPARE + 1, L, L), BF),
            pltpu.VMEM((OSPARE + 1, L, L), BF),
            pltpu.VMEM((NP, 80, L), BF),
            pltpu.VMEM((NP, 80, L), F32),
            pltpu.VMEM((S + 16, D), BF),
            pltpu.VMEM((D, L), F32),
            pltpu.VMEM((D, L), F32),
            pltpu.VMEM((NFC, FC, L), F32),
            pltpu.SemaphoreType.DMA((12,)),
        ],
        compiler_params=pltpu.CompilerParams(vmem_limit_bytes=120 << 20),
        name="hedgehog_mod",
    )(A_x, A_wqkv, A_w_phi, A_wo, B_w_r, B_w_gate, B_w_up, B_w_down)
```

```python
import jax
import jax.numpy as jnp
from jax import lax
import jax.experimental.pallas as pl
import jax.experimental.pallas.tpu as pltpu

BF = jnp.bfloat16
F32 = jnp.float32
U32 = jnp.uint32
NN = (((1,), (0,)), ((), ()))
NT = (((1,), (1,)), ((), ()))
LOG2E = 1.4426950408889634

S, D, H, DH, FF = 2048, 1024, 32, 32, 3584
L = 128
HK = D // 2
KH = HK // L
NG = H // 4
NP = H // 2
TT = 4 * L
NTILE = S // TT
FC = 4 * L
NFC = FF // FC
FROWS = 128
NSUB = HK // FROWS
EARLY = 3
NOP = 26
RAW = ((1, 26), (27, 2), (7, 8), (16, 28))
RAWL = ((26, 0), (3, 27), (7, 8), (28, 15))
STAGE = {k: i for i, k in enumerate(sum(RAWL, ()))}

XR = S // 4
XS = 0
AKV = XS + (NOP + 3) * KH * XR
AQ = AKV + NOP * KH * 4 * L
BO = AQ + NOP * KH * 2 * L
SPARE = BO + NOP * 2 * HK
GU = S
WD = GU + NFC * D
WO = WD + FF
ANCHOR = WO + D
OPART = (32 + 8 * NFC) * NSUB
NPART = OPART + 16 * NSUB
OSPARE = (NOP + 3) * KH

PIECES = {'.': (0, 0), 'L': (1, 0), '2': (2, 0), 'P': (0, 1), '3': (0, 2), '5': (0, 3), '9': (0, 8),
          'B': (1, 1), '6': (1, 2), 'E': (0, 0)}
FIRST_PLAN = '.935555555533355535535533P'
TILE0_PLAN = '.' * NOP + 'PP33PP3P33P333PP3PPPPP3PPP' '3B63BB6BBBB6B6P3BBB666PBB3' '2L2LLL22L22LL222LLLL2LLL2L'
NORM_PLAN = 'PBPLLPLPPPLLLL.L.LBLL.LL.P'
QUERY_PLAN = 'LBBBBBLBBBBB.BBBBBBBBBBLP.'
OUT_PLAN = ('L.L.LL.LLLL.LLLLLLLLL.LLL.' 'LBLLLL.LLLBPBPBLPPPPBPBPBB'
            '.LBP.LPLPLBPPLPBLPPPBLPPBP' 'LBLPLP.LLBPP.BBLBBLPL.LBL.'
            + ('LL.LLLLLBBPLPLP.BPLLPLPLBL' 'LPLLLBPLPBLPL.PLLBPLBLLBLL') * 4
            + 'LLLPLLBLBL.PLBLLPPLLPLLLBL' 'BBBLLLBPPBLPLBPPBPPPPPBPPP'
            'ELELELELLLELELELELLLEEEEEL' 'LEEEEEEEEEEEEEEEEEEEEEEEE.')
DOT_PLAN = ('11221121111111112211111222' '22111211211222112211121222'
            '12121211111111111111111111' '11111111111111121111111111'
            + ('11111112111211111112111121' '11211111111111111211111111') * 4
            + '11121211112211111211111111' '11211111111111111111111111'
            '11111111111111111111111111' '11111111111111111111111111')


def _dot(a, b, dims):
    return lax.dot_general(a, b, dims, preferred_element_type=F32)


def _unpack(words):
    return pltpu.bitcast(words, BF)


def _rnd(v):
    return v.astype(BF).astype(F32)


def _rcp(v):
    return pltpu.reciprocal(v, approx=True)


def _silu(v):
    h = 0.5 * v
    return h + h * jnp.tanh(h)


def _total(v):
    while len(v) > 1:
        v = [v[i] + v[i + 1] for i in range(0, len(v), 2)]
    return v[0]


def _pair_reduce(v, reduce, op):
    r = reduce(v, axis=0)
    r = op(r, pltpu.roll(r, 2, 0))
    return op(r, pltpu.roll(r, 4, 0))


def _dual_exp(p):
    v = p.reshape(8, 8, L)
    ep = jnp.exp2(v - _pair_reduce(v, jnp.max, jnp.maximum))
    en = jnp.exp2(_pair_reduce(v, jnp.min, jnp.minimum) - v)
    return ep, en, _pair_reduce(ep, jnp.sum, jnp.add), _pair_reduce(en, jnp.sum, jnp.add)


def _key_features(p):
    ep, en, sp, sn = _dual_exp(p)
    return jnp.concatenate([ep * _rcp(sp), en * _rcp(sn)], axis=0).reshape(L, L).astype(BF)


def _query_features(p):
    ep, en, sp, sn = _dual_exp(p)
    return jnp.concatenate([ep, en * (sp * _rcp(sn))], axis=0).reshape(L, L).astype(BF), sp


class _Signed:
    def __init__(self, sign, v):
        self.sign, self.v = sign, v

    def __neg__(self):
        return _Signed(-self.sign, self.v)

    def __add__(self, o):
        if self.sign == o.sign:
            return _Signed(self.sign, self.v + o.v)
        return _Signed(1, self.v - o.v if self.sign > 0 else o.v - self.v)

    def __sub__(self, o):
        return self + (-o)


def _nxt(k, d=1):
    return (k - 1 + d) % 3 + 1


def _operands(block, left):
    lo, hi = (1, 2) if left else (2, 1)

    def forms(i):
        x, y = block(i)
        if left:
            return {1: _Signed(1, x), 2: _Signed(-1, y), 3: _Signed(1, y - x)}
        return {1: _Signed(1, y), 2: _Signed(1, x), 3: _Signed(-1, x + y)}

    def diag(g, k):
        yield g[_nxt(k, lo)]
        yield g[_nxt(k, hi)]

    def pair(ga, gb, k, s):
        m = _nxt(k, 2)
        yield gb[k] - ga[_nxt(k)] if left else ga[_nxt(k)] - gb[k]
        for n in (_nxt(m, lo), _nxt(m, hi)):
            s[n] = ga[n] + gb[n]
            yield s[n]

    f0 = forms(0)
    yield from diag(f0, 1)
    f1 = forms(1)
    yield from diag(f1, 2)
    yield from pair(f0, f1, 1, {})
    f2 = forms(2)
    yield from diag(f2, 3)
    yield from pair(f1, f2, 2, {})
    s02 = {}
    yield from pair(f2, f0, 3, s02)
    s02[2] = f0[2] + f2[2]
    f3 = forms(3)
    yield from diag(f3, 1)
    yield from pair(f2, f3, 3, {})
    yield from pair(f3, s02, 1, {})
    yield from pair(f3, f1, 1, {})


_SIGNS = [a.sign * b.sign for a, b in zip(_operands(lambda i: (0, 0), True), _operands(lambda i: (0, 0), False))]


def _block_product(product):
    count = iter(range(NOP))

    def m(sign=1):
        k = next(count)
        return _Signed(sign * _SIGNS[k], product(k))

    def diag(i):
        x, y = m(), m(-1)
        yield i, i, x + y
        return x, y

    def pair(a, b, da, db, less=(None, None)):
        g = m()
        xs = m()
        ab = xs - da[1] - db[1] - g
        yield a, b, ab if less[0] is None else ab - less[0]
        ys = m(-1)
        ba = ys - da[0] - db[0] + g
        yield b, a, ba if less[1] is None else ba - less[1]
        return (xs, ys), (ab, ba)

    def steps():
        d0 = yield from diag(0)
        d1 = yield from diag(1)
        yield from pair(0, 1, d0, d1)
        d2 = yield from diag(2)
        yield from pair(1, 2, d1, d2)
        d02, _ = yield from pair(2, 0, d2, d0)
        d3 = yield from diag(3)
        _, (c23, c32) = yield from pair(2, 3, d2, d3)
        yield from pair(3, 0, d3, d02, (c32, c23))
        yield from pair(3, 1, d3, d1)

    for i, j, c in steps():
        assert c.sign > 0
        yield i, j, c.v


class _Tasks:
    def __init__(self):
        self.q = []

    def add(self, gen):
        self.q.append(gen)

    def step(self, n=1):
        while n > 0 and self.q:
            try:
                next(self.q[0])
                n -= 1
            except StopIteration:
                self.q.pop(0)

    def drain(self):
        while self.q:
            self.step()


def _kernel(x_hbm, wqkv_hbm, wphi_hbm, wo_hbm, wr_hbm, wg_hbm, wu_hbm, wd_hbm, out_hbm,
            wide, w_v, wphi_v, wr_v, fm_v, part, st, ar, stage, oa0, oa1, kvl, kv_acc, out_v, xb, ob, hb, sems):

    def x_rows(row0, rows):
        return x_hbm.at[0, pl.ds(row0, rows)], wide.at[pl.ds(row0, rows)]

    def w_cols(c):
        return wqkv_hbm.at[:, pl.ds(c * L, L)], w_v.at[c]

    def kv_cols(gp):
        return [w_cols(o + g) for g in (2 * gp, 2 * gp + 1) for o in (NG, 2 * NG)]

    def phi_heads(h0, heads):
        return wphi_hbm.at[pl.ds(h0, heads)], wphi_v.at[pl.ds(h0, heads)]

    def ffn_chunk(c):
        cols = pl.ds(c * FC, FC)
        rows = pl.ds(GU + c * D, D)
        return [(wg_hbm.at[:, cols], wide.at[rows, pl.ds(0, FC)]),
                (wu_hbm.at[:, cols], wide.at[rows, pl.ds(FC, FC)]),
                (wd_hbm.at[cols], wide.at[pl.ds(WD + c * FC, FC)])]

    loads = {
        'x00': [(wr_hbm, wr_v), x_rows(0, L)],
        'x01': [x_rows(L, L)],
        'x02': [x_rows(2 * L, L)],
        'x03': [x_rows(3 * L, L)],
        'kv0a': [phi_heads(0, 8)] + kv_cols(0)[:2],
        'kv0b': kv_cols(0)[2:],
        'kv1': [phi_heads(8, H - 8)] + kv_cols(1),
        'kv2': kv_cols(2),
        'kv3': [x_rows(TT, TT)] + kv_cols(3),
        'wo': [x_rows(n * TT, TT) for n in range(2, NTILE)] + [(wo_hbm, wide.at[pl.ds(WO, D)])],
        'wq': [w_cols(g) for g in range(NG)] + [p for c in range(EARLY) for p in ffn_chunk(c)],
        'ffn': [p for c in range(EARLY, NFC) for p in ffn_chunk(c)],
    }

    def copies(name):
        return [pltpu.make_async_copy(src, dst, sems.at[list(loads).index(name)]) for src, dst in loads[name]]

    def wait(name):
        for cp in copies(name):
            cp.wait()

    def out_copy(src0, dst0, rows, col0, cols, sem):
        return pltpu.make_async_copy(out_v.at[pl.ds(src0, rows), pl.ds(col0, cols)],
                                     out_hbm.at[0, pl.ds(dst0, rows), pl.ds(col0, cols)], sems.at[sem])

    for name in loads:
        for cp in copies(name):
            cp.start(priority=1)

    ar_w = ar.bitcast(U32)
    stored = set()
    ready = set()

    wait('x00')
    wr1 = wr_v[...].astype(F32).reshape(1, D)
    zero = pl.multiple_of(jnp.max(jnp.where(jnp.abs(wr1) < 0.0, pltpu.bitcast(wr1, jnp.int32), 0)), 16)
    never = zero > 0
    ar[pl.ds(SPARE, 16), :] = jnp.zeros((16, L), BF)
    part[NPART] = jnp.zeros((8, L), F32)
    st[64] = jnp.zeros((16, L), F32)
    stage[32, pl.ds(0, 16), :] = jnp.zeros((16, L), BF)
    for oa in (oa0, oa1):
        oa[OSPARE, pl.ds(0, 16), :] = jnp.zeros((16, L), BF)

    def fold_matrices(groups):
        rr = lax.broadcasted_iota(jnp.int32, (L, DH), 0)
        ff = lax.broadcasted_iota(jnp.int32, (L, DH), 1)
        sel = jnp.where(((rr & 63) >> 1) == ff, 1.0, 0.0).astype(BF)
        r2 = lax.broadcasted_iota(jnp.int32, (L, L), 0)
        c2 = lax.broadcasted_iota(jnp.int32, (L, L), 1)
        own = ((r2 >> 6) * 2 + (r2 & 1)) == (c2 >> 5)
        for g in groups:
            a = wphi_v[4 * g:4 * g + 4].reshape(L, DH)
            fm_v[g] = jnp.where(own, _dot(sel, a, NT), 0.0).astype(BF)

    def put(row, v):
        stored.add('ar')
        ar[pl.ds(row, v.shape[0]), :] = v.astype(BF)

    def slabs(start, stride, k, row0, rows):
        return jnp.concatenate(
            [ar_w[pl.ds((start + s * stride) // 2 + k * (KH * stride // 2) + row0, rows // 2), :]
             for s in range(KH)], axis=1)

    def folded(g, c, s):
        w = _unpack(w_v.bitcast(U32)[c, pl.ds(s * L // 2, L // 2), :])
        return _dot(_unpack(fm_v.bitcast(U32)[g]), w, NT) * (2.0 * LOG2E)

    def build(load, store, slots=range(NOP)):
        for r0 in range(0, L, 16):
            for k, v in enumerate(_operands(lambda i: [_unpack(load(k, r0)).astype(F32) for k in RAWL[i]], True)):
                if k in slots and k not in STAGE:
                    store(k, r0, v.v)
                if k == slots[-1]:
                    break
            yield

    def arena_build(row_of, slots=range(NOP)):
        return build(lambda k, r0: stage.bitcast(U32)[row_of(k)[1], pl.ds(r0 // 2, 8), :],
                     lambda k, r0, v: put(row_of(k)[0] + r0, v), slots)

    def put_plain(row_of, k, v):
        stored.add('stage')
        v = v.astype(BF)
        stage[row_of(k)[1]] = v
        if k < NOP:
            ar[pl.ds(row_of(k)[0], L), :] = v

    def kv_rows(gp, s):
        return lambda k: (AKV + ((k * KH + s) * 4 + gp) * L, 8 * s + STAGE.get(k, 0))

    def plain_kv(gp, s, which=(0, 1)):
        for i in which:
            g = 2 * gp + i
            for h in range(2):
                put_plain(kv_rows(gp, s), RAWL[2 * i][h], folded(g, NG + g, h * KH + s))
                put_plain(kv_rows(gp, s), RAWL[2 * i + 1][h], w_v[2 * NG + g, pl.ds(h * HK + s * L, L), :].T)

    def prep_kv(gp):
        for s in range(KH):
            plain_kv(gp, s)
            yield
            yield from arena_build(kv_rows(gp, s))

    def q_groups(gp):
        return (2 * gp, KH + 2 * gp, 2 * gp + 1, KH + 2 * gp + 1)

    def prep_q():
        for gp in range(2):
            for s in range(KH):
                def row_of(k):
                    return AQ + ((k * KH + s) * 2 + gp) * L, 8 * s + STAGE.get(k, 0)
                for i, g in enumerate(q_groups(gp)):
                    for h in range(2):
                        put_plain(row_of, RAWL[i][h], folded(g, g, h * KH + s))
                    if i % 2:
                        yield
                yield from arena_build(row_of)
            ready.add(('q', gp))

    def prep_o():
        for c in range(2):
            for r0 in range(0, HK, 16):
                blk = [wide[pl.ds(WO + h * HK + r0, 16), pl.ds(c * HK, HK)].astype(F32) for h in range(2)]
                for k, v in enumerate(_operands(lambda j: [b[:, j * L:(j + 1) * L] for b in blk], False)):
                    put(BO + (k * 2 + c) * HK + r0, v.v)
                yield

    wr = jnp.broadcast_to(wr1, (16, D))
    best = [jnp.full((16, 1), -jnp.inf, F32), jnp.zeros((16, 1), jnp.int32)]

    def row_mean(n, c, j):
        xf = wide[pl.ds(n * TT + j * L + c * 16, 16), :].astype(F32)
        mean = jnp.sum(xf, axis=1, keepdims=True) * (1.0 / D)
        stored.add('st')
        st[8 * c + 2 * j] = jnp.broadcast_to(mean, (16, L))

    def row_stats(n, c, j):
        r0 = n * TT + j * L + c * 16
        d = wide[pl.ds(r0, 16), :].astype(F32) - jnp.concatenate([st[8 * c + 2 * j]] * (D // L), axis=1)
        var = jnp.sum(d * d, axis=1, keepdims=True) * (1.0 / D)
        rs = _rcp(_rnd(jnp.sqrt(_rnd(_rnd(var) + 1e-5))))
        r = jnp.sum(d * wr, axis=1, keepdims=True) * rs
        up = (r > best[0]) | ((r == best[0]) & (r0 < best[1]))
        best[0] = jnp.where(up, r, best[0])
        best[1] = jnp.where(up, r0, best[1])
        stored.add('st')
        st[8 * c + 2 * j + 1] = jnp.broadcast_to(0.5 * rs, (16, L))
        st[64, pl.ds(8, 8), :] = jnp.broadcast_to(jnp.maximum(best[0][:8], best[0][8:]), (8, L))

    def token_operands(n, c, s):
        row = XS + s * XR + n * L + c * 16

        def block(j):
            b = [(wide[pl.ds(n * TT + j * L + c * 16, 16), pl.ds(h * HK + s * L, L)].astype(F32)
                  - st[8 * c + 2 * j]) * st[8 * c + 2 * j + 1] for h in range(2)]
            for k, v in zip(RAW[j], b):
                if k >= NOP:
                    put(row + k * KH * XR, v)
            return b

        for k, v in enumerate(_operands(block, False)):
            put(row + k * KH * XR, v.v)

    def layernorm(n):
        for j in range(4):
            row_mean(n, 0, j)
        yield
        for c in range(L // 16):
            for j in range(4):
                row_stats(n, c, j)
                if j % 2:
                    yield
            if c + 1 < L // 16:
                for j in range(4):
                    row_mean(n, c + 1, j)
                yield
            for s in range(KH):
                token_operands(n, c, s)
                yield

    side, prep, tail, tail2, extra = _Tasks(), _Tasks(), _Tasks(), _Tasks(), _Tasks()
    count = [0]
    plan = [FIRST_PLAN, 0]
    delay = [1]
    timed, pending, dots, flush = {}, [], {}, []
    release = [stage.at[32]]

    def anchor(v):
        wide[pl.ds(ANCHOR + zero, 8), pl.ds(0, 2 * L)] = v.astype(BF)

    def probe(name):
        if name == 'ar':
            return ar_w[pl.ds(SPARE // 2 + zero, 8), :]
        if name == 'part':
            return pltpu.bitcast(part[NPART + zero], U32)
        if name == 'st':
            return pltpu.bitcast(st[64, pl.ds(zero, 8), :], U32)
        if name == 'stage':
            return stage.bitcast(U32)[32, pl.ds(zero, 8), :]
        return (oa0, oa1)[name == 'oa1'].bitcast(U32)[OSPARE, pl.ds(zero, 8), :]

    def gap(m):
        count[0] += 1
        for action in timed.pop(count[0], ()):
            action()
        due = pending.pop(0) if len(pending) > delay[0] else ()
        if due:
            tied = pltpu.bitcast(m[96:104], U32)
            for name in due:
                tied = jnp.where(never, probe(name), tied)
            m = jnp.concatenate([m[:96], pltpu.bitcast(tied, F32), m[104:]], axis=0)
        if side.q or prep.q or extra.q:
            anchor(jnp.concatenate([m[:8], m[8:16]], axis=1))
        if prep.q:
            release[0][pl.ds(zero + 16, 16), :] = m[:16].astype(BF)
        tail.step(dots.get(count[0], 1))
        tail2.step()
        todo = plan[0][(count[0] - plan[1] - 1) % len(plan[0])]
        side.step(PIECES[todo][0])
        prep.step(PIECES[todo][1])
        extra.step(todo == 'E')
        pending.append(sorted(stored))
        stored.clear()
        return m

    def soon(action):
        timed.setdefault(count[0] + 1, []).append(action)

    def after(products, gen):
        start = count[0] + products

        def held():
            while count[0] < start and not flush:
                yield
            yield from gen
        return held()

    def drain_tail():
        flush.append(1)
        tail.drain()
        flush.clear()

    def unit(lhs, rhs, dims, on_block):
        for i, j, c in _block_product(lambda k: gap(_dot(_unpack(lhs(k)), _unpack(rhs(k)), dims))):
            on_block(i, j, c)

    route = {}

    def router():
        slot = lax.broadcasted_iota(jnp.int32, (16, 1), 0)
        lane_rows = lax.broadcasted_iota(jnp.int32, (16, D), 0)
        rows = jnp.zeros((16, D), F32)
        for i in range(16):
            group = pl.multiple_of(jnp.max(jnp.where(slot == i, best[1], 0)), 16)
            rows = jnp.where(lane_rows == i, wide[pl.ds(group, 16), :].astype(F32), rows)
        mean = jnp.sum(rows, axis=1, keepdims=True) * (1.0 / D)
        var = jnp.sum((rows - mean) * (rows - mean), axis=1, keepdims=True) * (1.0 / D)
        xn = _rnd(_rnd(rows - _rnd(mean)) / _rnd(jnp.sqrt(_rnd(_rnd(var) + 1e-5))))
        score = _rnd(jnp.sum(xn * wr, axis=1, keepdims=True))
        rmax = jnp.max(score)
        idx = jnp.min(jnp.where(score == rmax, best[1] + slot, S - 1))
        row = jnp.sum(jnp.where(lane_rows == idx % 16, xn, 0.0), axis=0, keepdims=True)
        route.update(rmax=rmax, idx=idx, row=row, tile=idx // TT, block=(idx // L) % 4,
                     word=pl.multiple_of(((idx % L) // 16) * 8, 8))
        for t in range(D // L):
            xb[pl.ds(t * L, L), :] = jnp.broadcast_to(row[:, t * L:(t + 1) * L], (L, L)).T
            yield

    def matvec(row0, col0, vec, k0, slot):
        vk = vec[pl.ds(k0, FROWS), :]
        wk = wide[pl.ds(row0 + k0, FROWS), pl.ds(col0, 2 * L)].astype(F32)
        pr = wk * jnp.concatenate([vk, vk], axis=1)
        acc = jnp.sum(pr.reshape(FROWS // 8, 8, 2 * L), axis=0)
        stored.add('part')
        for t in range(2):
            part[slot(t)] = acc[:, t * L:(t + 1) * L]

    def ffn():
        def gu_slot(c, t, p):
            return ((c % 2) * 8 + t) * 2 * NSUB + p

        def y_slot(c, t, p):
            return 32 * NSUB + (t * NFC + c) * NSUB + p

        def column(c, t):
            return jnp.sum(_total([part[gu_slot(c, t, p)] for p in range(2 * NSUB)]), axis=0, keepdims=True)

        def down(c):
            for t in range(0, 8, 2):
                for p in range(NSUB):
                    matvec(WD + c * FC, t * L, hb.at[c], p * FROWS, lambda u: y_slot(c, t + u, p))
                    yield

        for c in range(NFC):
            while c == EARLY and 'ffn' not in ready:
                yield
            for t in range(0, 8, 2):
                for p in range(2 * NSUB):
                    matvec(GU + c * D, t * L, xb, p * FROWS, lambda u: gu_slot(c, t + u, p))
                    yield
            for t in range(4):
                gate, up = column(c, t), column(c, 4 + t)
                hb[c, pl.ds(t * L, L), :] = jnp.broadcast_to(_silu(gate) * up, (L, L)).T
            yield
            if c > 0:
                yield from down(c - 1)
        yield
        yield from down(NFC - 1)
        y = [sum(_total([part[y_slot(c, t, p)] for p in range(NSUB)]) for c in range(NFC)) for t in range(8)]
        gate = 1.0 / (1.0 + jnp.exp(-jnp.full((1, D), route['rmax'], F32)))
        route['y'] = jnp.sum(jnp.concatenate(y, axis=1), axis=0, keepdims=True) * gate

    def finish_pair(p, sums):
        r = lax.broadcasted_iota(jnp.int32, (80, L), 0)
        c = lax.broadcasted_iota(jnp.int32, (80, L), 1)
        keep = jnp.where(r < 64, r >> 5, r & 1) == (c & 1)
        kvl[p] = jnp.where(keep, jnp.concatenate([2.0 * sums[:64], sums[64:]], axis=0), 0.0).astype(BF)

    def kv_unit(gp, n):
        seen, acc = {}, {}

        def combine(g, phis, vts):
            for pp in range(2):
                p = 2 * g + pp
                acc[p] = acc.get(p, []) + [_dot(vts[pp], phis[pp], NT)]
                if len(acc[p]) == 4:
                    upd = _total(acc[p]) if n == 0 else kv_acc[p] + _total(acc[p])
                    if n < NTILE - 1:
                        kv_acc[p] = upd
                    else:
                        finish_pair(p, upd)
                yield

        def on_block(i, j, c):
            if i % 2:
                seen[i, j] = [jnp.concatenate([c[pp * 64:(pp + 1) * 64], jnp.ones((16, L), F32)], axis=0).astype(BF)
                              for pp in range(2)]
            else:
                seen[i, j] = [_key_features(c[pp * 64:(pp + 1) * 64]) for pp in range(2)]
            if (i ^ 1, j) in seen:
                tail.add(after(3, combine(2 * gp + i // 2, seen[i & 2, j], seen[i | 1, j])))

        def weights(k):
            while (gp, n) == (0, 0) and k in (7, 15) and k not in ready:
                prep.step()
            return slabs(AKV, 4 * L, k, gp * L // 2, L)

        unit(weights, lambda k: slabs(XS, XR, k, n * L // 2, L), NT, on_block)

    def first_tokens():
        for j in range(4):
            if j:
                wait(f'x0{j}')
            for part_of in (row_mean, row_stats):
                for c in range(L // 16):
                    part_of(0, c, j)
                anchor(jnp.zeros((8, 2 * L), BF))
        done = []
        for c in range(L // 16):
            for s in range(KH):
                if len(done) == 28:
                    wait('kv0a')
                    fold_matrices(range(2))
                    for t in range(KH):
                        plain_kv(0, t, (0,))
                        prep.add(arena_build(kv_rows(0, t), range(7)))
                if len(done) >= 3:
                    anchor(jnp.concatenate([done[-3], done[-3]], axis=1))
                token_operands(0, c, s)
                prep.step(2)
                done.append(pltpu.bitcast(probe('ar'), F32))
        prep.drain()

    def more_weights():
        while count[0] < 3:
            yield
        wait('kv0b')
        for s in range(KH):
            plain_kv(0, s, (1,))
            yield
        for slots in (range(7, 15), range(15, NOP)):
            for s in range(KH):
                yield from arena_build(kv_rows(0, s), slots)
            ready.add(slots[0])
        while count[0] < 16:
            yield
        wait('kv1')
        fold_matrices(range(2, NG))
        yield from prep_kv(1)

    def start_side_work(n, gp):
        if (n, gp) == (0, 1):
            wait('kv2')
            prep.add(prep_kv(2))
            plan[0] = TILE0_PLAN
        elif (n, gp) == (0, 2):
            wait('kv3')
            prep.add(prep_kv(3))
            side.add(layernorm(1))
        elif n > 0 and gp == 0:
            plan[0] = NORM_PLAN
            delay[0] = 2
            if n == 1:
                wait('wo')
                prep.add(prep_o())
            if n + 1 < NTILE:
                side.add(layernorm(n + 1))
            else:
                wait('wq')
                plan[0] = QUERY_PLAN
                side.add(router())
                side.add(ffn())
                prep.add(prep_q())

    first_tokens()
    prep.add(more_weights())
    for n in range(NTILE):
        for gp in range(4):
            if n == 0 and gp:
                prep.drain()
            if n and not gp:
                side.drain()
            soon(lambda n=n, gp=gp: start_side_work(n, gp))
            kv_unit(gp, n)

    built = {}

    caught = [jnp.zeros((8, L), U32)] * (2 * KH)

    def catch_row(n, gp):
        for slab in (2 * gp, 2 * gp + 1):
            for h in range(2):
                k = sum(jnp.where(route['block'] == j, RAWL[j][h], 0) for j in range(4))
                words = (oa0, oa1)[n % 2].bitcast(U32)[k * KH + slab, pl.ds(route['word'], 8), :]
                caught[h * KH + slab] = jnp.where(route['tile'] == n, words, caught[h * KH + slab])

    def routed_projection():
        hit = lax.broadcasted_iota(jnp.int32, (16, L), 0) == route['idx'] % 16
        for t in range(2 * KH):
            row = jnp.sum(jnp.where(hit, _unpack(caught[t]).astype(F32), 0.0), axis=0, keepdims=True)
            ob[pl.ds(t * L, L), :] = jnp.broadcast_to(row, (L, L)).T
            if t % 2:
                yield
        for t in range(0, 8, 2):
            for p in range(2 * NSUB):
                matvec(WO, t * L, ob, p * FROWS, lambda u: OPART + (t + u) * 2 * NSUB + p)
                yield
        s = [_total([part[OPART + t * 2 * NSUB + p] for p in range(2 * NSUB)]) for t in range(8)]
        route['s'] = jnp.sum(jnp.concatenate(s, axis=1), axis=0, keepdims=True)

    def o_operands(n, gp):
        oa = (oa0, oa1)[n % 2]
        release[0] = oa.at[OSPARE]
        for slab in (2 * gp, 2 * gp + 1):
            def store(k, r0, v):
                stored.add(f'oa{n % 2}')
                oa[k * KH + slab, pl.ds(r0, 16), :] = v.astype(BF)
            yield from build(lambda k, r0: oa.bitcast(U32)[k * KH + slab, pl.ds(r0 // 2, 8), :], store)
        built[n] = built.get(n, 0) + 1

    def q_unit(gp, n):
        while ('q', gp) not in ready:
            prep.step()
        left = [16]
        oa = (oa0, oa1)[n % 2]

        def attend(i, j, feats):
            rows = []
            for pp, (phi, scale) in enumerate(feats):
                nd = _dot(_unpack(kvl.bitcast(U32)[2 * q_groups(gp)[i] + pp]), phi, NN)
                inv = _rcp(nd[64:72] + 1e-6 * scale)
                for head in range(2):
                    rd = jnp.broadcast_to(inv[head:head + 1], (8, L))
                    rows += [nd[head * DH + 8 * q:head * DH + 8 * q + 8] * rd for q in range(4)]
                if pp == 0:
                    yield
            oa[RAWL[j][i % 2] * KH + 2 * gp + i // 2] = jnp.concatenate(rows, axis=0).T.astype(BF)
            left[0] -= 1
            if not left[0]:
                catch_row(n, gp)
                prep.add(o_operands(n, gp))
                if (n, gp) == (NTILE - 1, 1):
                    extra.add(routed_projection())
            yield

        def on_block(i, j, c):
            tail.add(after(4, attend(i, j, [_query_features(c[pp * 64:(pp + 1) * 64]) for pp in range(2)])))

        unit(lambda k: slabs(AQ, 2 * L, k, gp * L // 2, L),
             lambda k: slabs(XS, XR, k, n * L // 2, L), NT, on_block)

    def o_unit(c, n):
        left = [16]

        def finish(j, col, s):
            rows = pl.ds(n * TT + j * L, L)
            cols = pl.ds(c * HK + col * L, L)
            half = _unpack(ar_w[pl.ds((XS + (RAW[j][c] * KH + col) * XR + n * L) // 2, L // 2), :]).astype(F32)
            sh = s * half
            out_v[rows, cols] = (wide[rows, cols].astype(F32) + sh + sh * jnp.tanh(half)).astype(BF)
            left[0] -= 1
            if (n, c) == (NTILE - 1, 1):
                out_copy(rows.start, rows.start, L, cols.start, L, 1).start()
            elif not left[0]:
                out_copy(n * TT, n * TT, TT, c * HK, HK, int(n == NTILE - 1)).start()
            yield

        if c == 0:
            if n == NTILE - 1:
                drain_tail()
            while built.get(n, 0) < 2:
                (prep if prep.q else tail).step()
        oa = (oa0, oa1)[n % 2].bitcast(U32)
        unit(lambda k: jnp.concatenate([oa[k * KH + s] for s in range(KH)], axis=1),
             lambda k: ar_w[pl.ds((BO + (k * 2 + c) * HK) // 2, HK // 2), :], NN,
             lambda j, col, s: tail2.add(finish(j, col, s)))

    dots.update((count[0] + 1 + t, int(n)) for t, n in enumerate(DOT_PLAN))
    plan[:] = [OUT_PLAN, count[0]]
    delay[0] = 1
    q_unit(0, 0)
    soon(lambda: wait('ffn'))
    soon(lambda: ready.add('ffn'))
    q_unit(1, 0)
    for n in range(1, NTILE):
        for gp in range(2):
            q_unit(gp, n)
            o_unit(gp, n - 1)
    for c in range(2):
        o_unit(c, NTILE - 1)
    drain_tail()
    tail2.drain()
    side.drain()
    extra.drain()

    row0 = pl.multiple_of((route['idx'] // 16) * 16, 16)
    half = 0.5 * (route['row'] + route['y'])
    sh = route['s'] * half
    fixed = wide[pl.ds(row0, 16), :].astype(F32) + (sh + sh * jnp.tanh(half))
    hit = lax.broadcasted_iota(jnp.int32, (16, D), 0) == route['idx'] % 16
    out_v[pl.ds(S, 16), :] = jnp.where(hit, fixed, out_v[pl.ds(row0, 16), :].astype(F32)).astype(BF)
    rows_copy = out_copy(S, row0, 16, 0, D, 2)
    for _ in range(2 * NTILE - 2):
        out_copy(0, 0, TT, 0, HK, 0).wait()
    pl.when(route['tile'] != NTILE - 1)(rows_copy.start)
    out_copy(0, 0, TT, 0, HK, 1).wait()
    for _ in range(16):
        out_copy(0, 0, L, 0, L, 1).wait()
    pl.when(route['tile'] == NTILE - 1)(rows_copy.start)
    rows_copy.wait()


@jax.jit
def pallas_recurrent_scan__linear_kernel_hedgehog__moe_arch_mod__prompt_kernel(
    A_x: jax.Array,
    A_wqkv: jax.Array,
    A_w_phi: jax.Array,
    A_wo: jax.Array,
    B_x: jax.Array,
    B_w_r: jax.Array,
    B_w_gate: jax.Array,
    B_w_up: jax.Array,
    B_w_down: jax.Array,
):
    del B_x
    hbm = pl.BlockSpec(memory_space=pl.ANY)
    return pl.pallas_call(
        _kernel,
        out_shape=jax.ShapeDtypeStruct(A_x.shape, A_x.dtype),
        in_specs=[hbm] * 8,
        out_specs=hbm,
        scratch_shapes=[
            pltpu.VMEM((ANCHOR + 8, D), BF),
            pltpu.VMEM((3 * NG, D, L), BF),
            pltpu.VMEM((H, DH, DH), BF),
            pltpu.VMEM((D,), BF),
            pltpu.VMEM((NG, L, L), BF),
            pltpu.VMEM((NPART + 1, 8, L), F32),
            pltpu.VMEM((65, 16, L), F32),
            pltpu.VMEM((SPARE + 16, L), BF),
            pltpu.VMEM((33, L, L), BF),
            pltpu.VMEM((OSPARE + 1, L, L), BF),
            pltpu.VMEM((OSPARE + 1, L, L), BF),
            pltpu.VMEM((NP, 80, L), BF),
            pltpu.VMEM((NP, 80, L), F32),
            pltpu.VMEM((S + 16, D), BF),
            pltpu.VMEM((D, L), F32),
            pltpu.VMEM((D, L), F32),
            pltpu.VMEM((NFC, FC, L), F32),
            pltpu.SemaphoreType.DMA((12,)),
        ],
        compiler_params=pltpu.CompilerParams(vmem_limit_bytes=120 << 20),
        name="hedgehog_mod",
    )(A_x, A_wqkv, A_w_phi, A_wo, B_w_r, B_w_gate, B_w_up, B_w_down)
```

```python
import jax
import jax.numpy as jnp
from jax import lax
import jax.experimental.pallas as pl
import jax.experimental.pallas.tpu as pltpu

BF = jnp.bfloat16
F32 = jnp.float32
U32 = jnp.uint32
NN = (((1,), (0,)), ((), ()))
NT = (((1,), (1,)), ((), ()))
LOG2E = 1.4426950408889634

S, D, H, DH, FF = 2048, 1024, 32, 32, 3584
L = 128
HK = D // 2
KH = HK // L
NG = H // 4
NP = H // 2
TT = 4 * L
NTILE = S // TT
FC = 4 * L
NFC = FF // FC
FROWS = 128
NSUB = HK // FROWS
EARLY = 3
NOP = 26
RAW = ((1, 26), (27, 2), (7, 8), (16, 28))
RAWL = ((26, 0), (3, 27), (7, 8), (28, 15))
STAGE = {k: i for i, k in enumerate(sum(RAWL, ()))}

XR = S // 4
XS = 0
AKV = XS + (NOP + 3) * KH * XR
AQ = AKV + NOP * KH * 4 * L
BO = AQ + NOP * KH * 2 * L
SPARE = BO + NOP * 2 * HK
GU = S
WD = GU + NFC * D
WO = WD + FF
ANCHOR = WO + D
OPART = (32 + 8 * NFC) * NSUB
NPART = OPART + 16 * NSUB
OSPARE = (NOP + 3) * KH

PIECES = {'.': (0, 0), 'L': (1, 0), '2': (2, 0), 'P': (0, 1), '3': (0, 2), '5': (0, 3), '9': (0, 8),
          'B': (1, 1), '6': (1, 2), 'E': (0, 0)}
FIRST_PLAN = '39.555555553335553553553P3'
TILE0_PLAN = '.' * NOP + 'PP33PP3P333PPPP33PP3PPPP3P' '3B63BB6PBBB6B6B3BBB666PBB3' '2L2LLL22L222222LL2LLLLLLLL'
NORM_PLAN = 'PPLLLBL.PPPLLL.L.LBLL.LLPP'
QUERY_PLAN = ('PBBLBBLBBBBB.BBBBBBBBBBLB.' 'BBBBLBB.BLBBLBBBBBPBBBPLBB'
              'LPLBBBPBBBBBBBBBBBB.BBLLBB' 'LBBBBBLBBBBBLBBBBBBBBBPLP.')
OUT_PLAN = ('L.L.LL.LLLL.LLLLLLLLL.LLL.' 'LBLLLL.LLLBPBPBLPPPPBPBPBB'
            '.LBP.LPLPLBPPLPBLPPPBLPPBP' 'LBLPLP.LLBPP.BBLBBLPL.LBL.'
            + ('LL.LLLLLBBPLPLP.BPLLPLPLBL' 'LPLLLBPLPBLPL.PLLBPLBLLBLL') * 4
            + 'LLLPLLBLBL.PLBLLPPLLPLLLBL' 'BBBLLLBPPBLPLBPPBPPPPPBPPP'
            'ELELELELLLELELELELLLEEEEEL' 'LEEEEEEEEEEEEEEEEEEEEEEEE.')
DOT_PLAN = ('11221121111111112211111222' '22111211211222112211121222'
            '12121211111111111111111111' '11111111111111121111111111'
            + ('11111112111211111112111121' '11211111111111111211111111') * 4
            + '11121211112211111211111111' '11211111111111111111111111'
            '11111111111111111111111111' '11111111111111111111111111')


def _dot(a, b, dims):
    return lax.dot_general(a, b, dims, preferred_element_type=F32)


def _unpack(words):
    return pltpu.bitcast(words, BF)


def _rnd(v):
    return v.astype(BF).astype(F32)


def _rcp(v):
    return pltpu.reciprocal(v, approx=True)


def _silu(v):
    h = 0.5 * v
    return h + h * jnp.tanh(h)


def _total(v):
    while len(v) > 1:
        v = [v[i] + v[i + 1] for i in range(0, len(v), 2)]
    return v[0]


def _pair_reduce(v, reduce, op):
    r = reduce(v, axis=0)
    r = op(r, pltpu.roll(r, 2, 0))
    return op(r, pltpu.roll(r, 4, 0))


def _dual_exp(p):
    v = p.reshape(8, 8, L)
    ep = jnp.exp2(v - _pair_reduce(v, jnp.max, jnp.maximum))
    en = jnp.exp2(_pair_reduce(v, jnp.min, jnp.minimum) - v)
    return ep, en, _pair_reduce(ep, jnp.sum, jnp.add), _pair_reduce(en, jnp.sum, jnp.add)


def _key_features(p):
    ep, en, sp, sn = _dual_exp(p)
    return jnp.concatenate([ep * _rcp(sp), en * _rcp(sn)], axis=0).reshape(L, L).astype(BF)


def _query_features(p):
    ep, en, sp, sn = _dual_exp(p)
    return jnp.concatenate([ep, en * (sp * _rcp(sn))], axis=0).reshape(L, L).astype(BF), sp


class _Signed:
    def __init__(self, sign, v):
        self.sign, self.v = sign, v

    def __neg__(self):
        return _Signed(-self.sign, self.v)

    def __add__(self, o):
        if self.sign == o.sign:
            return _Signed(self.sign, self.v + o.v)
        return _Signed(1, self.v - o.v if self.sign > 0 else o.v - self.v)

    def __sub__(self, o):
        return self + (-o)


def _nxt(k, d=1):
    return (k - 1 + d) % 3 + 1


def _operands(block, left):
    lo, hi = (1, 2) if left else (2, 1)

    def forms(i):
        x, y = block(i)
        if left:
            return {1: _Signed(1, x), 2: _Signed(-1, y), 3: _Signed(1, y - x)}
        return {1: _Signed(1, y), 2: _Signed(1, x), 3: _Signed(-1, x + y)}

    def diag(g, k):
        yield g[_nxt(k, lo)]
        yield g[_nxt(k, hi)]

    def pair(ga, gb, k, s):
        m = _nxt(k, 2)
        yield gb[k] - ga[_nxt(k)] if left else ga[_nxt(k)] - gb[k]
        for n in (_nxt(m, lo), _nxt(m, hi)):
            s[n] = ga[n] + gb[n]
            yield s[n]

    f0 = forms(0)
    yield from diag(f0, 1)
    f1 = forms(1)
    yield from diag(f1, 2)
    yield from pair(f0, f1, 1, {})
    f2 = forms(2)
    yield from diag(f2, 3)
    yield from pair(f1, f2, 2, {})
    s02 = {}
    yield from pair(f2, f0, 3, s02)
    s02[2] = f0[2] + f2[2]
    f3 = forms(3)
    yield from diag(f3, 1)
    yield from pair(f2, f3, 3, {})
    yield from pair(f3, s02, 1, {})
    yield from pair(f3, f1, 1, {})


_SIGNS = [a.sign * b.sign for a, b in zip(_operands(lambda i: (0, 0), True), _operands(lambda i: (0, 0), False))]


def _block_product(product):
    count = iter(range(NOP))

    def m(sign=1):
        k = next(count)
        return _Signed(sign * _SIGNS[k], product(k))

    def diag(i):
        x, y = m(), m(-1)
        yield i, i, x + y
        return x, y

    def pair(a, b, da, db, less=(None, None)):
        g = m()
        xs = m()
        ab = xs - da[1] - db[1] - g
        yield a, b, ab if less[0] is None else ab - less[0]
        ys = m(-1)
        ba = ys - da[0] - db[0] + g
        yield b, a, ba if less[1] is None else ba - less[1]
        return (xs, ys), (ab, ba)

    def steps():
        d0 = yield from diag(0)
        d1 = yield from diag(1)
        yield from pair(0, 1, d0, d1)
        d2 = yield from diag(2)
        yield from pair(1, 2, d1, d2)
        d02, _ = yield from pair(2, 0, d2, d0)
        d3 = yield from diag(3)
        _, (c23, c32) = yield from pair(2, 3, d2, d3)
        yield from pair(3, 0, d3, d02, (c32, c23))
        yield from pair(3, 1, d3, d1)

    for i, j, c in steps():
        assert c.sign > 0
        yield i, j, c.v


class _Tasks:
    def __init__(self):
        self.q = []

    def add(self, gen):
        self.q.append(gen)

    def step(self, n=1):
        while n > 0 and self.q:
            try:
                next(self.q[0])
                n -= 1
            except StopIteration:
                self.q.pop(0)

    def drain(self):
        while self.q:
            self.step()


def _kernel(x_hbm, wqkv_hbm, wphi_hbm, wo_hbm, wr_hbm, wg_hbm, wu_hbm, wd_hbm, out_hbm,
            wide, w_v, wphi_v, wr_v, fm_v, part, st, ar, stage, oa0, oa1, kvl, kv_acc, out_v, xb, ob, hb, sems):

    def x_rows(row0, rows):
        return x_hbm.at[0, pl.ds(row0, rows)], wide.at[pl.ds(row0, rows)]

    def w_cols(c):
        return wqkv_hbm.at[:, pl.ds(c * L, L)], w_v.at[c]

    def kv_cols(gp):
        return [w_cols(o + g) for g in (2 * gp, 2 * gp + 1) for o in (NG, 2 * NG)]

    def phi_heads(h0, heads):
        return wphi_hbm.at[pl.ds(h0, heads)], wphi_v.at[pl.ds(h0, heads)]

    def ffn_chunk(c):
        cols = pl.ds(c * FC, FC)
        rows = pl.ds(GU + c * D, D)
        return [(wg_hbm.at[:, cols], wide.at[rows, pl.ds(0, FC)]),
                (wu_hbm.at[:, cols], wide.at[rows, pl.ds(FC, FC)]),
                (wd_hbm.at[cols], wide.at[pl.ds(WD + c * FC, FC)])]

    loads = {
        'x00': [(wr_hbm, wr_v), x_rows(0, L)],
        'x01': [x_rows(L, L)],
        'x02': [x_rows(2 * L, L)],
        'x03': [x_rows(3 * L, L)],
        'kv0a': [phi_heads(0, 8)] + kv_cols(0)[:2],
        'kv0b': kv_cols(0)[2:],
        'kv1': [phi_heads(8, H - 8)] + kv_cols(1),
        'kv2': kv_cols(2),
        'kv3': [x_rows(TT, TT)] + kv_cols(3),
        'wo': [x_rows(n * TT, TT) for n in range(2, NTILE)] + [(wo_hbm, wide.at[pl.ds(WO, D)])],
        'wq': [w_cols(g) for g in range(NG)] + [p for c in range(EARLY) for p in ffn_chunk(c)],
        'ffn': [p for c in range(EARLY, NFC) for p in ffn_chunk(c)],
    }

    def copies(name):
        return [pltpu.make_async_copy(src, dst, sems.at[list(loads).index(name)]) for src, dst in loads[name]]

    def wait(name):
        for cp in copies(name):
            cp.wait()

    def out_copy(src0, dst0, rows, col0, cols, sem):
        return pltpu.make_async_copy(out_v.at[pl.ds(src0, rows), pl.ds(col0, cols)],
                                     out_hbm.at[0, pl.ds(dst0, rows), pl.ds(col0, cols)], sems.at[sem])

    for name in loads:
        for cp in copies(name):
            cp.start(priority=1)

    ar_w = ar.bitcast(U32)
    stored = set()
    ready = set()

    wait('x00')
    wr1 = wr_v[...].astype(F32).reshape(1, D)
    zero = pl.multiple_of(jnp.max(jnp.where(jnp.abs(wr1) < 0.0, pltpu.bitcast(wr1, jnp.int32), 0)), 16)
    never = zero > 0
    ar[pl.ds(SPARE, 16), :] = jnp.zeros((16, L), BF)
    part[NPART] = jnp.zeros((8, L), F32)
    st[64] = jnp.zeros((16, L), F32)
    stage[32, pl.ds(0, 16), :] = jnp.zeros((16, L), BF)
    for oa in (oa0, oa1):
        oa[OSPARE, pl.ds(0, 16), :] = jnp.zeros((16, L), BF)

    def fold_matrices(groups):
        rr = lax.broadcasted_iota(jnp.int32, (L, DH), 0)
        ff = lax.broadcasted_iota(jnp.int32, (L, DH), 1)
        sel = jnp.where(((rr & 63) >> 1) == ff, 1.0, 0.0).astype(BF)
        r2 = lax.broadcasted_iota(jnp.int32, (L, L), 0)
        c2 = lax.broadcasted_iota(jnp.int32, (L, L), 1)
        own = ((r2 >> 6) * 2 + (r2 & 1)) == (c2 >> 5)
        for g in groups:
            a = wphi_v[4 * g:4 * g + 4].reshape(L, DH)
            fm_v[g] = jnp.where(own, _dot(sel, a, NT), 0.0).astype(BF)

    def put(row, v):
        stored.add('ar')
        ar[pl.ds(row, v.shape[0]), :] = v.astype(BF)

    def slabs(start, stride, k, row0, rows):
        return jnp.concatenate(
            [ar_w[pl.ds((start + s * stride) // 2 + k * (KH * stride // 2) + row0, rows // 2), :]
             for s in range(KH)], axis=1)

    def folded(g, c, s):
        w = _unpack(w_v.bitcast(U32)[c, pl.ds(s * L // 2, L // 2), :])
        return _dot(_unpack(fm_v.bitcast(U32)[g]), w, NT) * (2.0 * LOG2E)

    def build(load, store, slots=range(NOP)):
        for r0 in range(0, L, 16):
            for k, v in enumerate(_operands(lambda i: [_unpack(load(k, r0)).astype(F32) for k in RAWL[i]], True)):
                if k in slots and k not in STAGE:
                    store(k, r0, v.v)
                if k == slots[-1]:
                    break
            yield

    def arena_build(row_of, slots=range(NOP)):
        return build(lambda k, r0: stage.bitcast(U32)[row_of(k)[1], pl.ds(r0 // 2, 8), :],
                     lambda k, r0, v: put(row_of(k)[0] + r0, v), slots)

    def put_plain(row_of, k, v):
        stored.add('stage')
        v = v.astype(BF)
        stage[row_of(k)[1]] = v
        if k < NOP:
            ar[pl.ds(row_of(k)[0], L), :] = v

    def kv_rows(gp, s):
        return lambda k: (AKV + ((k * KH + s) * 4 + gp) * L, 8 * s + STAGE.get(k, 0))

    def plain_kv(gp, s, which=(0, 1)):
        for i in which:
            g = 2 * gp + i
            for h in range(2):
                put_plain(kv_rows(gp, s), RAWL[2 * i][h], folded(g, NG + g, h * KH + s))
                put_plain(kv_rows(gp, s), RAWL[2 * i + 1][h], w_v[2 * NG + g, pl.ds(h * HK + s * L, L), :].T)

    def prep_kv(gp):
        for s in range(KH):
            plain_kv(gp, s)
            yield
            yield from arena_build(kv_rows(gp, s))

    def q_groups(gp):
        return (2 * gp, KH + 2 * gp, 2 * gp + 1, KH + 2 * gp + 1)

    def prep_q():
        for gp in range(2):
            for s in range(KH):
                def row_of(k):
                    return AQ + ((k * KH + s) * 2 + gp) * L, 8 * s + STAGE.get(k, 0)
                for i, g in enumerate(q_groups(gp)):
                    for h in range(2):
                        put_plain(row_of, RAWL[i][h], folded(g, g, h * KH + s))
                    if i % 2:
                        yield
                yield from arena_build(row_of)
            ready.add(('q', gp))

    def prep_o():
        for c in range(2):
            for r0 in range(0, HK, 16):
                blk = [wide[pl.ds(WO + h * HK + r0, 16), pl.ds(c * HK, HK)].astype(F32) for h in range(2)]
                for k, v in enumerate(_operands(lambda j: [b[:, j * L:(j + 1) * L] for b in blk], False)):
                    put(BO + (k * 2 + c) * HK + r0, v.v)
                yield

    wr = jnp.broadcast_to(wr1, (16, D))
    best = [jnp.full((16, 1), -jnp.inf, F32), jnp.zeros((16, 1), jnp.int32)]

    def row_mean(n, c, j):
        xf = wide[pl.ds(n * TT + j * L + c * 16, 16), :].astype(F32)
        mean = jnp.sum(xf, axis=1, keepdims=True) * (1.0 / D)
        stored.add('st')
        st[8 * c + 2 * j] = jnp.broadcast_to(mean, (16, L))

    def row_stats(n, c, j):
        r0 = n * TT + j * L + c * 16
        d = wide[pl.ds(r0, 16), :].astype(F32) - jnp.concatenate([st[8 * c + 2 * j]] * (D // L), axis=1)
        var = jnp.sum(d * d, axis=1, keepdims=True) * (1.0 / D)
        rs = _rcp(_rnd(jnp.sqrt(_rnd(_rnd(var) + 1e-5))))
        r = jnp.sum(d * wr, axis=1, keepdims=True) * rs
        up = (r > best[0]) | ((r == best[0]) & (r0 < best[1]))
        best[0] = jnp.where(up, r, best[0])
        best[1] = jnp.where(up, r0, best[1])
        stored.add('st')
        st[8 * c + 2 * j + 1] = jnp.broadcast_to(0.5 * rs, (16, L))
        st[64, pl.ds(8, 8), :] = jnp.broadcast_to(jnp.maximum(best[0][:8], best[0][8:]), (8, L))

    def token_operands(n, c, s):
        row = XS + s * XR + n * L + c * 16

        def block(j):
            b = [(wide[pl.ds(n * TT + j * L + c * 16, 16), pl.ds(h * HK + s * L, L)].astype(F32)
                  - st[8 * c + 2 * j]) * st[8 * c + 2 * j + 1] for h in range(2)]
            for k, v in zip(RAW[j], b):
                if k >= NOP:
                    put(row + k * KH * XR, v)
            return b

        for k, v in enumerate(_operands(block, False)):
            put(row + k * KH * XR, v.v)

    def layernorm(n):
        for j in range(4):
            row_mean(n, 0, j)
        yield
        for c in range(L // 16):
            for j in range(4):
                row_stats(n, c, j)
                if j % 2:
                    yield
            if c + 1 < L // 16:
                for j in range(4):
                    row_mean(n, c + 1, j)
                yield
            for s in range(KH):
                token_operands(n, c, s)
                yield

    side, prep, tail, tail2, extra = _Tasks(), _Tasks(), _Tasks(), _Tasks(), _Tasks()
    count = [0]
    plan = [FIRST_PLAN, 0]
    delay = [1]
    timed, pending, dots, flush = {}, [], {}, []
    release = [stage.at[32]]

    def anchor(v):
        wide[pl.ds(ANCHOR + zero, 8), pl.ds(0, 2 * L)] = v.astype(BF)

    def probe(name):
        if name == 'ar':
            return ar_w[pl.ds(SPARE // 2 + zero, 8), :]
        if name == 'part':
            return pltpu.bitcast(part[NPART + zero], U32)
        if name == 'st':
            return pltpu.bitcast(st[64, pl.ds(zero, 8), :], U32)
        if name == 'stage':
            return stage.bitcast(U32)[32, pl.ds(zero, 8), :]
        return (oa0, oa1)[name == 'oa1'].bitcast(U32)[OSPARE, pl.ds(zero, 8), :]

    def gap(m):
        count[0] += 1
        for action in timed.pop(count[0], ()):
            action()
        due = pending.pop(0) if len(pending) > delay[0] else ()
        if due:
            tied = pltpu.bitcast(m[96:104], U32)
            for name in due:
                tied = jnp.where(never, probe(name), tied)
            m = jnp.concatenate([m[:96], pltpu.bitcast(tied, F32), m[104:]], axis=0)
        if side.q or prep.q or extra.q:
            anchor(jnp.concatenate([m[:8], m[8:16]], axis=1))
        if prep.q:
            release[0][pl.ds(zero + 16, 16), :] = m[:16].astype(BF)
        tail.step(dots.get(count[0], 1))
        tail2.step()
        todo = plan[0][(count[0] - plan[1] - 1) % len(plan[0])]
        side.step(PIECES[todo][0])
        prep.step(PIECES[todo][1])
        extra.step(todo == 'E')
        pending.append(sorted(stored))
        stored.clear()
        return m

    def soon(action):
        timed.setdefault(count[0] + 1, []).append(action)

    def after(products, gen):
        start = count[0] + products

        def held():
            while count[0] < start and not flush:
                yield
            yield from gen
        return held()

    def drain_tail():
        flush.append(1)
        tail.drain()
        flush.clear()

    def unit(lhs, rhs, dims, on_block):
        for i, j, c in _block_product(lambda k: gap(_dot(_unpack(lhs(k)), _unpack(rhs(k)), dims))):
            on_block(i, j, c)

    route = {}

    def router():
        slot = lax.broadcasted_iota(jnp.int32, (16, 1), 0)
        lane_rows = lax.broadcasted_iota(jnp.int32, (16, D), 0)
        rows = jnp.zeros((16, D), F32)
        for i in range(16):
            group = pl.multiple_of(jnp.max(jnp.where(slot == i, best[1], 0)), 16)
            rows = jnp.where(lane_rows == i, wide[pl.ds(group, 16), :].astype(F32), rows)
        mean = jnp.sum(rows, axis=1, keepdims=True) * (1.0 / D)
        var = jnp.sum((rows - mean) * (rows - mean), axis=1, keepdims=True) * (1.0 / D)
        xn = _rnd(_rnd(rows - _rnd(mean)) / _rnd(jnp.sqrt(_rnd(_rnd(var) + 1e-5))))
        score = _rnd(jnp.sum(xn * wr, axis=1, keepdims=True))
        rmax = jnp.max(score)
        idx = jnp.min(jnp.where(score == rmax, best[1] + slot, S - 1))
        row = jnp.sum(jnp.where(lane_rows == idx % 16, xn, 0.0), axis=0, keepdims=True)
        route.update(rmax=rmax, idx=idx, row=row, tile=idx // TT, block=(idx // L) % 4,
                     word=pl.multiple_of(((idx % L) // 16) * 8, 8))
        for t in range(D // L):
            xb[pl.ds(t * L, L), :] = jnp.broadcast_to(row[:, t * L:(t + 1) * L], (L, L)).T
            yield

    def matvec(row0, col0, vec, k0, slot):
        vk = vec[pl.ds(k0, FROWS), :]
        wk = wide[pl.ds(row0 + k0, FROWS), pl.ds(col0, 2 * L)].astype(F32)
        pr = wk * jnp.concatenate([vk, vk], axis=1)
        acc = jnp.sum(pr.reshape(FROWS // 8, 8, 2 * L), axis=0)
        stored.add('part')
        for t in range(2):
            part[slot(t)] = acc[:, t * L:(t + 1) * L]

    def ffn():
        def gu_slot(c, t, p):
            return ((c % 2) * 8 + t) * 2 * NSUB + p

        def y_slot(c, t, p):
            return 32 * NSUB + (t * NFC + c) * NSUB + p

        def column(c, t):
            return jnp.sum(_total([part[gu_slot(c, t, p)] for p in range(2 * NSUB)]), axis=0, keepdims=True)

        def down(c):
            for t in range(0, 8, 2):
                for p in range(NSUB):
                    matvec(WD + c * FC, t * L, hb.at[c], p * FROWS, lambda u: y_slot(c, t + u, p))
                    yield

        for c in range(NFC):
            while c == EARLY and 'ffn' not in ready:
                yield
            for t in range(0, 8, 2):
                for p in range(2 * NSUB):
                    matvec(GU + c * D, t * L, xb, p * FROWS, lambda u: gu_slot(c, t + u, p))
                    yield
            for t in range(4):
                gate, up = column(c, t), column(c, 4 + t)
                hb[c, pl.ds(t * L, L), :] = jnp.broadcast_to(_silu(gate) * up, (L, L)).T
            yield
            if c > 0:
                yield from down(c - 1)
        yield
        yield from down(NFC - 1)
        y = [sum(_total([part[y_slot(c, t, p)] for p in range(NSUB)]) for c in range(NFC)) for t in range(8)]
        gate = 1.0 / (1.0 + jnp.exp(-jnp.full((1, D), route['rmax'], F32)))
        route['y'] = jnp.sum(jnp.concatenate(y, axis=1), axis=0, keepdims=True) * gate

    def finish_pair(p, sums):
        r = lax.broadcasted_iota(jnp.int32, (80, L), 0)
        c = lax.broadcasted_iota(jnp.int32, (80, L), 1)
        keep = jnp.where(r < 64, r >> 5, r & 1) == (c & 1)
        kvl[p] = jnp.where(keep, jnp.concatenate([2.0 * sums[:64], sums[64:]], axis=0), 0.0).astype(BF)

    def kv_unit(gp, n):
        seen, acc = {}, {}

        def combine(g, phis, vts):
            for pp in range(2):
                p = 2 * g + pp
                acc[p] = acc.get(p, []) + [_dot(vts[pp], phis[pp], NT)]
                if len(acc[p]) == 4:
                    upd = _total(acc[p]) if n == 0 else kv_acc[p] + _total(acc[p])
                    if n < NTILE - 1:
                        kv_acc[p] = upd
                    else:
                        finish_pair(p, upd)
                yield

        def on_block(i, j, c):
            if i % 2:
                seen[i, j] = [jnp.concatenate([c[pp * 64:(pp + 1) * 64], jnp.ones((16, L), F32)], axis=0).astype(BF)
                              for pp in range(2)]
            else:
                seen[i, j] = [_key_features(c[pp * 64:(pp + 1) * 64]) for pp in range(2)]
            if (i ^ 1, j) in seen:
                tail.add(after(3, combine(2 * gp + i // 2, seen[i & 2, j], seen[i | 1, j])))

        def weights(k):
            while (gp, n) == (0, 0) and k in (7, 15) and k not in ready:
                prep.step()
            return slabs(AKV, 4 * L, k, gp * L // 2, L)

        unit(weights, lambda k: slabs(XS, XR, k, n * L // 2, L), NT, on_block)

    def first_tokens():
        for j in range(4):
            if j:
                wait(f'x0{j}')
            for part_of in (row_mean, row_stats):
                for c in range(L // 16):
                    part_of(0, c, j)
                anchor(jnp.zeros((8, 2 * L), BF))
        done = []
        for c in range(L // 16):
            for s in range(KH):
                if len(done) == 28:
                    wait('kv0a')
                    fold_matrices(range(2))
                    for t in range(KH):
                        plain_kv(0, t, (0,))
                        prep.add(arena_build(kv_rows(0, t), range(7)))
                if len(done) >= 3:
                    anchor(jnp.concatenate([done[-3], done[-3]], axis=1))
                token_operands(0, c, s)
                prep.step(2)
                done.append(pltpu.bitcast(probe('ar'), F32))
        prep.drain()

    def more_weights():
        while count[0] < 3:
            yield
        wait('kv0b')
        for s in range(KH):
            plain_kv(0, s, (1,))
            yield
        for slots in (range(7, 15), range(15, NOP)):
            for s in range(KH):
                yield from arena_build(kv_rows(0, s), slots)
            ready.add(slots[0])
        while count[0] < 16:
            yield
        wait('kv1')
        fold_matrices(range(2, NG))
        yield from prep_kv(1)

    def start_side_work(n, gp):
        if (n, gp) == (0, 1):
            wait('kv2')
            prep.add(prep_kv(2))
            plan[0] = TILE0_PLAN
        elif (n, gp) == (0, 2):
            wait('kv3')
            prep.add(prep_kv(3))
            side.add(layernorm(1))
        elif n > 0 and gp == 0:
            plan[0] = NORM_PLAN
            delay[0] = 2
            if n == 1:
                wait('wo')
                prep.add(prep_o())
            if n + 1 < NTILE:
                side.add(layernorm(n + 1))
            else:
                wait('wq')
                plan[0] = QUERY_PLAN
                side.add(router())
                side.add(ffn())
                prep.add(prep_q())

    first_tokens()
    prep.add(more_weights())
    for n in range(NTILE):
        for gp in range(4):
            if n == 0 and gp:
                prep.drain()
            if n and not gp:
                side.drain()
            soon(lambda n=n, gp=gp: start_side_work(n, gp))
            kv_unit(gp, n)

    built = {}

    caught = [jnp.zeros((8, L), U32)] * (2 * KH)

    def catch_row(n, gp):
        for slab in (2 * gp, 2 * gp + 1):
            for h in range(2):
                k = sum(jnp.where(route['block'] == j, RAWL[j][h], 0) for j in range(4))
                words = (oa0, oa1)[n % 2].bitcast(U32)[k * KH + slab, pl.ds(route['word'], 8), :]
                caught[h * KH + slab] = jnp.where(route['tile'] == n, words, caught[h * KH + slab])

    def routed_projection():
        hit = lax.broadcasted_iota(jnp.int32, (16, L), 0) == route['idx'] % 16
        for t in range(2 * KH):
            row = jnp.sum(jnp.where(hit, _unpack(caught[t]).astype(F32), 0.0), axis=0, keepdims=True)
            ob[pl.ds(t * L, L), :] = jnp.broadcast_to(row, (L, L)).T
            if t % 2:
                yield
        for t in range(0, 8, 2):
            for p in range(2 * NSUB):
                matvec(WO, t * L, ob, p * FROWS, lambda u: OPART + (t + u) * 2 * NSUB + p)
                yield
        s = [_total([part[OPART + t * 2 * NSUB + p] for p in range(2 * NSUB)]) for t in range(8)]
        route['s'] = jnp.sum(jnp.concatenate(s, axis=1), axis=0, keepdims=True)

    def o_operands(n, gp):
        oa = (oa0, oa1)[n % 2]
        release[0] = oa.at[OSPARE]
        for slab in (2 * gp, 2 * gp + 1):
            def store(k, r0, v):
                stored.add(f'oa{n % 2}')
                oa[k * KH + slab, pl.ds(r0, 16), :] = v.astype(BF)
            yield from build(lambda k, r0: oa.bitcast(U32)[k * KH + slab, pl.ds(r0 // 2, 8), :], store)
        built[n] = built.get(n, 0) + 1

    def q_unit(gp, n):
        while ('q', gp) not in ready:
            prep.step()
        left = [16]
        oa = (oa0, oa1)[n % 2]

        def attend(i, j, feats):
            rows = []
            for pp, (phi, scale) in enumerate(feats):
                nd = _dot(_unpack(kvl.bitcast(U32)[2 * q_groups(gp)[i] + pp]), phi, NN)
                inv = _rcp(nd[64:72] + 1e-6 * scale)
                for head in range(2):
                    rd = jnp.broadcast_to(inv[head:head + 1], (8, L))
                    rows += [nd[head * DH + 8 * q:head * DH + 8 * q + 8] * rd for q in range(4)]
                if pp == 0:
                    yield
            oa[RAWL[j][i % 2] * KH + 2 * gp + i // 2] = jnp.concatenate(rows, axis=0).T.astype(BF)
            left[0] -= 1
            if not left[0]:
                catch_row(n, gp)
                prep.add(o_operands(n, gp))
                if (n, gp) == (NTILE - 1, 1):
                    extra.add(routed_projection())
            yield

        def on_block(i, j, c):
            tail.add(after(4, attend(i, j, [_query_features(c[pp * 64:(pp + 1) * 64]) for pp in range(2)])))

        unit(lambda k: slabs(AQ, 2 * L, k, gp * L // 2, L),
             lambda k: slabs(XS, XR, k, n * L // 2, L), NT, on_block)

    def o_unit(c, n):
        left = [16]

        def finish(j, col, s):
            rows = pl.ds(n * TT + j * L, L)
            cols = pl.ds(c * HK + col * L, L)
            half = _unpack(ar_w[pl.ds((XS + (RAW[j][c] * KH + col) * XR + n * L) // 2, L // 2), :]).astype(F32)
            sh = s * half
            out_v[rows, cols] = (wide[rows, cols].astype(F32) + sh + sh * jnp.tanh(half)).astype(BF)
            left[0] -= 1
            if (n, c) == (NTILE - 1, 1):
                out_copy(rows.start, rows.start, L, cols.start, L, 1).start()
            elif not left[0]:
                out_copy(n * TT, n * TT, TT, c * HK, HK, int(n == NTILE - 1)).start()
            yield

        if c == 0:
            if n == NTILE - 1:
                drain_tail()
            while built.get(n, 0) < 2:
                (prep if prep.q else tail).step()
        oa = (oa0, oa1)[n % 2].bitcast(U32)
        unit(lambda k: jnp.concatenate([oa[k * KH + s] for s in range(KH)], axis=1),
             lambda k: ar_w[pl.ds((BO + (k * 2 + c) * HK) // 2, HK // 2), :], NN,
             lambda j, col, s: tail2.add(finish(j, col, s)))

    dots.update((count[0] + 1 + t, int(n)) for t, n in enumerate(DOT_PLAN))
    plan[:] = [OUT_PLAN, count[0]]
    delay[0] = 1
    q_unit(0, 0)
    soon(lambda: wait('ffn'))
    soon(lambda: ready.add('ffn'))
    q_unit(1, 0)
    for n in range(1, NTILE):
        for gp in range(2):
            q_unit(gp, n)
            o_unit(gp, n - 1)
    for c in range(2):
        o_unit(c, NTILE - 1)
    drain_tail()
    tail2.drain()
    side.drain()
    extra.drain()

    row0 = pl.multiple_of((route['idx'] // 16) * 16, 16)
    half = 0.5 * (route['row'] + route['y'])
    sh = route['s'] * half
    fixed = wide[pl.ds(row0, 16), :].astype(F32) + (sh + sh * jnp.tanh(half))
    hit = lax.broadcasted_iota(jnp.int32, (16, D), 0) == route['idx'] % 16
    out_v[pl.ds(S, 16), :] = jnp.where(hit, fixed, out_v[pl.ds(row0, 16), :].astype(F32)).astype(BF)
    rows_copy = out_copy(S, row0, 16, 0, D, 2)
    for _ in range(2 * NTILE - 2):
        out_copy(0, 0, TT, 0, HK, 0).wait()
    pl.when(route['tile'] != NTILE - 1)(rows_copy.start)
    out_copy(0, 0, TT, 0, HK, 1).wait()
    for _ in range(16):
        out_copy(0, 0, L, 0, L, 1).wait()
    pl.when(route['tile'] == NTILE - 1)(rows_copy.start)
    rows_copy.wait()


@jax.jit
def pallas_recurrent_scan__linear_kernel_hedgehog__moe_arch_mod__prompt_kernel(
    A_x: jax.Array,
    A_wqkv: jax.Array,
    A_w_phi: jax.Array,
    A_wo: jax.Array,
    B_x: jax.Array,
    B_w_r: jax.Array,
    B_w_gate: jax.Array,
    B_w_up: jax.Array,
    B_w_down: jax.Array,
):
    del B_x
    hbm = pl.BlockSpec(memory_space=pl.ANY)
    return pl.pallas_call(
        _kernel,
        out_shape=jax.ShapeDtypeStruct(A_x.shape, A_x.dtype),
        in_specs=[hbm] * 8,
        out_specs=hbm,
        scratch_shapes=[
            pltpu.VMEM((ANCHOR + 8, D), BF),
            pltpu.VMEM((3 * NG, D, L), BF),
            pltpu.VMEM((H, DH, DH), BF),
            pltpu.VMEM((D,), BF),
            pltpu.VMEM((NG, L, L), BF),
            pltpu.VMEM((NPART + 1, 8, L), F32),
            pltpu.VMEM((65, 16, L), F32),
            pltpu.VMEM((SPARE + 16, L), BF),
            pltpu.VMEM((33, L, L), BF),
            pltpu.VMEM((OSPARE + 1, L, L), BF),
            pltpu.VMEM((OSPARE + 1, L, L), BF),
            pltpu.VMEM((NP, 80, L), BF),
            pltpu.VMEM((NP, 80, L), F32),
            pltpu.VMEM((S + 16, D), BF),
            pltpu.VMEM((D, L), F32),
            pltpu.VMEM((D, L), F32),
            pltpu.VMEM((NFC, FC, L), F32),
            pltpu.SemaphoreType.DMA((12,)),
        ],
        compiler_params=pltpu.CompilerParams(vmem_limit_bytes=120 << 20),
        name="hedgehog_mod",
    )(A_x, A_wqkv, A_w_phi, A_wo, B_w_r, B_w_gate, B_w_up, B_w_down)
```

```python
import jax
import jax.numpy as jnp
from jax import lax
import jax.experimental.pallas as pl
import jax.experimental.pallas.tpu as pltpu

BF = jnp.bfloat16
F32 = jnp.float32
U32 = jnp.uint32
NN = (((1,), (0,)), ((), ()))
NT = (((1,), (1,)), ((), ()))
LOG2E = 1.4426950408889634

S, D, H, DH, FF = 2048, 1024, 32, 32, 3584
L = 128
HK = D // 2
KH = HK // L
NG = H // 4
NP = H // 2
TT = 4 * L
NTILE = S // TT
FC = 4 * L
NFC = FF // FC
FROWS = 128
NSUB = HK // FROWS
EARLY = 3
NOP = 26
RAW = ((1, 26), (27, 2), (7, 8), (16, 28))
RAWL = ((26, 0), (3, 27), (7, 8), (28, 15))
STAGE = {k: i for i, k in enumerate(sum(RAWL, ()))}

XR = S // 4
XS = 0
AKV = XS + (NOP + 3) * KH * XR
AQ = AKV + NOP * KH * 4 * L
BO = AQ + NOP * KH * 2 * L
SPARE = BO + NOP * 2 * HK
GU = S
WD = GU + NFC * D
WO = WD + FF
ANCHOR = WO + D
OPART = (32 + 8 * NFC) * NSUB
NPART = OPART + 16 * NSUB
OSPARE = (NOP + 3) * KH

PIECES = {'.': (0, 0), 'L': (1, 0), '2': (2, 0), 'P': (0, 1), '3': (0, 2), '5': (0, 3), '9': (0, 8),
          'B': (1, 1), '6': (1, 2), 'E': (0, 0)}
FIRST_PLAN = '35.35P55935535355555353535'
TILE0_PLAN = '.' * NOP + 'PPP3PPPP3P3PP3P33PP33P3P3P' '3B63BB6PBBB6B6B3BBB666PBB3' '2L2LL222L2L2222LL2LLLLLLLL'
NORM_PLAN = ('PPLLLBL.PPPLLL.L.LBLL.LLPP' 'PPLLLBL.PPPLLL.L.LBLL.LLPP'
             'PLLLLBL.PPPLLL.L.LBLP.LLPP' 'PPBLLBL.LLPLLL.B.PBLL..L.P')
QUERY_PLAN = ('PBBLBBLBBBBB.BBBBBBBBBBLB.' 'BBBBLBB.BLBBLBBBBBPBBBPLBB'
              'LPLBBBPBBBBBBBBBBBB.BBLLBB' 'LBBBBBLBBBBBLBBBBBBBBBPLP.')
OUT_PLAN = ('L.L.LL.LLLL.LLLLLLLLL.LLL.' 'LBLLLL.LLLBPBPBLPPPPBPBPBB'
            '.LBP.LPLPLBPPLPBLPPPBLPPBP' 'LBLPLP.LLBPP.BBLBBLPL.LBL.'
            + ('LL.LLLLLBBPLPLP.BPLLPLPLBL' 'LPLLLBPLPBLPL.PLLBPLBLLBLL') * 4
            + 'LLLPLLBLBL.PLBLLPPLLPLLLBL' 'BBBLLLBPPBLPLBPPBPPPPPBPPP'
            'ELELELELLLELELELELLLEEEEEL' 'LEEEEEEEEEEEEEEEEEEEEEEEE.')
DOT_PLAN = ('11221121111111112211111222' '22111211211222112211121222'
            '12121211111111111111111111' '11111111111111121111111111'
            + ('11111112111211111112111121' '11211111111111111211111111') * 4
            + '11121211112211111211111111' '11211111111111111111111111'
            '11111111111111111111111111' '11111111111111111111111111')


def _dot(a, b, dims):
    return lax.dot_general(a, b, dims, preferred_element_type=F32)


def _unpack(words):
    return pltpu.bitcast(words, BF)


def _rnd(v):
    return v.astype(BF).astype(F32)


def _rcp(v):
    return pltpu.reciprocal(v, approx=True)


def _silu(v):
    h = 0.5 * v
    return h + h * jnp.tanh(h)


def _total(v):
    while len(v) > 1:
        v = [v[i] + v[i + 1] for i in range(0, len(v), 2)]
    return v[0]


def _pair_reduce(v, reduce, op):
    r = reduce(v, axis=0)
    r = op(r, pltpu.roll(r, 2, 0))
    return op(r, pltpu.roll(r, 4, 0))


def _dual_exp(p):
    v = p.reshape(8, 8, L)
    ep = jnp.exp2(v - _pair_reduce(v, jnp.max, jnp.maximum))
    en = jnp.exp2(_pair_reduce(v, jnp.min, jnp.minimum) - v)
    return ep, en, _pair_reduce(ep, jnp.sum, jnp.add), _pair_reduce(en, jnp.sum, jnp.add)


def _key_features(p):
    ep, en, sp, sn = _dual_exp(p)
    return jnp.concatenate([ep * _rcp(sp), en * _rcp(sn)], axis=0).reshape(L, L).astype(BF)


def _query_features(p):
    ep, en, sp, sn = _dual_exp(p)
    return jnp.concatenate([ep, en * (sp * _rcp(sn))], axis=0).reshape(L, L).astype(BF), sp


class _Signed:
    def __init__(self, sign, v):
        self.sign, self.v = sign, v

    def __neg__(self):
        return _Signed(-self.sign, self.v)

    def __add__(self, o):
        if self.sign == o.sign:
            return _Signed(self.sign, self.v + o.v)
        return _Signed(1, self.v - o.v if self.sign > 0 else o.v - self.v)

    def __sub__(self, o):
        return self + (-o)


def _nxt(k, d=1):
    return (k - 1 + d) % 3 + 1


def _operands(block, left):
    lo, hi = (1, 2) if left else (2, 1)

    def forms(i):
        x, y = block(i)
        if left:
            return {1: _Signed(1, x), 2: _Signed(-1, y), 3: _Signed(1, y - x)}
        return {1: _Signed(1, y), 2: _Signed(1, x), 3: _Signed(-1, x + y)}

    def diag(g, k):
        yield g[_nxt(k, lo)]
        yield g[_nxt(k, hi)]

    def pair(ga, gb, k, s):
        m = _nxt(k, 2)
        yield gb[k] - ga[_nxt(k)] if left else ga[_nxt(k)] - gb[k]
        for n in (_nxt(m, lo), _nxt(m, hi)):
            s[n] = ga[n] + gb[n]
            yield s[n]

    f0 = forms(0)
    yield from diag(f0, 1)
    f1 = forms(1)
    yield from diag(f1, 2)
    yield from pair(f0, f1, 1, {})
    f2 = forms(2)
    yield from diag(f2, 3)
    yield from pair(f1, f2, 2, {})
    s02 = {}
    yield from pair(f2, f0, 3, s02)
    s02[2] = f0[2] + f2[2]
    f3 = forms(3)
    yield from diag(f3, 1)
    yield from pair(f2, f3, 3, {})
    yield from pair(f3, s02, 1, {})
    yield from pair(f3, f1, 1, {})


_SIGNS = [a.sign * b.sign for a, b in zip(_operands(lambda i: (0, 0), True), _operands(lambda i: (0, 0), False))]


def _block_product(product):
    count = iter(range(NOP))

    def m(sign=1):
        k = next(count)
        return _Signed(sign * _SIGNS[k], product(k))

    def diag(i):
        x, y = m(), m(-1)
        yield i, i, x + y
        return x, y

    def pair(a, b, da, db, less=(None, None)):
        g = m()
        xs = m()
        ab = xs - da[1] - db[1] - g
        yield a, b, ab if less[0] is None else ab - less[0]
        ys = m(-1)
        ba = ys - da[0] - db[0] + g
        yield b, a, ba if less[1] is None else ba - less[1]
        return (xs, ys), (ab, ba)

    def steps():
        d0 = yield from diag(0)
        d1 = yield from diag(1)
        yield from pair(0, 1, d0, d1)
        d2 = yield from diag(2)
        yield from pair(1, 2, d1, d2)
        d02, _ = yield from pair(2, 0, d2, d0)
        d3 = yield from diag(3)
        _, (c23, c32) = yield from pair(2, 3, d2, d3)
        yield from pair(3, 0, d3, d02, (c32, c23))
        yield from pair(3, 1, d3, d1)

    for i, j, c in steps():
        assert c.sign > 0
        yield i, j, c.v


class _Tasks:
    def __init__(self):
        self.q = []

    def add(self, gen):
        self.q.append(gen)

    def step(self, n=1):
        while n > 0 and self.q:
            try:
                next(self.q[0])
                n -= 1
            except StopIteration:
                self.q.pop(0)

    def drain(self):
        while self.q:
            self.step()


def _kernel(x_hbm, wqkv_hbm, wphi_hbm, wo_hbm, wr_hbm, wg_hbm, wu_hbm, wd_hbm, out_hbm,
            wide, w_v, wphi_v, wr_v, fm_v, part, st, ar, stage, oa0, oa1, kvl, kv_acc, out_v, xb, ob, hb, sems):

    def x_rows(row0, rows):
        return x_hbm.at[0, pl.ds(row0, rows)], wide.at[pl.ds(row0, rows)]

    def w_cols(c):
        return wqkv_hbm.at[:, pl.ds(c * L, L)], w_v.at[c]

    def kv_cols(gp):
        return [w_cols(o + g) for g in (2 * gp, 2 * gp + 1) for o in (NG, 2 * NG)]

    def phi_heads(h0, heads):
        return wphi_hbm.at[pl.ds(h0, heads)], wphi_v.at[pl.ds(h0, heads)]

    def ffn_chunk(c):
        cols = pl.ds(c * FC, FC)
        rows = pl.ds(GU + c * D, D)
        return [(wg_hbm.at[:, cols], wide.at[rows, pl.ds(0, FC)]),
                (wu_hbm.at[:, cols], wide.at[rows, pl.ds(FC, FC)]),
                (wd_hbm.at[cols], wide.at[pl.ds(WD + c * FC, FC)])]

    loads = {
        'x00': [(wr_hbm, wr_v), x_rows(0, L)],
        'x01': [x_rows(L, L)],
        'x02': [x_rows(2 * L, L)],
        'x03': [x_rows(3 * L, L)],
        'kv0a': [phi_heads(0, 8)] + kv_cols(0)[:2],
        'kv0b': kv_cols(0)[2:],
        'kv1': [phi_heads(8, H - 8)] + kv_cols(1),
        'kv2': kv_cols(2),
        'kv3': [x_rows(TT, TT)] + kv_cols(3),
        'wo': [x_rows(n * TT, TT) for n in range(2, NTILE)] + [(wo_hbm, wide.at[pl.ds(WO, D)])],
        'wq': [w_cols(g) for g in range(NG)] + [p for c in range(EARLY) for p in ffn_chunk(c)],
        'ffn': [p for c in range(EARLY, NFC) for p in ffn_chunk(c)],
    }

    def copies(name):
        return [pltpu.make_async_copy(src, dst, sems.at[list(loads).index(name)]) for src, dst in loads[name]]

    def wait(name):
        for cp in copies(name):
            cp.wait()

    def out_copy(src0, dst0, rows, col0, cols, sem):
        return pltpu.make_async_copy(out_v.at[pl.ds(src0, rows), pl.ds(col0, cols)],
                                     out_hbm.at[0, pl.ds(dst0, rows), pl.ds(col0, cols)], sems.at[sem])

    for name in loads:
        for cp in copies(name):
            cp.start(priority=1)

    ar_w = ar.bitcast(U32)
    stored = set()
    ready = set()

    wait('x00')
    wr1 = wr_v[...].astype(F32).reshape(1, D)
    zero = pl.multiple_of(jnp.max(jnp.where(jnp.abs(wr1) < 0.0, pltpu.bitcast(wr1, jnp.int32), 0)), 16)
    never = zero > 0
    ar[pl.ds(SPARE, 16), :] = jnp.zeros((16, L), BF)
    part[NPART] = jnp.zeros((8, L), F32)
    st[64] = jnp.zeros((16, L), F32)
    stage[32, pl.ds(0, 16), :] = jnp.zeros((16, L), BF)
    for oa in (oa0, oa1):
        oa[OSPARE, pl.ds(0, 16), :] = jnp.zeros((16, L), BF)

    def fold_matrices(groups):
        rr = lax.broadcasted_iota(jnp.int32, (L, DH), 0)
        ff = lax.broadcasted_iota(jnp.int32, (L, DH), 1)
        sel = jnp.where(((rr & 63) >> 1) == ff, 1.0, 0.0).astype(BF)
        r2 = lax.broadcasted_iota(jnp.int32, (L, L), 0)
        c2 = lax.broadcasted_iota(jnp.int32, (L, L), 1)
        own = ((r2 >> 6) * 2 + (r2 & 1)) == (c2 >> 5)
        for g in groups:
            a = wphi_v[4 * g:4 * g + 4].reshape(L, DH)
            fm_v[g] = jnp.where(own, _dot(sel, a, NT), 0.0).astype(BF)

    def put(row, v):
        stored.add('ar')
        ar[pl.ds(row, v.shape[0]), :] = v.astype(BF)

    def slabs(start, stride, k, row0, rows):
        return jnp.concatenate(
            [ar_w[pl.ds((start + s * stride) // 2 + k * (KH * stride // 2) + row0, rows // 2), :]
             for s in range(KH)], axis=1)

    def folded(g, c, s):
        w = _unpack(w_v.bitcast(U32)[c, pl.ds(s * L // 2, L // 2), :])
        return _dot(_unpack(fm_v.bitcast(U32)[g]), w, NT) * (2.0 * LOG2E)

    def build(load, store, slots=range(NOP)):
        for r0 in range(0, L, 16):
            for k, v in enumerate(_operands(lambda i: [_unpack(load(k, r0)).astype(F32) for k in RAWL[i]], True)):
                if k in slots and k not in STAGE:
                    store(k, r0, v.v)
                if k == slots[-1]:
                    break
            yield

    def arena_build(row_of, slots=range(NOP)):
        return build(lambda k, r0: stage.bitcast(U32)[row_of(k)[1], pl.ds(r0 // 2, 8), :],
                     lambda k, r0, v: put(row_of(k)[0] + r0, v), slots)

    def put_plain(row_of, k, v):
        stored.add('stage')
        v = v.astype(BF)
        stage[row_of(k)[1]] = v
        if k < NOP:
            ar[pl.ds(row_of(k)[0], L), :] = v

    def kv_rows(gp, s):
        return lambda k: (AKV + ((k * KH + s) * 4 + gp) * L, 8 * s + STAGE.get(k, 0))

    def plain_kv(gp, s, which=(0, 1)):
        for i in which:
            g = 2 * gp + i
            for h in range(2):
                put_plain(kv_rows(gp, s), RAWL[2 * i][h], folded(g, NG + g, h * KH + s))
                put_plain(kv_rows(gp, s), RAWL[2 * i + 1][h], w_v[2 * NG + g, pl.ds(h * HK + s * L, L), :].T)

    def prep_kv(gp):
        for s in range(KH):
            plain_kv(gp, s)
            yield
            yield from arena_build(kv_rows(gp, s))

    def q_groups(gp):
        return (2 * gp, KH + 2 * gp, 2 * gp + 1, KH + 2 * gp + 1)

    def prep_q():
        for gp in range(2):
            for s in range(KH):
                def row_of(k):
                    return AQ + ((k * KH + s) * 2 + gp) * L, 8 * s + STAGE.get(k, 0)
                for i, g in enumerate(q_groups(gp)):
                    for h in range(2):
                        put_plain(row_of, RAWL[i][h], folded(g, g, h * KH + s))
                    if i % 2:
                        yield
                yield from arena_build(row_of)
            ready.add(('q', gp))

    def prep_o():
        for c in range(2):
            for r0 in range(0, HK, 16):
                blk = [wide[pl.ds(WO + h * HK + r0, 16), pl.ds(c * HK, HK)].astype(F32) for h in range(2)]
                for k, v in enumerate(_operands(lambda j: [b[:, j * L:(j + 1) * L] for b in blk], False)):
                    put(BO + (k * 2 + c) * HK + r0, v.v)
                yield

    wr = jnp.broadcast_to(wr1, (16, D))
    best = [jnp.full((16, 1), -jnp.inf, F32), jnp.zeros((16, 1), jnp.int32)]

    def row_mean(n, c, j):
        xf = wide[pl.ds(n * TT + j * L + c * 16, 16), :].astype(F32)
        mean = jnp.sum(xf, axis=1, keepdims=True) * (1.0 / D)
        stored.add('st')
        st[8 * c + 2 * j] = jnp.broadcast_to(mean, (16, L))

    def row_stats(n, c, j):
        r0 = n * TT + j * L + c * 16
        d = wide[pl.ds(r0, 16), :].astype(F32) - jnp.concatenate([st[8 * c + 2 * j]] * (D // L), axis=1)
        var = jnp.sum(d * d, axis=1, keepdims=True) * (1.0 / D)
        rs = _rcp(_rnd(jnp.sqrt(_rnd(_rnd(var) + 1e-5))))
        r = jnp.sum(d * wr, axis=1, keepdims=True) * rs
        up = (r > best[0]) | ((r == best[0]) & (r0 < best[1]))
        best[0] = jnp.where(up, r, best[0])
        best[1] = jnp.where(up, r0, best[1])
        stored.add('st')
        st[8 * c + 2 * j + 1] = jnp.broadcast_to(0.5 * rs, (16, L))
        st[64, pl.ds(8, 8), :] = jnp.broadcast_to(jnp.maximum(best[0][:8], best[0][8:]), (8, L))

    def token_operands(n, c, s):
        row = XS + s * XR + n * L + c * 16

        def block(j):
            b = [(wide[pl.ds(n * TT + j * L + c * 16, 16), pl.ds(h * HK + s * L, L)].astype(F32)
                  - st[8 * c + 2 * j]) * st[8 * c + 2 * j + 1] for h in range(2)]
            for k, v in zip(RAW[j], b):
                if k >= NOP:
                    put(row + k * KH * XR, v)
            return b

        for k, v in enumerate(_operands(block, False)):
            put(row + k * KH * XR, v.v)

    def layernorm(n):
        for j in range(4):
            row_mean(n, 0, j)
        yield
        for c in range(L // 16):
            for j in range(4):
                row_stats(n, c, j)
                if j % 2:
                    yield
            if c + 1 < L // 16:
                for j in range(4):
                    row_mean(n, c + 1, j)
                yield
            for s in range(KH):
                token_operands(n, c, s)
                yield

    side, prep, tail, tail2, extra = _Tasks(), _Tasks(), _Tasks(), _Tasks(), _Tasks()
    count = [0]
    plan = [FIRST_PLAN, 0]
    delay = [1]
    timed, pending, dots, flush = {}, [], {}, []
    release = [stage.at[32]]

    def anchor(v):
        wide[pl.ds(ANCHOR + zero, 8), pl.ds(0, 2 * L)] = v.astype(BF)

    def probe(name):
        if name == 'ar':
            return ar_w[pl.ds(SPARE // 2 + zero, 8), :]
        if name == 'part':
            return pltpu.bitcast(part[NPART + zero], U32)
        if name == 'st':
            return pltpu.bitcast(st[64, pl.ds(zero, 8), :], U32)
        if name == 'stage':
            return stage.bitcast(U32)[32, pl.ds(zero, 8), :]
        return (oa0, oa1)[name == 'oa1'].bitcast(U32)[OSPARE, pl.ds(zero, 8), :]

    def gap(m):
        count[0] += 1
        for action in timed.pop(count[0], ()):
            action()
        due = pending.pop(0) if len(pending) > delay[0] else ()
        if due:
            tied = pltpu.bitcast(m[96:104], U32)
            for name in due:
                tied = jnp.where(never, probe(name), tied)
            m = jnp.concatenate([m[:96], pltpu.bitcast(tied, F32), m[104:]], axis=0)
        if side.q or prep.q or extra.q:
            anchor(jnp.concatenate([m[:8], m[8:16]], axis=1))
        if prep.q:
            release[0][pl.ds(zero + 16, 16), :] = m[:16].astype(BF)
        tail.step(dots.get(count[0], 1))
        tail2.step()
        todo = plan[0][(count[0] - plan[1] - 1) % len(plan[0])]
        side.step(PIECES[todo][0])
        prep.step(PIECES[todo][1])
        extra.step(todo == 'E')
        pending.append(sorted(stored))
        stored.clear()
        return m

    def soon(action):
        timed.setdefault(count[0] + 1, []).append(action)

    def after(products, gen):
        start = count[0] + products

        def held():
            while count[0] < start and not flush:
                yield
            yield from gen
        return held()

    def drain_tail():
        flush.append(1)
        tail.drain()
        flush.clear()

    def unit(lhs, rhs, dims, on_block):
        for i, j, c in _block_product(lambda k: gap(_dot(_unpack(lhs(k)), _unpack(rhs(k)), dims))):
            on_block(i, j, c)

    route = {}

    def router():
        slot = lax.broadcasted_iota(jnp.int32, (16, 1), 0)
        lane_rows = lax.broadcasted_iota(jnp.int32, (16, D), 0)
        rows = jnp.zeros((16, D), F32)
        for i in range(16):
            group = pl.multiple_of(jnp.max(jnp.where(slot == i, best[1], 0)), 16)
            rows = jnp.where(lane_rows == i, wide[pl.ds(group, 16), :].astype(F32), rows)
        mean = jnp.sum(rows, axis=1, keepdims=True) * (1.0 / D)
        var = jnp.sum((rows - mean) * (rows - mean), axis=1, keepdims=True) * (1.0 / D)
        xn = _rnd(_rnd(rows - _rnd(mean)) / _rnd(jnp.sqrt(_rnd(_rnd(var) + 1e-5))))
        score = _rnd(jnp.sum(xn * wr, axis=1, keepdims=True))
        rmax = jnp.max(score)
        idx = jnp.min(jnp.where(score == rmax, best[1] + slot, S - 1))
        row = jnp.sum(jnp.where(lane_rows == idx % 16, xn, 0.0), axis=0, keepdims=True)
        route.update(rmax=rmax, idx=idx, row=row, tile=idx // TT, block=(idx // L) % 4,
                     word=pl.multiple_of(((idx % L) // 16) * 8, 8))
        for t in range(D // L):
            xb[pl.ds(t * L, L), :] = jnp.broadcast_to(row[:, t * L:(t + 1) * L], (L, L)).T
            yield

    def matvec(row0, col0, vec, k0, slot):
        vk = vec[pl.ds(k0, FROWS), :]
        wk = wide[pl.ds(row0 + k0, FROWS), pl.ds(col0, 2 * L)].astype(F32)
        pr = wk * jnp.concatenate([vk, vk], axis=1)
        acc = jnp.sum(pr.reshape(FROWS // 8, 8, 2 * L), axis=0)
        stored.add('part')
        for t in range(2):
            part[slot(t)] = acc[:, t * L:(t + 1) * L]

    def ffn():
        def gu_slot(c, t, p):
            return ((c % 2) * 8 + t) * 2 * NSUB + p

        def y_slot(c, t, p):
            return 32 * NSUB + (t * NFC + c) * NSUB + p

        def column(c, t):
            return jnp.sum(_total([part[gu_slot(c, t, p)] for p in range(2 * NSUB)]), axis=0, keepdims=True)

        def down(c):
            for t in range(0, 8, 2):
                for p in range(NSUB):
                    matvec(WD + c * FC, t * L, hb.at[c], p * FROWS, lambda u: y_slot(c, t + u, p))
                    yield

        for c in range(NFC):
            while c == EARLY and 'ffn' not in ready:
                yield
            for t in range(0, 8, 2):
                for p in range(2 * NSUB):
                    matvec(GU + c * D, t * L, xb, p * FROWS, lambda u: gu_slot(c, t + u, p))
                    yield
            for t in range(4):
                gate, up = column(c, t), column(c, 4 + t)
                hb[c, pl.ds(t * L, L), :] = jnp.broadcast_to(_silu(gate) * up, (L, L)).T
            yield
            if c > 0:
                yield from down(c - 1)
        yield
        yield from down(NFC - 1)
        y = [sum(_total([part[y_slot(c, t, p)] for p in range(NSUB)]) for c in range(NFC)) for t in range(8)]
        gate = 1.0 / (1.0 + jnp.exp(-jnp.full((1, D), route['rmax'], F32)))
        route['y'] = jnp.sum(jnp.concatenate(y, axis=1), axis=0, keepdims=True) * gate

    def finish_pair(p, sums):
        r = lax.broadcasted_iota(jnp.int32, (80, L), 0)
        c = lax.broadcasted_iota(jnp.int32, (80, L), 1)
        keep = jnp.where(r < 64, r >> 5, r & 1) == (c & 1)
        kvl[p] = jnp.where(keep, jnp.concatenate([2.0 * sums[:64], sums[64:]], axis=0), 0.0).astype(BF)

    def kv_unit(gp, n):
        seen, acc = {}, {}

        def combine(g, phis, vts):
            for pp in range(2):
                p = 2 * g + pp
                acc[p] = acc.get(p, []) + [_dot(vts[pp], phis[pp], NT)]
                if len(acc[p]) == 4:
                    upd = _total(acc[p]) if n == 0 else kv_acc[p] + _total(acc[p])
                    if n < NTILE - 1:
                        kv_acc[p] = upd
                    else:
                        finish_pair(p, upd)
                yield

        def on_block(i, j, c):
            if i % 2:
                seen[i, j] = [jnp.concatenate([c[pp * 64:(pp + 1) * 64], jnp.ones((16, L), F32)], axis=0).astype(BF)
                              for pp in range(2)]
            else:
                seen[i, j] = [_key_features(c[pp * 64:(pp + 1) * 64]) for pp in range(2)]
            if (i ^ 1, j) in seen:
                tail.add(after(3, combine(2 * gp + i // 2, seen[i & 2, j], seen[i | 1, j])))

        def weights(k):
            while (gp, n) == (0, 0) and k in (7, 15) and k not in ready:
                prep.step()
            return slabs(AKV, 4 * L, k, gp * L // 2, L)

        unit(weights, lambda k: slabs(XS, XR, k, n * L // 2, L), NT, on_block)

    def first_tokens():
        for j in range(4):
            if j:
                wait(f'x0{j}')
            for part_of in (row_mean, row_stats):
                for c in range(L // 16):
                    part_of(0, c, j)
                anchor(jnp.zeros((8, 2 * L), BF))
        done = []
        for c in range(L // 16):
            for s in range(KH):
                if len(done) == 28:
                    wait('kv0a')
                    fold_matrices(range(2))
                    for t in range(KH):
                        plain_kv(0, t, (0,))
                        prep.add(arena_build(kv_rows(0, t), range(7)))
                if len(done) >= 3:
                    anchor(jnp.concatenate([done[-3], done[-3]], axis=1))
                token_operands(0, c, s)
                prep.step(2)
                done.append(pltpu.bitcast(probe('ar'), F32))
        prep.drain()

    def more_weights():
        while count[0] < 3:
            yield
        wait('kv0b')
        for s in range(KH):
            plain_kv(0, s, (1,))
            yield
        for slots in (range(7, 15), range(15, NOP)):
            for s in range(KH):
                yield from arena_build(kv_rows(0, s), slots)
            ready.add(slots[0])
        while count[0] < 16:
            yield
        wait('kv1')
        fold_matrices(range(2, NG))
        yield from prep_kv(1)

    def start_side_work(n, gp):
        if (n, gp) == (0, 1):
            wait('kv2')
            prep.add(prep_kv(2))
            plan[0] = TILE0_PLAN
        elif (n, gp) == (0, 2):
            wait('kv3')
            prep.add(prep_kv(3))
            side.add(layernorm(1))
        elif n > 0 and gp == 0:
            plan[0] = NORM_PLAN
            delay[0] = 2
            if n == 1:
                wait('wo')
                prep.add(prep_o())
            if n + 1 < NTILE:
                side.add(layernorm(n + 1))
            else:
                wait('wq')
                plan[0] = QUERY_PLAN
                side.add(router())
                side.add(ffn())
                prep.add(prep_q())

    first_tokens()
    prep.add(more_weights())
    for n in range(NTILE):
        for gp in range(4):
            if n == 0 and gp:
                prep.drain()
            if n and not gp:
                side.drain()
            soon(lambda n=n, gp=gp: start_side_work(n, gp))
            kv_unit(gp, n)

    built = {}

    caught = [jnp.zeros((8, L), U32)] * (2 * KH)

    def catch_row(n, gp):
        for slab in (2 * gp, 2 * gp + 1):
            for h in range(2):
                k = sum(jnp.where(route['block'] == j, RAWL[j][h], 0) for j in range(4))
                words = (oa0, oa1)[n % 2].bitcast(U32)[k * KH + slab, pl.ds(route['word'], 8), :]
                caught[h * KH + slab] = jnp.where(route['tile'] == n, words, caught[h * KH + slab])

    def routed_projection():
        hit = lax.broadcasted_iota(jnp.int32, (16, L), 0) == route['idx'] % 16
        for t in range(2 * KH):
            row = jnp.sum(jnp.where(hit, _unpack(caught[t]).astype(F32), 0.0), axis=0, keepdims=True)
            ob[pl.ds(t * L, L), :] = jnp.broadcast_to(row, (L, L)).T
            if t % 2:
                yield
        for t in range(0, 8, 2):
            for p in range(2 * NSUB):
                matvec(WO, t * L, ob, p * FROWS, lambda u: OPART + (t + u) * 2 * NSUB + p)
                yield
        s = [_total([part[OPART + t * 2 * NSUB + p] for p in range(2 * NSUB)]) for t in range(8)]
        route['s'] = jnp.sum(jnp.concatenate(s, axis=1), axis=0, keepdims=True)

    def o_operands(n, gp):
        oa = (oa0, oa1)[n % 2]
        release[0] = oa.at[OSPARE]
        for slab in (2 * gp, 2 * gp + 1):
            def store(k, r0, v):
                stored.add(f'oa{n % 2}')
                oa[k * KH + slab, pl.ds(r0, 16), :] = v.astype(BF)
            yield from build(lambda k, r0: oa.bitcast(U32)[k * KH + slab, pl.ds(r0 // 2, 8), :], store)
        built[n] = built.get(n, 0) + 1

    def q_unit(gp, n):
        while ('q', gp) not in ready:
            prep.step()
        left = [16]
        oa = (oa0, oa1)[n % 2]

        def attend(i, j, feats):
            rows = []
            for pp, (phi, scale) in enumerate(feats):
                nd = _dot(_unpack(kvl.bitcast(U32)[2 * q_groups(gp)[i] + pp]), phi, NN)
                inv = _rcp(nd[64:72] + 1e-6 * scale)
                for head in range(2):
                    rd = jnp.broadcast_to(inv[head:head + 1], (8, L))
                    rows += [nd[head * DH + 8 * q:head * DH + 8 * q + 8] * rd for q in range(4)]
                if pp == 0:
                    yield
            oa[RAWL[j][i % 2] * KH + 2 * gp + i // 2] = jnp.concatenate(rows, axis=0).T.astype(BF)
            left[0] -= 1
            if not left[0]:
                catch_row(n, gp)
                prep.add(o_operands(n, gp))
                if (n, gp) == (NTILE - 1, 1):
                    extra.add(routed_projection())
            yield

        def on_block(i, j, c):
            tail.add(after(4, attend(i, j, [_query_features(c[pp * 64:(pp + 1) * 64]) for pp in range(2)])))

        unit(lambda k: slabs(AQ, 2 * L, k, gp * L // 2, L),
             lambda k: slabs(XS, XR, k, n * L // 2, L), NT, on_block)

    def o_unit(c, n):
        left = [16]

        def finish(j, col, s):
            rows = pl.ds(n * TT + j * L, L)
            cols = pl.ds(c * HK + col * L, L)
            half = _unpack(ar_w[pl.ds((XS + (RAW[j][c] * KH + col) * XR + n * L) // 2, L // 2), :]).astype(F32)
            sh = s * half
            out_v[rows, cols] = (wide[rows, cols].astype(F32) + sh + sh * jnp.tanh(half)).astype(BF)
            left[0] -= 1
            if (n, c) == (NTILE - 1, 1):
                out_copy(rows.start, rows.start, L, cols.start, L, 1).start()
            elif not left[0]:
                out_copy(n * TT, n * TT, TT, c * HK, HK, int(n == NTILE - 1)).start()
            yield

        if c == 0:
            if n == NTILE - 1:
                drain_tail()
            while built.get(n, 0) < 2:
                (prep if prep.q else tail).step()
        oa = (oa0, oa1)[n % 2].bitcast(U32)
        unit(lambda k: jnp.concatenate([oa[k * KH + s] for s in range(KH)], axis=1),
             lambda k: ar_w[pl.ds((BO + (k * 2 + c) * HK) // 2, HK // 2), :], NN,
             lambda j, col, s: tail2.add(finish(j, col, s)))

    dots.update((count[0] + 1 + t, int(n)) for t, n in enumerate(DOT_PLAN))
    plan[:] = [OUT_PLAN, count[0]]
    delay[0] = 1
    q_unit(0, 0)
    soon(lambda: wait('ffn'))
    soon(lambda: ready.add('ffn'))
    q_unit(1, 0)
    for n in range(1, NTILE):
        for gp in range(2):
            q_unit(gp, n)
            o_unit(gp, n - 1)
    for c in range(2):
        o_unit(c, NTILE - 1)
    drain_tail()
    tail2.drain()
    side.drain()
    extra.drain()

    row0 = pl.multiple_of((route['idx'] // 16) * 16, 16)
    half = 0.5 * (route['row'] + route['y'])
    sh = route['s'] * half
    fixed = wide[pl.ds(row0, 16), :].astype(F32) + (sh + sh * jnp.tanh(half))
    hit = lax.broadcasted_iota(jnp.int32, (16, D), 0) == route['idx'] % 16
    out_v[pl.ds(S, 16), :] = jnp.where(hit, fixed, out_v[pl.ds(row0, 16), :].astype(F32)).astype(BF)
    rows_copy = out_copy(S, row0, 16, 0, D, 2)
    for _ in range(2 * NTILE - 2):
        out_copy(0, 0, TT, 0, HK, 0).wait()
    pl.when(route['tile'] != NTILE - 1)(rows_copy.start)
    out_copy(0, 0, TT, 0, HK, 1).wait()
    for _ in range(16):
        out_copy(0, 0, L, 0, L, 1).wait()
    pl.when(route['tile'] == NTILE - 1)(rows_copy.start)
    rows_copy.wait()


@jax.jit
def pallas_recurrent_scan__linear_kernel_hedgehog__moe_arch_mod__prompt_kernel(
    A_x: jax.Array,
    A_wqkv: jax.Array,
    A_w_phi: jax.Array,
    A_wo: jax.Array,
    B_x: jax.Array,
    B_w_r: jax.Array,
    B_w_gate: jax.Array,
    B_w_up: jax.Array,
    B_w_down: jax.Array,
):
    del B_x
    hbm = pl.BlockSpec(memory_space=pl.ANY)
    return pl.pallas_call(
        _kernel,
        out_shape=jax.ShapeDtypeStruct(A_x.shape, A_x.dtype),
        in_specs=[hbm] * 8,
        out_specs=hbm,
        scratch_shapes=[
            pltpu.VMEM((ANCHOR + 8, D), BF),
            pltpu.VMEM((3 * NG, D, L), BF),
            pltpu.VMEM((H, DH, DH), BF),
            pltpu.VMEM((D,), BF),
            pltpu.VMEM((NG, L, L), BF),
            pltpu.VMEM((NPART + 1, 8, L), F32),
            pltpu.VMEM((65, 16, L), F32),
            pltpu.VMEM((SPARE + 16, L), BF),
            pltpu.VMEM((33, L, L), BF),
            pltpu.VMEM((OSPARE + 1, L, L), BF),
            pltpu.VMEM((OSPARE + 1, L, L), BF),
            pltpu.VMEM((NP, 80, L), BF),
            pltpu.VMEM((NP, 80, L), F32),
            pltpu.VMEM((S + 16, D), BF),
            pltpu.VMEM((D, L), F32),
            pltpu.VMEM((D, L), F32),
            pltpu.VMEM((NFC, FC, L), F32),
            pltpu.SemaphoreType.DMA((12,)),
        ],
        compiler_params=pltpu.CompilerParams(vmem_limit_bytes=120 << 20),
        name="hedgehog_mod",
    )(A_x, A_wqkv, A_w_phi, A_wo, B_w_r, B_w_gate, B_w_up, B_w_down)
```

```python
import jax
import jax.numpy as jnp
from jax import lax
import jax.experimental.pallas as pl
import jax.experimental.pallas.tpu as pltpu

BF = jnp.bfloat16
F32 = jnp.float32
U32 = jnp.uint32
NN = (((1,), (0,)), ((), ()))
NT = (((1,), (1,)), ((), ()))
LOG2E = 1.4426950408889634

S, D, H, DH, FF = 2048, 1024, 32, 32, 3584
L = 128
HK = D // 2
KH = HK // L
NG = H // 4
NP = H // 2
TT = 4 * L
NTILE = S // TT
FC = 4 * L
NFC = FF // FC
FROWS = 128
NSUB = HK // FROWS
EARLY = 3
NOP = 26
RAW = ((1, 26), (27, 2), (7, 8), (16, 28))
RAWL = ((26, 0), (3, 27), (7, 8), (28, 15))
STAGE = {k: i for i, k in enumerate(sum(RAWL, ()))}

XR = S // 4
XS = 0
AKV = XS + (NOP + 3) * KH * XR
AQ = AKV + NOP * KH * 4 * L
BO = AQ + NOP * KH * 2 * L
SPARE = BO + NOP * 2 * HK
GU = S
WD = GU + NFC * D
WO = WD + FF
ANCHOR = WO + D
OPART = (32 + 8 * NFC) * NSUB
NPART = OPART + 16 * NSUB
OSPARE = (NOP + 3) * KH

PIECES = {'.': (0, 0), 'L': (1, 0), '2': (2, 0), 'P': (0, 1), '3': (0, 2), '5': (0, 3), '9': (0, 8),
          'B': (1, 1), '6': (1, 2), 'E': (0, 0)}
FIRST_PLAN = '35.35P55935535355555353535'
TILE0_PLAN = '.' * NOP + 'PPP3PPPP3P3PP3P33PP33P3P3P' '3B63BB6PBBB6B6B3BBB666PBB3' '2L2LL222L2L2222LL2LLLLLLLL'
NORM_PLAN = ('PPLLLBL.PPPLLL.L.LBLL.LLPP' 'PPLLLBL.PPPLLL.L.LBLL.LLPP'
             'PLLLLBL.PPPLLL.L.LBLP.LLPP' 'PPBLLBL.LLPLLL.B.PBLL..L.P')
QUERY_PLAN = ('PBBLBBLBBBBB.BBBBBBBBBBLB.' 'BBBBLBB.BLBBLBBBBBPBBBPLBB'
              'LPLBBBPBBBBBBBBBBBB.BBLLBB' 'LBBBBBLBBBBBLBBBBBBBBBPLP.')
OUT_PLAN = ('L.L.LL.LLLL.LLLLLLLLL.LLL.' 'LBLLLL.LLLBPBPBLPPPPBPBPBB'
            '.LBP.LPLPLBPPLPBLPPPBLPPBP' 'LBLPLP.LLBPP.BBLBBLPL.LBL.'
            + ('LL.LLLLLBBPLPLP.BPLLPLPLBL' 'LPLLLBPLPBLPL.PLLBPLBLLBLL') * 4
            + 'LLLPLLBLBL.PLBLLPPLLPLLLBL' 'BBBLLLBPPBLPLBPPBPPPPPBPPP'
            'ELELELELLLELELELELLLEEEEEL' 'LEEEEEEEEEEEEEEEEEEEEEEEE.')
DOT_PLAN = ('11221121111111112211111222' '22111211211222112211121222'
            '12121211111111111111111111' '11111111111111121111111111'
            + ('11111112111211111112111121' '11211111111111111211111111') * 4
            + '11121211112211111211111111' '11211111111111111111111111'
            '11111111111111111111111111' '11111111111111111111111111')


def _dot(a, b, dims):
    return lax.dot_general(a, b, dims, preferred_element_type=F32)


def _unpack(words):
    return pltpu.bitcast(words, BF)


def _rnd(v):
    return v.astype(BF).astype(F32)


def _rcp(v):
    return pltpu.reciprocal(v, approx=True)


def _silu(v):
    h = 0.5 * v
    return h + h * jnp.tanh(h)


def _total(v):
    while len(v) > 1:
        v = [v[i] + v[i + 1] for i in range(0, len(v), 2)]
    return v[0]


def _pair_reduce(v, reduce, op):
    r = reduce(v, axis=0)
    r = op(r, pltpu.roll(r, 2, 0))
    return op(r, pltpu.roll(r, 4, 0))


def _dual_exp(p):
    v = p.reshape(8, 8, L)
    ep = jnp.exp2(v - _pair_reduce(v, jnp.max, jnp.maximum))
    en = jnp.exp2(_pair_reduce(v, jnp.min, jnp.minimum) - v)
    return ep, en, _pair_reduce(ep, jnp.sum, jnp.add), _pair_reduce(en, jnp.sum, jnp.add)


def _key_features(p):
    ep, en, sp, sn = _dual_exp(p)
    return jnp.concatenate([ep * _rcp(sp), en * _rcp(sn)], axis=0).reshape(L, L).astype(BF)


def _query_features(p):
    ep, en, sp, sn = _dual_exp(p)
    return jnp.concatenate([ep, en * (sp * _rcp(sn))], axis=0).reshape(L, L).astype(BF), sp


class _Signed:
    def __init__(self, sign, v):
        self.sign, self.v = sign, v

    def __neg__(self):
        return _Signed(-self.sign, self.v)

    def __add__(self, o):
        if self.sign == o.sign:
            return _Signed(self.sign, self.v + o.v)
        return _Signed(1, self.v - o.v if self.sign > 0 else o.v - self.v)

    def __sub__(self, o):
        return self + (-o)


def _nxt(k, d=1):
    return (k - 1 + d) % 3 + 1


def _operands(block, left):
    lo, hi = (1, 2) if left else (2, 1)

    def forms(i):
        x, y = block(i)
        if left:
            return {1: _Signed(1, x), 2: _Signed(-1, y), 3: _Signed(1, y - x)}
        return {1: _Signed(1, y), 2: _Signed(1, x), 3: _Signed(-1, x + y)}

    def diag(g, k):
        yield g[_nxt(k, lo)]
        yield g[_nxt(k, hi)]

    def pair(ga, gb, k, s):
        m = _nxt(k, 2)
        yield gb[k] - ga[_nxt(k)] if left else ga[_nxt(k)] - gb[k]
        for n in (_nxt(m, lo), _nxt(m, hi)):
            s[n] = ga[n] + gb[n]
            yield s[n]

    f0 = forms(0)
    yield from diag(f0, 1)
    f1 = forms(1)
    yield from diag(f1, 2)
    yield from pair(f0, f1, 1, {})
    f2 = forms(2)
    yield from diag(f2, 3)
    yield from pair(f1, f2, 2, {})
    s02 = {}
    yield from pair(f2, f0, 3, s02)
    s02[2] = f0[2] + f2[2]
    f3 = forms(3)
    yield from diag(f3, 1)
    yield from pair(f2, f3, 3, {})
    yield from pair(f3, s02, 1, {})
    yield from pair(f3, f1, 1, {})


_SIGNS = [a.sign * b.sign for a, b in zip(_operands(lambda i: (0, 0), True), _operands(lambda i: (0, 0), False))]


def _block_product(product):
    count = iter(range(NOP))

    def m(sign=1):
        k = next(count)
        return _Signed(sign * _SIGNS[k], product(k))

    def diag(i):
        x, y = m(), m(-1)
        yield i, i, x + y
        return x, y

    def pair(a, b, da, db, less=(None, None)):
        g = m()
        xs = m()
        ab = xs - da[1] - db[1] - g
        yield a, b, ab if less[0] is None else ab - less[0]
        ys = m(-1)
        ba = ys - da[0] - db[0] + g
        yield b, a, ba if less[1] is None else ba - less[1]
        return (xs, ys), (ab, ba)

    def steps():
        d0 = yield from diag(0)
        d1 = yield from diag(1)
        yield from pair(0, 1, d0, d1)
        d2 = yield from diag(2)
        yield from pair(1, 2, d1, d2)
        d02, _ = yield from pair(2, 0, d2, d0)
        d3 = yield from diag(3)
        _, (c23, c32) = yield from pair(2, 3, d2, d3)
        yield from pair(3, 0, d3, d02, (c32, c23))
        yield from pair(3, 1, d3, d1)

    for i, j, c in steps():
        assert c.sign > 0
        yield i, j, c.v


class _Tasks:
    def __init__(self):
        self.q = []

    def add(self, gen):
        self.q.append(gen)

    def step(self, n=1):
        while n > 0 and self.q:
            try:
                next(self.q[0])
                n -= 1
            except StopIteration:
                self.q.pop(0)

    def drain(self):
        while self.q:
            self.step()


def _kernel(x_hbm, wqkv_hbm, wphi_hbm, wo_hbm, wr_hbm, wg_hbm, wu_hbm, wd_hbm, out_hbm,
            wide, w_v, wphi_v, wr_v, fm_v, part, st, ar, stage, oa0, oa1, kvl, kv_acc, out_v, xb, ob, hb, sems):

    def x_rows(row0, rows):
        return x_hbm.at[0, pl.ds(row0, rows)], wide.at[pl.ds(row0, rows)]

    def w_cols(c):
        return wqkv_hbm.at[:, pl.ds(c * L, L)], w_v.at[c]

    def kv_cols(gp):
        return [w_cols(o + g) for g in (2 * gp, 2 * gp + 1) for o in (NG, 2 * NG)]

    def phi_heads(h0, heads):
        return wphi_hbm.at[pl.ds(h0, heads)], wphi_v.at[pl.ds(h0, heads)]

    def ffn_chunk(c):
        cols = pl.ds(c * FC, FC)
        rows = pl.ds(GU + c * D, D)
        return [(wg_hbm.at[:, cols], wide.at[rows, pl.ds(0, FC)]),
                (wu_hbm.at[:, cols], wide.at[rows, pl.ds(FC, FC)]),
                (wd_hbm.at[cols], wide.at[pl.ds(WD + c * FC, FC)])]

    loads = {
        'x00': [(wr_hbm, wr_v), x_rows(0, L)],
        'x01': [x_rows(L, L)],
        'x02': [x_rows(2 * L, L)],
        'x03': [x_rows(3 * L, L)],
        'kv0a': [phi_heads(0, 8)] + kv_cols(0)[:2],
        'kv0b': kv_cols(0)[2:],
        'kv1': [phi_heads(8, H - 8)] + kv_cols(1),
        'kv2': kv_cols(2),
        'kv3': [x_rows(TT, TT)] + kv_cols(3),
        'wo': [x_rows(n * TT, TT) for n in range(2, NTILE)] + [(wo_hbm, wide.at[pl.ds(WO, D)])],
        'wq': [w_cols(g) for g in range(NG)] + [p for c in range(EARLY) for p in ffn_chunk(c)],
        'ffn': [p for c in range(EARLY, NFC) for p in ffn_chunk(c)],
    }

    def copies(name):
        return [pltpu.make_async_copy(src, dst, sems.at[list(loads).index(name)]) for src, dst in loads[name]]

    def wait(name):
        for cp in copies(name):
            cp.wait()

    def out_copy(src0, dst0, rows, col0, cols, sem):
        return pltpu.make_async_copy(out_v.at[pl.ds(src0, rows), pl.ds(col0, cols)],
                                     out_hbm.at[0, pl.ds(dst0, rows), pl.ds(col0, cols)], sems.at[sem])

    for name in loads:
        for cp in copies(name):
            cp.start(priority=1)

    ar_w = ar.bitcast(U32)
    stored = set()
    ready = set()

    wait('x00')
    wr1 = wr_v[...].astype(F32).reshape(1, D)
    zero = pl.multiple_of(jnp.max(jnp.where(jnp.abs(wr1) < 0.0, pltpu.bitcast(wr1, jnp.int32), 0)), 16)
    never = zero > 0
    ar[pl.ds(SPARE, 16), :] = jnp.zeros((16, L), BF)
    part[NPART] = jnp.zeros((8, L), F32)
    st[64] = jnp.zeros((16, L), F32)
    stage[32, pl.ds(0, 16), :] = jnp.zeros((16, L), BF)
    for oa in (oa0, oa1):
        oa[OSPARE, pl.ds(0, 16), :] = jnp.zeros((16, L), BF)

    def fold_matrices(groups):
        rr = lax.broadcasted_iota(jnp.int32, (L, DH), 0)
        ff = lax.broadcasted_iota(jnp.int32, (L, DH), 1)
        sel = jnp.where(((rr & 63) >> 1) == ff, 1.0, 0.0).astype(BF)
        r2 = lax.broadcasted_iota(jnp.int32, (L, L), 0)
        c2 = lax.broadcasted_iota(jnp.int32, (L, L), 1)
        own = ((r2 >> 6) * 2 + (r2 & 1)) == (c2 >> 5)
        for g in groups:
            a = wphi_v[4 * g:4 * g + 4].reshape(L, DH)
            fm_v[g] = jnp.where(own, _dot(sel, a, NT), 0.0).astype(BF)

    def put(row, v):
        stored.add('ar')
        ar[pl.ds(row, v.shape[0]), :] = v.astype(BF)

    def slabs(start, stride, k, row0, rows):
        return jnp.concatenate(
            [ar_w[pl.ds((start + s * stride) // 2 + k * (KH * stride // 2) + row0, rows // 2), :]
             for s in range(KH)], axis=1)

    def folded(g, c, s):
        w = _unpack(w_v.bitcast(U32)[c, pl.ds(s * L // 2, L // 2), :])
        return _dot(_unpack(fm_v.bitcast(U32)[g]), w, NT) * (2.0 * LOG2E)

    def build(load, store, slots=range(NOP)):
        for r0 in range(0, L, 16):
            for k, v in enumerate(_operands(lambda i: [load(k, r0).astype(F32) for k in RAWL[i]], True)):
                if k in slots and k not in STAGE:
                    store(k, r0, v.v)
                if k == slots[-1]:
                    break
            yield

    def arena_build(row_of, slots=range(NOP)):
        return build(lambda k, r0: stage[row_of(k)[1], pl.ds(r0, 16), :],
                     lambda k, r0, v: put(row_of(k)[0] + r0, v), slots)

    def put_plain(row_of, k, v):
        stored.add('stage')
        v = v.astype(BF)
        stage[row_of(k)[1]] = v
        if k < NOP:
            ar[pl.ds(row_of(k)[0], L), :] = v

    def kv_rows(gp, s):
        return lambda k: (AKV + ((k * KH + s) * 4 + gp) * L, 8 * s + STAGE.get(k, 0))

    def plain_kv(gp, s, which=(0, 1)):
        for i in which:
            g = 2 * gp + i
            for h in range(2):
                put_plain(kv_rows(gp, s), RAWL[2 * i][h], folded(g, NG + g, h * KH + s))
                put_plain(kv_rows(gp, s), RAWL[2 * i + 1][h], w_v[2 * NG + g, pl.ds(h * HK + s * L, L), :].T)

    def prep_kv(gp):
        for s in range(KH):
            plain_kv(gp, s)
            yield
            yield from arena_build(kv_rows(gp, s))

    def q_groups(gp):
        return (2 * gp, KH + 2 * gp, 2 * gp + 1, KH + 2 * gp + 1)

    def prep_q():
        for gp in range(2):
            for s in range(KH):
                def row_of(k):
                    return AQ + ((k * KH + s) * 2 + gp) * L, 8 * s + STAGE.get(k, 0)
                for i, g in enumerate(q_groups(gp)):
                    for h in range(2):
                        put_plain(row_of, RAWL[i][h], folded(g, g, h * KH + s))
                    if i % 2:
                        yield
                yield from arena_build(row_of)
            ready.add(('q', gp))

    def prep_o():
        for c in range(2):
            for r0 in range(0, HK, 16):
                blk = [wide[pl.ds(WO + h * HK + r0, 16), pl.ds(c * HK, HK)].astype(F32) for h in range(2)]
                for k, v in enumerate(_operands(lambda j: [b[:, j * L:(j + 1) * L] for b in blk], False)):
                    put(BO + (k * 2 + c) * HK + r0, v.v)
                yield

    wr = jnp.broadcast_to(wr1, (16, D))
    best = [jnp.full((16, 1), -jnp.inf, F32), jnp.zeros((16, 1), jnp.int32)]

    def row_mean(n, c, j):
        xf = wide[pl.ds(n * TT + j * L + c * 16, 16), :].astype(F32)
        mean = jnp.sum(xf, axis=1, keepdims=True) * (1.0 / D)
        stored.add('st')
        st[8 * c + 2 * j] = jnp.broadcast_to(mean, (16, L))

    def row_stats(n, c, j):
        r0 = n * TT + j * L + c * 16
        d = wide[pl.ds(r0, 16), :].astype(F32) - jnp.concatenate([st[8 * c + 2 * j]] * (D // L), axis=1)
        var = jnp.sum(d * d, axis=1, keepdims=True) * (1.0 / D)
        rs = _rcp(_rnd(jnp.sqrt(_rnd(_rnd(var) + 1e-5))))
        r = jnp.sum(d * wr, axis=1, keepdims=True) * rs
        up = (r > best[0]) | ((r == best[0]) & (r0 < best[1]))
        best[0] = jnp.where(up, r, best[0])
        best[1] = jnp.where(up, r0, best[1])
        stored.add('st')
        st[8 * c + 2 * j + 1] = jnp.broadcast_to(0.5 * rs, (16, L))
        st[64, pl.ds(8, 8), :] = jnp.broadcast_to(jnp.maximum(best[0][:8], best[0][8:]), (8, L))

    def token_operands(n, c, s):
        row = XS + s * XR + n * L + c * 16

        def block(j):
            mean, scale = st[8 * c + 2 * j], st[8 * c + 2 * j + 1]
            b = [(wide[pl.ds(n * TT + j * L + c * 16, 16), pl.ds(h * HK + s * L, L)].astype(F32) - mean) * scale
                 for h in range(2)]
            for k, v in zip(RAW[j], b):
                if k >= NOP:
                    put(row + k * KH * XR, v)
            return b

        for k, v in enumerate(_operands(block, False)):
            put(row + k * KH * XR, v.v)

    def layernorm(n):
        for j in range(4):
            row_mean(n, 0, j)
        yield
        for c in range(L // 16):
            for j in range(4):
                row_stats(n, c, j)
                if j % 2:
                    yield
            if c + 1 < L // 16:
                for j in range(4):
                    row_mean(n, c + 1, j)
                yield
            for s in range(KH):
                token_operands(n, c, s)
                yield

    side, prep, tail, tail2, extra = _Tasks(), _Tasks(), _Tasks(), _Tasks(), _Tasks()
    count = [0]
    plan = [FIRST_PLAN, 0]
    delay = [1]
    timed, pending, dots, flush = {}, [], {}, []
    release = [stage.at[32]]

    def anchor(v):
        wide[pl.ds(ANCHOR + zero, 8), pl.ds(0, 2 * L)] = v.astype(BF)

    def probe(name):
        if name == 'ar':
            return ar_w[pl.ds(SPARE // 2 + zero, 8), :]
        if name == 'part':
            return pltpu.bitcast(part[NPART + zero], U32)
        if name == 'st':
            return pltpu.bitcast(st[64, pl.ds(zero, 8), :], U32)
        if name == 'stage':
            return stage.bitcast(U32)[32, pl.ds(zero, 8), :]
        return (oa0, oa1)[name == 'oa1'].bitcast(U32)[OSPARE, pl.ds(zero, 8), :]

    def gap(m):
        count[0] += 1
        for action in timed.pop(count[0], ()):
            action()
        due = pending.pop(0) if len(pending) > delay[0] else ()
        if due:
            tied = pltpu.bitcast(m[96:104], U32)
            for name in due:
                tied = jnp.where(never, probe(name), tied)
            m = jnp.concatenate([m[:96], pltpu.bitcast(tied, F32), m[104:]], axis=0)
        if side.q or prep.q or extra.q:
            anchor(jnp.concatenate([m[:8], m[8:16]], axis=1))
        if prep.q:
            release[0][pl.ds(zero + 16, 16), :] = m[:16].astype(BF)
        tail.step(dots.get(count[0], 1))
        tail2.step()
        todo = plan[0][(count[0] - plan[1] - 1) % len(plan[0])]
        side.step(PIECES[todo][0])
        prep.step(PIECES[todo][1])
        extra.step(todo == 'E')
        pending.append(sorted(stored))
        stored.clear()
        return m

    def soon(action):
        timed.setdefault(count[0] + 1, []).append(action)

    def after(products, gen):
        start = count[0] + products

        def held():
            while count[0] < start and not flush:
                yield
            yield from gen
        return held()

    def drain_tail():
        flush.append(1)
        tail.drain()
        flush.clear()

    def unit(lhs, rhs, dims, on_block):
        for i, j, c in _block_product(lambda k: gap(_dot(_unpack(lhs(k)), _unpack(rhs(k)), dims))):
            on_block(i, j, c)

    route = {}

    def router():
        slot = lax.broadcasted_iota(jnp.int32, (16, 1), 0)
        lane_rows = lax.broadcasted_iota(jnp.int32, (16, D), 0)
        rows = jnp.zeros((16, D), F32)
        for i in range(16):
            group = pl.multiple_of(jnp.max(jnp.where(slot == i, best[1], 0)), 16)
            rows = jnp.where(lane_rows == i, wide[pl.ds(group, 16), :].astype(F32), rows)
        mean = jnp.sum(rows, axis=1, keepdims=True) * (1.0 / D)
        var = jnp.sum((rows - mean) * (rows - mean), axis=1, keepdims=True) * (1.0 / D)
        xn = _rnd(_rnd(rows - _rnd(mean)) / _rnd(jnp.sqrt(_rnd(_rnd(var) + 1e-5))))
        score = _rnd(jnp.sum(xn * wr, axis=1, keepdims=True))
        rmax = jnp.max(score)
        idx = jnp.min(jnp.where(score == rmax, best[1] + slot, S - 1))
        row = jnp.sum(jnp.where(lane_rows == idx % 16, xn, 0.0), axis=0, keepdims=True)
        route.update(rmax=rmax, idx=idx, row=row, tile=idx // TT, block=(idx // L) % 4,
                     word=pl.multiple_of(((idx % L) // 16) * 8, 8))
        for t in range(D // L):
            xb[pl.ds(t * L, L), :] = jnp.broadcast_to(row[:, t * L:(t + 1) * L], (L, L)).T
            yield

    def matvec(row0, col0, vec, k0, slot):
        vk = vec[pl.ds(k0, FROWS), :]
        wk = wide[pl.ds(row0 + k0, FROWS), pl.ds(col0, 2 * L)].astype(F32)
        pr = wk * jnp.concatenate([vk, vk], axis=1)
        acc = jnp.sum(pr.reshape(FROWS // 8, 8, 2 * L), axis=0)
        stored.add('part')
        for t in range(2):
            part[slot(t)] = acc[:, t * L:(t + 1) * L]

    def ffn():
        def gu_slot(c, t, p):
            return ((c % 2) * 8 + t) * 2 * NSUB + p

        def y_slot(c, t, p):
            return 32 * NSUB + (t * NFC + c) * NSUB + p

        def column(c, t):
            return jnp.sum(_total([part[gu_slot(c, t, p)] for p in range(2 * NSUB)]), axis=0, keepdims=True)

        def down(c):
            for t in range(0, 8, 2):
                for p in range(NSUB):
                    matvec(WD + c * FC, t * L, hb.at[c], p * FROWS, lambda u: y_slot(c, t + u, p))
                    yield

        for c in range(NFC):
            while c == EARLY and 'ffn' not in ready:
                yield
            for t in range(0, 8, 2):
                for p in range(2 * NSUB):
                    matvec(GU + c * D, t * L, xb, p * FROWS, lambda u: gu_slot(c, t + u, p))
                    yield
            for t in range(4):
                gate, up = column(c, t), column(c, 4 + t)
                hb[c, pl.ds(t * L, L), :] = jnp.broadcast_to(_silu(gate) * up, (L, L)).T
            yield
            if c > 0:
                yield from down(c - 1)
        yield
        yield from down(NFC - 1)
        y = [sum(_total([part[y_slot(c, t, p)] for p in range(NSUB)]) for c in range(NFC)) for t in range(8)]
        gate = 1.0 / (1.0 + jnp.exp(-jnp.full((1, D), route['rmax'], F32)))
        route['y'] = jnp.sum(jnp.concatenate(y, axis=1), axis=0, keepdims=True) * gate

    def finish_pair(p, sums):
        r = lax.broadcasted_iota(jnp.int32, (80, L), 0)
        c = lax.broadcasted_iota(jnp.int32, (80, L), 1)
        keep = jnp.where(r < 64, r >> 5, r & 1) == (c & 1)
        kvl[p] = jnp.where(keep, jnp.concatenate([2.0 * sums[:64], sums[64:]], axis=0), 0.0).astype(BF)

    def kv_unit(gp, n):
        seen, acc = {}, {}

        def combine(g, phis, vts):
            for pp in range(2):
                p = 2 * g + pp
                acc[p] = acc.get(p, []) + [_dot(vts[pp], phis[pp], NT)]
                if len(acc[p]) == 4:
                    upd = _total(acc[p]) if n == 0 else kv_acc[p] + _total(acc[p])
                    if n < NTILE - 1:
                        kv_acc[p] = upd
                    else:
                        finish_pair(p, upd)
                yield

        def on_block(i, j, c):
            if i % 2:
                seen[i, j] = [jnp.concatenate([c[pp * 64:(pp + 1) * 64], jnp.ones((16, L), F32)], axis=0).astype(BF)
                              for pp in range(2)]
            else:
                seen[i, j] = [_key_features(c[pp * 64:(pp + 1) * 64]) for pp in range(2)]
            if (i ^ 1, j) in seen:
                tail.add(after(3, combine(2 * gp + i // 2, seen[i & 2, j], seen[i | 1, j])))

        def weights(k):
            while (gp, n) == (0, 0) and k in (7, 15) and k not in ready:
                prep.step()
            return slabs(AKV, 4 * L, k, gp * L // 2, L)

        unit(weights, lambda k: slabs(XS, XR, k, n * L // 2, L), NT, on_block)

    def first_tokens():
        for j in range(4):
            if j:
                wait(f'x0{j}')
            for part_of in (row_mean, row_stats):
                for c in range(L // 16):
                    part_of(0, c, j)
                anchor(jnp.zeros((8, 2 * L), BF))
        done = []
        for c in range(L // 16):
            for s in range(KH):
                if len(done) == 28:
                    wait('kv0a')
                    fold_matrices(range(2))
                    for t in range(KH):
                        plain_kv(0, t, (0,))
                        prep.add(arena_build(kv_rows(0, t), range(7)))
                if len(done) >= 3:
                    anchor(jnp.concatenate([done[-3], done[-3]], axis=1))
                token_operands(0, c, s)
                prep.step(2)
                done.append(pltpu.bitcast(probe('ar'), F32))
        prep.drain()

    def more_weights():
        while count[0] < 3:
            yield
        wait('kv0b')
        for s in range(KH):
            plain_kv(0, s, (1,))
            yield
        for slots in (range(7, 15), range(15, NOP)):
            for s in range(KH):
                yield from arena_build(kv_rows(0, s), slots)
            ready.add(slots[0])
        while count[0] < 16:
            yield
        wait('kv1')
        fold_matrices(range(2, NG))
        yield from prep_kv(1)

    def start_side_work(n, gp):
        if (n, gp) == (0, 1):
            wait('kv2')
            prep.add(prep_kv(2))
            plan[0] = TILE0_PLAN
        elif (n, gp) == (0, 2):
            wait('kv3')
            prep.add(prep_kv(3))
            side.add(layernorm(1))
        elif n > 0 and gp == 0:
            plan[0] = NORM_PLAN
            delay[0] = 2
            if n == 1:
                wait('wo')
                prep.add(prep_o())
            if n + 1 < NTILE:
                side.add(layernorm(n + 1))
            else:
                wait('wq')
                plan[0] = QUERY_PLAN
                side.add(router())
                side.add(ffn())
                prep.add(prep_q())

    first_tokens()
    prep.add(more_weights())
    for n in range(NTILE):
        for gp in range(4):
            if n == 0 and gp:
                prep.drain()
            if n and not gp:
                side.drain()
            soon(lambda n=n, gp=gp: start_side_work(n, gp))
            kv_unit(gp, n)

    built = {}

    caught = [jnp.zeros((8, L), U32)] * (2 * KH)

    def catch_row(n, gp):
        for slab in (2 * gp, 2 * gp + 1):
            for h in range(2):
                k = sum(jnp.where(route['block'] == j, RAWL[j][h], 0) for j in range(4))
                words = (oa0, oa1)[n % 2].bitcast(U32)[k * KH + slab, pl.ds(route['word'], 8), :]
                caught[h * KH + slab] = jnp.where(route['tile'] == n, words, caught[h * KH + slab])

    def routed_projection():
        hit = lax.broadcasted_iota(jnp.int32, (16, L), 0) == route['idx'] % 16
        for t in range(2 * KH):
            row = jnp.sum(jnp.where(hit, _unpack(caught[t]).astype(F32), 0.0), axis=0, keepdims=True)
            ob[pl.ds(t * L, L), :] = jnp.broadcast_to(row, (L, L)).T
            if t % 2:
                yield
        for t in range(0, 8, 2):
            for p in range(2 * NSUB):
                matvec(WO, t * L, ob, p * FROWS, lambda u: OPART + (t + u) * 2 * NSUB + p)
                yield
        s = [_total([part[OPART + t * 2 * NSUB + p] for p in range(2 * NSUB)]) for t in range(8)]
        route['s'] = jnp.sum(jnp.concatenate(s, axis=1), axis=0, keepdims=True)

    def o_operands(n, gp):
        oa = (oa0, oa1)[n % 2]
        release[0] = oa.at[OSPARE]
        for slab in (2 * gp, 2 * gp + 1):
            def store(k, r0, v):
                stored.add(f'oa{n % 2}')
                oa[k * KH + slab, pl.ds(r0, 16), :] = v.astype(BF)
            yield from build(lambda k, r0: oa[k * KH + slab, pl.ds(r0, 16), :], store)
        built[n] = built.get(n, 0) + 1

    def q_unit(gp, n):
        while ('q', gp) not in ready:
            prep.step()
        left = [16]
        oa = (oa0, oa1)[n % 2]

        def attend(i, j, feats):
            rows = []
            for pp, (phi, scale) in enumerate(feats):
                nd = _dot(_unpack(kvl.bitcast(U32)[2 * q_groups(gp)[i] + pp]), phi, NN)
                inv = _rcp(nd[64:72] + 1e-6 * scale)
                rows += [nd[head * DH:(head + 1) * DH] * inv[head:head + 1] for head in range(2)]
                if pp == 0:
                    yield
            oa[RAWL[j][i % 2] * KH + 2 * gp + i // 2] = jnp.concatenate(rows, axis=0).T.astype(BF)
            left[0] -= 1
            if not left[0]:
                catch_row(n, gp)
                prep.add(o_operands(n, gp))
                if (n, gp) == (NTILE - 1, 1):
                    extra.add(routed_projection())
            yield

        def on_block(i, j, c):
            tail.add(after(4, attend(i, j, [_query_features(c[pp * 64:(pp + 1) * 64]) for pp in range(2)])))

        unit(lambda k: slabs(AQ, 2 * L, k, gp * L // 2, L),
             lambda k: slabs(XS, XR, k, n * L // 2, L), NT, on_block)

    def o_unit(c, n):
        left = [16]

        def finish(j, col, s):
            rows = pl.ds(n * TT + j * L, L)
            cols = pl.ds(c * HK + col * L, L)
            half = ar[pl.ds(XS + (RAW[j][c] * KH + col) * XR + n * L, L), :].astype(F32)
            sh = s * half
            out_v[rows, cols] = (wide[rows, cols].astype(F32) + sh + sh * jnp.tanh(half)).astype(BF)
            left[0] -= 1
            if (n, c) == (NTILE - 1, 1):
                out_copy(rows.start, rows.start, L, cols.start, L, 1).start()
            elif not left[0]:
                out_copy(n * TT, n * TT, TT, c * HK, HK, int(n == NTILE - 1)).start()
            yield

        if c == 0:
            if n == NTILE - 1:
                drain_tail()
            while built.get(n, 0) < 2:
                (prep if prep.q else tail).step()
        oa = (oa0, oa1)[n % 2].bitcast(U32)
        unit(lambda k: jnp.concatenate([oa[k * KH + s] for s in range(KH)], axis=1),
             lambda k: ar_w[pl.ds((BO + (k * 2 + c) * HK) // 2, HK // 2), :], NN,
             lambda j, col, s: tail2.add(finish(j, col, s)))

    dots.update((count[0] + 1 + t, int(n)) for t, n in enumerate(DOT_PLAN))
    plan[:] = [OUT_PLAN, count[0]]
    delay[0] = 1
    q_unit(0, 0)
    soon(lambda: wait('ffn'))
    soon(lambda: ready.add('ffn'))
    q_unit(1, 0)
    for n in range(1, NTILE):
        for gp in range(2):
            q_unit(gp, n)
            o_unit(gp, n - 1)
    for c in range(2):
        o_unit(c, NTILE - 1)
    drain_tail()
    tail2.drain()
    side.drain()
    extra.drain()

    row0 = pl.multiple_of((route['idx'] // 16) * 16, 16)
    half = 0.5 * (route['row'] + route['y'])
    sh = route['s'] * half
    fixed = wide[pl.ds(row0, 16), :].astype(F32) + (sh + sh * jnp.tanh(half))
    hit = lax.broadcasted_iota(jnp.int32, (16, D), 0) == route['idx'] % 16
    out_v[pl.ds(S, 16), :] = jnp.where(hit, fixed, out_v[pl.ds(row0, 16), :].astype(F32)).astype(BF)
    rows_copy = out_copy(S, row0, 16, 0, D, 2)
    for _ in range(2 * NTILE - 2):
        out_copy(0, 0, TT, 0, HK, 0).wait()
    pl.when(route['tile'] != NTILE - 1)(rows_copy.start)
    out_copy(0, 0, TT, 0, HK, 1).wait()
    for _ in range(16):
        out_copy(0, 0, L, 0, L, 1).wait()
    pl.when(route['tile'] == NTILE - 1)(rows_copy.start)
    rows_copy.wait()


@jax.jit
def pallas_recurrent_scan__linear_kernel_hedgehog__moe_arch_mod__prompt_kernel(
    A_x: jax.Array,
    A_wqkv: jax.Array,
    A_w_phi: jax.Array,
    A_wo: jax.Array,
    B_x: jax.Array,
    B_w_r: jax.Array,
    B_w_gate: jax.Array,
    B_w_up: jax.Array,
    B_w_down: jax.Array,
):
    del B_x
    hbm = pl.BlockSpec(memory_space=pl.ANY)
    return pl.pallas_call(
        _kernel,
        out_shape=jax.ShapeDtypeStruct(A_x.shape, A_x.dtype),
        in_specs=[hbm] * 8,
        out_specs=hbm,
        scratch_shapes=[
            pltpu.VMEM((ANCHOR + 8, D), BF),
            pltpu.VMEM((3 * NG, D, L), BF),
            pltpu.VMEM((H, DH, DH), BF),
            pltpu.VMEM((D,), BF),
            pltpu.VMEM((NG, L, L), BF),
            pltpu.VMEM((NPART + 1, 8, L), F32),
            pltpu.VMEM((65, 16, L), F32),
            pltpu.VMEM((SPARE + 16, L), BF),
            pltpu.VMEM((33, L, L), BF),
            pltpu.VMEM((OSPARE + 1, L, L), BF),
            pltpu.VMEM((OSPARE + 1, L, L), BF),
            pltpu.VMEM((NP, 80, L), BF),
            pltpu.VMEM((NP, 80, L), F32),
            pltpu.VMEM((S + 16, D), BF),
            pltpu.VMEM((D, L), F32),
            pltpu.VMEM((D, L), F32),
            pltpu.VMEM((NFC, FC, L), F32),
            pltpu.SemaphoreType.DMA((12,)),
        ],
        compiler_params=pltpu.CompilerParams(vmem_limit_bytes=120 << 20),
        name="hedgehog_mod",
    )(A_x, A_wqkv, A_w_phi, A_wo, B_w_r, B_w_gate, B_w_up, B_w_down)
```
